```python
import jax
import jax.numpy as jnp

def _softmax(x, axis=-1):
    return jax.nn.softmax(x, axis=axis)
def _gelu(x):
    return jax.nn.gelu(x, approximate=True)
def _silu(x):
    return jax.nn.silu(x)
def _sigmoid(x):
    return jax.nn.sigmoid(x)
def _layernorm(x, axis=-1, eps=1e-5):
    m = jnp.mean(x, axis=axis, keepdims=True)
    v = jnp.var(x, axis=axis, keepdims=True)
    return (x - m) / jnp.sqrt(v + eps)
def _scatter_add(tgt, idx, src, axis=0):
    return tgt.at[idx].add(src)
def _segment_sum(src, seg, n):
    return jax.ops.segment_sum(src, seg, n)
class _Rng:
    def __init__(self, key):
        self._k = key
    def _next(self):
        self._k, sub = jax.random.split(self._k)
        return sub
    def normal(self, shape):
        return jax.random.normal(self._next(), shape, dtype=jnp.bfloat16)
    def randint(self, lo, hi, shape):
        return jax.random.randint(self._next(), shape, lo, hi, dtype=jnp.int32)
    def uniform(self, shape, lo=0.0, hi=1.0):
        return jax.random.uniform(self._next(), shape, jnp.bfloat16, lo, hi)
    def permutation(self, n):
        return jax.random.permutation(self._next(), n)


kernel_name = 'gated_mix__sliding_local_dilated__glu_gated_reglu__prompt'

def setup_inputs():
    _rng = _Rng(jax.random.key(int.from_bytes(__import__("os").urandom(4), "little")))
    _w = (lambda a: (lambda t: t.astype(jnp.bfloat16) if jnp.issubdtype(t.dtype, jnp.floating) else t)(jnp.asarray(a)))
    def _A_setup():
        B, S, D = 1, 2048, 1024
        return {
            "x": _w((lambda *s: _rng.normal(s) * 0.05)(B, S, D)),
            "wqkv": _w((lambda *s: _rng.normal(s) * 0.05)(D, 3 * D)),
            "wo": _w((lambda *s: _rng.normal(s) * 0.05)(D, D)),
        }
    _A_in = _A_setup()

    def _B_setup():
        B, S, D, F = 1, 2048, 1024, 3584
        return {
            "x": _w((lambda *s: _rng.normal(s) * 0.05)(B, S, D)),
            "W_gate": _w((lambda *s: _rng.normal(s) * 0.05)(D, F) * (2.0 / D) ** 0.5),
            "W_up": _w((lambda *s: _rng.normal(s) * 0.05)(D, F) * (2.0 / D) ** 0.5),
            "W_down": _w((lambda *s: _rng.normal(s) * 0.05)(F, D) * (1.0 / F) ** 0.5),
        }
    _B_in = _B_setup()

    return {
        "A_x": _A_in["x"],
        "A_wqkv": _A_in["wqkv"],
        "A_wo": _A_in["wo"],
        "B_x": _B_in["x"],
        "B_W_gate": _B_in["W_gate"],
        "B_W_up": _B_in["W_up"],
        "B_W_down": _B_in["W_down"],
        "gate_w": _w((lambda *s: _rng.normal(s) * 0.05)(1024)),
    }

def reference(A_x, A_wqkv, A_wo, B_x, B_W_gate, B_W_up, B_W_down, gate_w):
    def _A_ref(x, wqkv, wo):
        B, S, D = x.shape
        H = 32; Dh = D // H
        W, dil = 8, 2
        qkv = (lambda x, *d: x.transpose(*d))((x @ wqkv).reshape(B, S, 3, H, Dh), 2, 0, 3, 1, 4)
        q, k, v = qkv[0], qkv[1], qkv[2]
        scale = Dh ** -0.5
        pos = jnp.arange(S)
        off = jnp.arange(W) * dil
        idx = pos[:, None] - off[None, :]
        mask = idx >= 0
        idx_c = jnp.where(mask, idx, 0).reshape(-1)
        kg = k[:, :, idx_c, :].reshape(B, H, S, W, Dh)
        vg = v[:, :, idx_c, :].reshape(B, H, S, W, Dh)
        logits = jnp.einsum("bhsd,bhswd->bhsw", q, kg) * scale
        logits = jnp.where(mask[None, None, :, :], logits, -1e9)
        attn = _softmax(logits, axis=-1)
        o = jnp.einsum("bhsw,bhswd->bhsd", attn, vg)
        return (lambda x, *d: x.transpose(*d))(o, 0, 2, 1, 3).reshape(B, S, D) @ wo

    def _B_ref(x, W_gate, W_up, W_down):
        gate = jnp.einsum("bsd,df->bsf", x, W_gate)
        up = jnp.einsum("bsd,df->bsf", x, W_up)
        gate = gate * (lambda x, dt: x.astype(dt))(gate > 0, gate.dtype)
        h = gate * up
        return jnp.einsum("bsf,fd->bsd", h, W_down)

    x = A_x
    g = _sigmoid((x * gate_w).sum(-1, keepdims=True))
    a = _A_ref(x, A_wqkv, A_wo)
    b = _B_ref(x, B_W_gate, B_W_up, B_W_down)
    return g * a + (1 - g) * b
```

```python
import functools
import jax
import jax.numpy as jnp
from jax import lax
import jax.experimental.pallas as pl
import jax.experimental.pallas.tpu as pltpu

S, D, F = 2048, 1024, 3584
H, DH, W, DIL = 32, 32, 8, 2
HALO = 16
LOG2E = 1.4426950408889634
SCALE = DH ** -0.5
BF = jnp.bfloat16
F32 = jnp.float32
U32 = jnp.uint32


def scoped(fn, name, on):
    if not on:
        return fn

    def g(i, c):
        with jax.named_scope(name):
            return fn(i, c)
    return g


def _swap(vs, vbit, lbit, lane):
    out = list(vs)
    sh = 1 << lbit
    hi = (lane & sh) != 0
    for i in range(8):
        if i & (1 << vbit):
            continue
        a, b = vs[i], vs[i | (1 << vbit)]
        out[i] = jnp.where(hi, pltpu.roll(b, sh, 1), a)
        out[i | (1 << vbit)] = jnp.where(hi, b, pltpu.roll(a, 128 - sh, 1))
    return out


def _permute_cols(vs, lane):
    for vb, lb in ((2, 4), (1, 3), (0, 2), (2, 6), (2, 1), (1, 5), (1, 0)):
        vs = _swap(vs, vb, lb, lane)
    out = [None] * 8
    for i in range(8):
        v2, v1, v0 = (i >> 2) & 1, (i >> 1) & 1, i & 1
        out[(v0 << 2) | (v2 << 1) | v1] = vs[i]
    return out


def _dot(a, b):
    return jnp.dot(a, b, preferred_element_type=F32)


def build(prof=False, tiny=True, opieces=4, gw1d=True, rows1=2048):
    tm2 = 256
    rb = 8
    FC = 512
    NFC = F // FC
    XB = 512
    WC = 256
    n2 = S // tm2
    OC = D // opieces
    if tiny:
        NT = 3
    else:
        NT = 1
    SW1 = NT
    SX = NT + 1
    SM = SX + 3
    SD = SM + NFC - 1
    SOUT = SD + 1
    NSEM = SOUT + 1

    def kernel(x_hbm, gw_hbm, wqkv_hbm, wo_hbm, wg_hbm, wu_hbm, wd_hbm, o_hbm,
               x_v, wqkv_v, wqkv_p, wo_v, wo_p, wo_f32, wg_v, wu_v, wd_v, h_v, q_s, k_s, v_s, oa_v, out_v, gw_ref, sems):
        def cp_x(r0, n, s):
            return pltpu.make_async_copy(x_hbm.at[pl.ds(r0, n)], x_v.at[pl.ds(r0, n)], sems.at[s])

        def cp_w(c0, n, s):
            c = pl.ds(c0, n)
            return [pltpu.make_async_copy(wg_hbm.at[:, c], wg_v.at[:, c], sems.at[s]),
                    pltpu.make_async_copy(wu_hbm.at[:, c], wu_v.at[:, c], sems.at[s])]

        cp_qo = [pltpu.make_async_copy(wqkv_hbm, wqkv_v, sems.at[SM]),
                 pltpu.make_async_copy(wo_hbm, wo_v, sems.at[SM])]
        cp_d = [pltpu.make_async_copy(wd_hbm, wd_v, sems.at[SD]),
                pltpu.make_async_copy(gw_hbm, gw_ref, sems.at[SD])]

        if tiny:
            first = [[cp_x(0, 256, 0)] + cp_w(0, 128, 0), cp_w(128, 128, 1), [cp_x(256, 256, 2)]]
        else:
            first = [[cp_x(0, XB, 0)] + cp_w(0, WC, 0)]
        starts = sum(first, []) + cp_w(WC, WC, SW1)
        starts += [cp_x(b * XB, XB, SX + b - 1) for b in range(1, 4)]
        starts += cp_w(FC, FC, SM) + cp_qo
        for j in range(2, NFC):
            starts += cp_w(j * FC, FC, SM + j - 1)
        starts += cp_d
        for c in starts:
            c.start()

        k_s[:, 0:HALO, :] = jnp.zeros((8, HALO, 128), F32)
        v_s[:, 0:HALO, :] = jnp.zeros((8, HALO, 128), F32)

        def ffn_up(rows, c0, n):
            xx = x_v[rows, :]
            c = pl.ds(c0, n)
            gt = _dot(xx, wg_v[:, c])
            up = _dot(xx, wu_v[:, c])
            hh = (jnp.maximum(gt, 0.0) * up).astype(BF)
            t0 = c0 // 128
            for t in range(n // 128):
                h_v[t0 + t, rows, :] = hh[:, t * 128:(t + 1) * 128]

        if tiny:
            def warm0(u, carry):
                for k in range(3):
                    @pl.when(u == k)
                    def _():
                        for c in first[k]:
                            c.wait()
                ffn_up(pl.ds(pl.multiple_of((u // 2) * 256, 256), 256), pl.multiple_of((u % 2) * 128, 128), 128)
                return carry
            lax.fori_loop(0, 4, scoped(warm0, 'warm0', prof), 0)

        def warm(u, carry):
            b = u // 2
            half = u % 2
            if not tiny:
                @pl.when(u == 0)
                def _():
                    for c in first[0]:
                        c.wait()

            @pl.when(u == 1)
            def _():
                for c in cp_w(WC, WC, SW1):
                    c.wait()

            @pl.when(jnp.logical_and(half == 0, u > 0))
            def _():
                cp_x(pl.multiple_of(b * XB, XB), XB, SX + b - 1).wait()

            ffn_up(pl.ds(pl.multiple_of(b * XB, XB), XB), pl.multiple_of(half * WC, WC), WC)
            return carry
        lax.fori_loop(1 if tiny else 0, 8, scoped(warm, 'warm', prof), 0)

        lane = lax.broadcasted_iota(jnp.int32, (8, 128), 1)

        def main1(j, carry):
            @pl.when(j == 1)
            def _():
                for c in cp_qo:
                    c.wait()
            c0 = pl.multiple_of(j * FC, FC)
            for c in cp_w(c0, FC, SM + j - 1):
                c.wait()

            zv = jnp.full((8, 128), lax.shift_right_logical(j, 20), jnp.int32).astype(U32)
            p = j - 1
            m = p // 2
            hf = p % 2
            deps = []
            for rr in range(0, 512, 16):
                r0 = pl.multiple_of(hf * 512 + rr, 16)
                vs = [pltpu.bitcast(wqkv_v[pl.ds(r0, 16), pl.ds(pl.multiple_of(m * D + cc * 128, 128), 128)], U32)
                      for cc in range(8)]
                vs = _permute_cols(vs, lane)
                for cc in range(8):
                    wqkv_p[m * 8 + cc, pl.ds(r0, 16), :] = pltpu.bitcast(vs[cc], BF)
                deps.append(vs[7] & zv)
            for r0 in range(0, S, rows1):
                ffn_up(slice(r0, r0 + rows1), c0, FC)
            cbs = [jnp.minimum(2 * p + t, 7) for t in range(2)]
            for t in range(2):
                cs = pl.ds(pl.multiple_of(cbs[t] * 128, 128), 128)
                for hh in range(H):
                    for q in range(2):
                        val = pltpu.bitcast(wo_v[hh * 32 + q * 16:hh * 32 + (q + 1) * 16, cs], U32) | deps[hh // 2]
                        wo_f32[t, hh * 33 + q * 16:hh * 33 + (q + 1) * 16, :] = pltpu.bitcast(val, BF).astype(F32)
            for t in range(2):
                for b in range(8):
                    for a in range(4):
                        dep = deps[16 + (b * 4 + a) // 2]
                        for q in range(2):
                            parts = [pltpu.bitcast(pltpu.bitcast(
                                wo_f32[t, pl.ds(a * 8 + b + (q * 16 + e * 8) * 33, 8, stride=33), :], U32) | dep, F32)
                                for e in range(2)]
                            r0 = b * 128 + a * 32 + q * 16
                            wo_p[cbs[t], r0:r0 + 16, :] = jnp.concatenate(parts, axis=0).astype(BF)
            return carry
        lax.fori_loop(1, NFC, scoped(main1, 'main1', prof), 0)

        for c in cp_d:
            c.wait()

        cexp = SCALE * LOG2E

        def main2(i, carry):
            r0 = pl.multiple_of(i * tm2, tm2)
            rows = pl.ds(r0, tm2)
            qkv = _dot(x_v[rows, :], jnp.concatenate([wqkv_p[t] for t in range(24)], axis=1))
            for c in range(8):
                q_s[c] = qkv[:, c * 128:(c + 1) * 128]
                k_s[c, HALO:HALO + tm2, :] = qkv[:, D + c * 128:D + (c + 1) * 128]
                v_s[c, HALO:HALO + tm2, :] = qkv[:, 2 * D + c * 128:2 * D + (c + 1) * 128]
            zs = [lax.shift_right_logical(i, 20), lax.shift_right_logical(i, 21)]
            zv = jnp.full((rb, 128), zs[0], jnp.int32)

            def after(t, dep):
                return pltpu.bitcast(pltpu.bitcast(t, jnp.int32) | (pltpu.bitcast(dep, jnp.int32) & zv), F32)
            den = None
            last_o = None
            pend = [None] * 8
            for gi, r in enumerate(range(0, tm2, rb)):
                z = zs[gi % 2]
                q = [q_s[c, pl.ds(z + r, rb), :] for c in range(8)]
                if gi >= 1:
                    dep = pltpu.bitcast(den, jnp.int32) & zv
                    q = [pltpu.bitcast(pltpu.bitcast(t, jnp.int32) | dep, F32) for t in q]
                s = []
                raw = None
                for w in range(W):
                    st = HALO + r - DIL * w
                    q0 = q[0] if raw is None else after(q[0], raw)
                    acc = q0 * k_s[0, pl.ds(z + st, rb), :]
                    for c in range(1, 8):
                        acc = acc + q[c] * k_s[c, pl.ds(z + st, rb), :]
                    raw = acc
                    acc = acc + pltpu.roll(acc, 64, 1)
                    acc = acc + pltpu.roll(acc, 32, 1)
                    if r < HALO and w > 0:
                        pos = i * tm2 + r + lax.broadcasted_iota(jnp.int32, (rb, 128), 0)
                        acc = jnp.where(pos >= DIL * w, acc, -1e9 / SCALE)
                    s.append(acc)
                m = s[0]
                for w in range(1, W):
                    m = jnp.maximum(m, s[w])
                e = [jnp.exp2((s[w] - m) * cexp) for w in range(W)]
                den = e[0]
                for w in range(1, W):
                    den = den + e[w]
                inv = 1.0 / den
                for c in range(8):
                    st = HALO + r
                    e0 = e[0] if last_o is None else after(e[0], last_o)
                    acc = e0 * v_s[c, pl.ds(z + st, rb), :]
                    for w in range(1, W):
                        st = HALO + r - DIL * w
                        acc = acc + e[w] * v_s[c, pl.ds(z + st, rb), :]
                    last_o = acc
                    acc = acc * inv
                    if gi % 2 == 0:
                        pend[c] = acc
                    else:
                        oa_v[c, r - rb:r + rb, :] = jnp.concatenate([pend[c], acc], axis=0).astype(BF)
            for c in range(8):
                for r in range(0, HALO, rb):
                    k_s[c, r:r + rb, :] = after(k_s[c, tm2 + r:tm2 + r + rb, :], last_o)
                    v_s[c, r:r + rb, :] = after(v_s[c, tm2 + r:tm2 + r + rb, :], last_o)
            b = _dot(jnp.concatenate([h_v[t, rows, :] for t in range(F // 128)], axis=1), wd_v[...])
            if gw1d:
                gw = gw_ref[...].astype(F32).reshape(1, D)
            else:
                gw = gw_ref[...].astype(F32)
            zg = jnp.sum(x_v[rows, :].astype(F32) * gw, axis=-1, keepdims=True)
            g = jax.nn.sigmoid(zg)
            oa = jnp.concatenate([oa_v[c] for c in range(8)], axis=1)
            for pc in range(opieces):
                cs = slice(pc * OC, (pc + 1) * OC)
                a = _dot(oa, jnp.concatenate([wo_p[t] for t in range(pc * OC // 128, (pc + 1) * OC // 128)], axis=1))
                out_v[rows, cs] = (g * a + (1.0 - g) * b[:, cs]).astype(BF)
                pltpu.make_async_copy(out_v.at[rows, cs], o_hbm.at[rows, cs], sems.at[SOUT]).start()
            return carry
        lax.fori_loop(0, n2, scoped(main2, 'main2', prof), 0)
        pltpu.make_async_copy(out_v, o_hbm, sems.at[SOUT]).wait()

    @jax.jit
    def f(A_x, A_wqkv, A_wo, B_x, B_W_gate, B_W_up, B_W_down, gate_w):
        x = A_x.reshape(S, D)
        gw = gate_w if gw1d else gate_w.reshape(1, D)
        anyspec = pl.BlockSpec(memory_space=pl.ANY)
        out = pl.pallas_call(
            kernel,
            in_specs=[anyspec, anyspec, anyspec, anyspec, anyspec, anyspec, anyspec],
            out_specs=anyspec,
            out_shape=jax.ShapeDtypeStruct((S, D), BF),
            scratch_shapes=[
                pltpu.VMEM((S, D), BF),
                pltpu.VMEM((D, 3 * D), BF),
                pltpu.VMEM((24, D, 128), BF),
                pltpu.VMEM((D, D), BF),
                pltpu.VMEM((8, D, 128), BF),
                pltpu.VMEM((2, 1088, 128), F32),
                pltpu.VMEM((D, F), BF),
                pltpu.VMEM((D, F), BF),
                pltpu.VMEM((F, D), BF),
                pltpu.VMEM((F // 128, S, 128), BF),
                pltpu.VMEM((8, tm2, 128), F32),
                pltpu.VMEM((8, tm2 + HALO, 128), F32),
                pltpu.VMEM((8, tm2 + HALO, 128), F32),
                pltpu.VMEM((8, tm2, 128), BF),
                pltpu.VMEM((S, D), BF),
                pltpu.VMEM((D,) if gw1d else (1, D), BF),
                pltpu.SemaphoreType.DMA((NSEM,)),
            ],
            compiler_params=pltpu.CompilerParams(vmem_limit_bytes=110 * 1024 * 1024),
        )(x, gw, A_wqkv, A_wo, B_W_gate, B_W_up, B_W_down)
        return out.reshape(1, S, D)
    return f


_impl = build()


@jax.jit
def pallas_gated_mix__sliding_local_dilated__glu_gated_reglu__prompt_kernel(
    A_x: jax.Array,
    A_wqkv: jax.Array,
    A_wo: jax.Array,
    B_x: jax.Array,
    B_W_gate: jax.Array,
    B_W_up: jax.Array,
    B_W_down: jax.Array,
    gate_w: jax.Array,
):
    return _impl(A_x, A_wqkv, A_wo, B_x, B_W_gate, B_W_up, B_W_down, gate_w)
```

```python
import jax
import jax.numpy as jnp
from jax import lax
import jax.experimental.pallas as pl
import jax.experimental.pallas.tpu as pltpu

S, D, F = 2048, 1024, 3584
H, DH, W, DIL = 32, 32, 8, 2
HALO = 16
LOG2E = 1.4426950408889634
SCALE = DH ** -0.5
BF = jnp.bfloat16
F32 = jnp.float32
U32 = jnp.uint32
I32 = jnp.int32


def scoped(fn, name, on):
    if not on:
        return fn

    def g(i, c):
        with jax.named_scope(name):
            return fn(i, c)
    return g


def _swap(vs, vbit, lbit, lane):
    out = list(vs)
    sh = 1 << lbit
    hi = (lane & sh) != 0
    for i in range(8):
        if i & (1 << vbit):
            continue
        a, b = vs[i], vs[i | (1 << vbit)]
        out[i] = jnp.where(hi, pltpu.roll(b, sh, 1), a)
        out[i | (1 << vbit)] = jnp.where(hi, b, pltpu.roll(a, 128 - sh, 1))
    return out


def _permute_cols(vs, lane):
    for vb, lb in ((2, 4), (1, 3), (0, 2), (2, 6), (2, 1), (1, 5), (1, 0)):
        vs = _swap(vs, vb, lb, lane)
    out = [None] * 8
    for i in range(8):
        v2, v1, v0 = (i >> 2) & 1, (i >> 1) & 1, i & 1
        out[(v0 << 2) | (v2 << 1) | v1] = vs[i]
    return out


def _dot(a, b):
    return jnp.dot(a, b, preferred_element_type=F32)


def _shr(x, n):
    return x >> n if isinstance(x, int) else lax.shift_right_logical(x, n)


def _al(x, n):
    return x if isinstance(x, int) else pl.multiple_of(x, n)


def build(prof=False, opieces=4, rows1=2048, pks='qoha', ring=True, wser=True, pvw=1, qkw=1, qlag=0, order='qkv', gdep=False):
    tm2 = 256
    rb = 8
    FC = 512
    NFC = F // FC
    XB = 512
    WC = 256
    n2 = S // tm2
    OC = D // opieces
    NT = 3
    SW1 = NT
    SX = NT + 1
    SM = SX + 3
    SD = SM + NFC - 1
    SOUT = SD + 1
    NSEM = SOUT + 1

    def st_pk(ref, t, r0, n, val):
        if ref.dtype == U32:
            ref[t, pl.ds(_al(_shr(r0, 1), 8), n // 2), :] = pltpu.bitcast(val, U32)
        else:
            ref[t, pl.ds(r0, n), :] = val

    def ld_pk(ref, t, r0, n):
        if ref.dtype == U32:
            return pltpu.bitcast(ref[t, pl.ds(_al(_shr(r0, 1), 8), n // 2), :], BF)
        return ref[t, pl.ds(r0, n), :]

    def pk_shape(nt, rows, key):
        return pltpu.VMEM((nt, rows // 2, 128), U32) if key in pks else pltpu.VMEM((nt, rows, 128), BF)

    def kernel(x_hbm, gw_hbm, wqkv_hbm, wo_hbm, wg_hbm, wu_hbm, wd_hbm, o_hbm,
               x_v, wqkv_v, wqkv_p, wo_v, wo_p, wo_f32, wg0, wu0, wg_v, wu_v, wd_v, h_v, q_s, k_s, v_s, oa_v, omg_s,
               out_v, gw_ref, sems):
        def cp_x(r0, n, s):
            return pltpu.make_async_copy(x_hbm.at[pl.ds(r0, n)], x_v.at[pl.ds(r0, n)], sems.at[s])

        def cp_w0(t, s):
            c = pl.ds(t * 128, 128)
            return [pltpu.make_async_copy(wg_hbm.at[:, c], wg0.at[t], sems.at[s]),
                    pltpu.make_async_copy(wu_hbm.at[:, c], wu0.at[t], sems.at[s])]

        def cp_w(j):
            c = pl.ds(_al(j * FC, FC), FC)
            return [pltpu.make_async_copy(wg_hbm.at[:, c], wg_v.at[j - 1], sems.at[SM + j - 1]),
                    pltpu.make_async_copy(wu_hbm.at[:, c], wu_v.at[j - 1], sems.at[SM + j - 1])]

        cp_qo = [pltpu.make_async_copy(wqkv_hbm, wqkv_v, sems.at[SM]),
                 pltpu.make_async_copy(wo_hbm, wo_v, sems.at[SM])]
        cp_d = [pltpu.make_async_copy(wd_hbm, wd_v, sems.at[SD]),
                pltpu.make_async_copy(gw_hbm, gw_ref, sems.at[SD])]

        first = [[cp_x(0, 256, 0)] + cp_w0(0, 0), [cp_x(256, 256, 1)], cp_w0(1, 2)]
        second = cp_w0(2, SW1) + cp_w0(3, SW1)
        starts = sum(first, []) + second
        starts += [cp_x(b * XB, XB, SX + b - 1) for b in range(1, 4)]
        starts += cp_w(1) + cp_qo
        for j in range(2, NFC):
            starts += cp_w(j)
        starts += cp_d

        def ffn_up(r0, nr, wg, wu, t0):
            xx = x_v[pl.ds(r0, nr), :]
            gt = _dot(xx, wg)
            up = _dot(xx, wu)
            hh = (jnp.maximum(gt, 0.0) * up).astype(BF)
            for t in range(hh.shape[1] // 128):
                st_pk(h_v, t0 + t, r0, nr, hh[:, t * 128:(t + 1) * 128])

        def phase1():
            for c in starts:
                c.start()

            k_s[:, 0:HALO, :] = jnp.zeros((8, HALO, 128), F32)
            v_s[:, 0:HALO, :] = jnp.zeros((8, HALO, 128), F32)

            def warm0(u, carry):
                for k in range(3):
                    @pl.when(u == k)
                    def _():
                        for c in first[k]:
                            c.wait()
                t = _shr(u, 1)
                ffn_up(_al((u & 1) * 256, 256), 256, wg0[t], wu0[t], t)
                return carry
            lax.fori_loop(0, 4, scoped(warm0, 'warm0', prof), 0)

            def warm(u, carry):
                b = _shr(u, 1)
                half = u & 1

                @pl.when(u == 1)
                def _():
                    for c in second:
                        c.wait()

                @pl.when(half == 0)
                def _():
                    cp_x(_al(b * XB, XB), XB, SX + b - 1).wait()

                t = half * 2
                ffn_up(_al(b * XB, XB), XB, jnp.concatenate([wg0[t], wg0[t + 1]], axis=1),
                       jnp.concatenate([wu0[t], wu0[t + 1]], axis=1), t)
                return carry
            lax.fori_loop(1, 8, scoped(warm, 'warm', prof), 0)

            lane = lax.broadcasted_iota(I32, (8, 128), 1)

            def main1(j, carry):
                @pl.when(j == 1)
                def _():
                    for c in cp_qo:
                        c.wait()
                for c in cp_w(j):
                    c.wait()

                zv = jnp.full((8, 128), _shr(j, 20), I32).astype(U32)
                p = j - 1
                m = _shr(p, 1)
                hf = p & 1
                src = wqkv_v.at[pl.ds(_al(hf * 512, 512), 512), pl.ds(_al(m * D, D), D)]
                if 'q' in pks:
                    dst = wqkv_p.at[pl.ds(m * 8, 8), pl.ds(_al(hf * 256, 256), 256)]
                else:
                    dst = wqkv_p.at[pl.ds(m * 8, 8), pl.ds(_al(hf * 512, 512), 512)]
                deps = []
                for rr in range(0, 512, 16):
                    vs = [pltpu.bitcast(src[rr:rr + 16, cc * 128:(cc + 1) * 128], U32) for cc in range(8)]
                    vs = _permute_cols(vs, lane)
                    for cc in range(8):
                        st_pk(dst, cc, rr, 16, pltpu.bitcast(vs[cc], BF))
                    deps.append(vs[7] & zv)
                for r0 in range(0, S, rows1):
                    ffn_up(r0, rows1, wg_v[p], wu_v[p], j * 4)
                cbs = [jnp.minimum(2 * p + t, 7) for t in range(2)]
                wsrc = [wo_v.at[:, pl.ds(_al(cbs[t] * 128, 128), 128)] for t in range(2)]
                for hh in range(H):
                    if hh % 2 == 0 or not wser:
                        dep = deps[hh // 2]
                    for t in range(2):
                        for q in range(2):
                            val = pltpu.bitcast(wsrc[t][hh * 32 + q * 16:hh * 32 + (q + 1) * 16, :], U32) | dep
                            vf = pltpu.bitcast(val, BF).astype(F32)
                            wo_f32[t, hh * 33 + q * 16:hh * 33 + (q + 1) * 16, :] = vf
                            if wser:
                                dep = pltpu.bitcast(vf[8:16], U32) & zv
                for b in range(8):
                    for a in range(4):
                        if a % 2 == 0 or not wser:
                            dep = deps[16 + (b * 4 + a) // 2]
                        for t in range(2):
                            for q in range(2):
                                parts = [pltpu.bitcast(pltpu.bitcast(
                                    wo_f32[t, pl.ds(a * 8 + b + (q * 16 + e * 8) * 33, 8, stride=33), :], U32) | dep, F32)
                                    for e in range(2)]
                                pv = jnp.concatenate(parts, axis=0).astype(BF)
                                st_pk(wo_p, cbs[t], b * 128 + a * 32 + q * 16, 16, pv)
                                if wser:
                                    dep = pltpu.bitcast(pv, U32) & zv
                return carry
            lax.fori_loop(1, NFC, scoped(main1, 'main1', prof), 0)

        def phase2():
            for c in cp_d:
                c.wait()

            cexp = SCALE * LOG2E

            def main2(i, carry):
                r0 = _al(i * tm2, tm2)
                rows = pl.ds(r0, tm2)
                xb = x_v.at[rows]
                tl = [8 * 'qkv'.index(ch) + c for ch in order for c in range(8)]
                qkv = _dot(xb[...], jnp.concatenate([ld_pk(wqkv_p, t, 0, D) for t in tl], axis=1))
                kb = r0 if ring else 0
                for n, t in enumerate(tl):
                    val = qkv[:, n * 128:(n + 1) * 128]
                    if t < 8:
                        q_s[t] = val
                    elif t < 16:
                        k_s[t - 8, pl.ds(kb + HALO, tm2), :] = val
                    else:
                        v_s[t - 16, pl.ds(kb + HALO, tm2), :] = val
                zs = [_shr(i, 20), _shr(i, 21)]
                kzs = [kb + zz for zz in zs]
                zv = jnp.full((rb, 128), zs[0], I32)
                gw = gw_ref[...].astype(F32).reshape(1, D)

                def gate(t, dep):
                    return pltpu.bitcast(pltpu.bitcast(t, I32) | dep, F32)

                def after(t, dep):
                    return gate(t, pltpu.bitcast(dep, I32) & zv)
                den = None
                outs = []
                raws = []
                pend = [None] * 8
                for gi, r in enumerate(range(0, tm2, rb)):
                    z = zs[gi % 2]
                    kz = kzs[gi % 2]
                    q = [q_s[c, pl.ds(z + r, rb), :] for c in range(8)]
                    xf = xb[r:r + rb, :].astype(F32)
                    xf = [xf[:, c * 128:(c + 1) * 128] for c in range(8)]
                    if gi >= 1:
                        dep = pltpu.bitcast(den, I32)
                        if qlag and gi >= qlag:
                            dep = dep | pltpu.bitcast(outs[(gi - qlag) * 8 + 7], I32)
                        dep = dep & zv
                        q = [gate(t, dep) for t in q]
                    else:
                        dep = pltpu.bitcast(q[0], I32) & zv
                    if gdep:
                        xf = [gate(t, dep) for t in xf]
                    else:
                        gd = pltpu.bitcast(q[0] if gi == 0 else g, I32) & zv
                        xf = [gate(t, gd) for t in xf]
                    zg = xf[0] * gw[:, 0:128]
                    for c in range(1, 8):
                        zg = zg + xf[c] * gw[:, c * 128:(c + 1) * 128]
                    g = jax.nn.sigmoid(jnp.broadcast_to(jnp.sum(zg, axis=-1, keepdims=True), (rb, 128)))
                    omg_s[r:r + rb, :] = 1.0 - g
                    s = []
                    for w in range(W):
                        st = HALO + r - DIL * w
                        q0 = q[0] if w < qkw else after(q[0], raws[-qkw])
                        acc = q0 * k_s[0, pl.ds(kz + st, rb), :]
                        for c in range(1, 8):
                            acc = acc + q[c] * k_s[c, pl.ds(kz + st, rb), :]
                        raws.append(acc)
                        acc = acc + pltpu.roll(acc, 64, 1)
                        acc = acc + pltpu.roll(acc, 32, 1)
                        if r < HALO and w > 0:
                            pos = i * tm2 + r + lax.broadcasted_iota(I32, (rb, 128), 0)
                            acc = jnp.where(pos >= DIL * w, acc, -1e9 / SCALE)
                        s.append(acc)
                    m = s[0]
                    for w in range(1, W):
                        m = jnp.maximum(m, s[w])
                    e = [jnp.exp2((s[w] - m) * cexp) for w in range(W)]
                    den = e[0]
                    for w in range(1, W):
                        den = den + e[w]
                    inv = g / den
                    for c in range(8):
                        st = HALO + r
                        e0 = e[0] if len(outs) < pvw else after(e[0], outs[-pvw])
                        acc = e0 * v_s[c, pl.ds(kz + st, rb), :]
                        for w in range(1, W):
                            st = HALO + r - DIL * w
                            acc = acc + e[w] * v_s[c, pl.ds(kz + st, rb), :]
                        outs.append(acc)
                        acc = acc * inv
                        if gi % 2 == 0:
                            pend[c] = acc
                        else:
                            st_pk(oa_v, c, r - rb, 2 * rb, jnp.concatenate([pend[c], acc], axis=0).astype(BF))
                for c in range(0 if ring else 8):
                    for r in range(0, HALO, rb):
                        k_s[c, r:r + rb, :] = after(k_s[c, tm2 + r:tm2 + r + rb, :], outs[-1])
                        v_s[c, r:r + rb, :] = after(v_s[c, tm2 + r:tm2 + r + rb, :], outs[-1])
                b = _dot(jnp.concatenate([ld_pk(h_v, t, r0, tm2) for t in range(F // 128)], axis=1), wd_v[...])
                oa = jnp.concatenate([ld_pk(oa_v, c, 0, tm2) for c in range(8)], axis=1)
                omg = omg_s[...]
                for pc in range(opieces):
                    cs = slice(pc * OC, (pc + 1) * OC)
                    nt = OC // 128
                    a = _dot(oa, jnp.concatenate([ld_pk(wo_p, t, 0, D) for t in range(pc * nt, (pc + 1) * nt)], axis=1))
                    out_v[rows, cs] = (a + jnp.concatenate([omg] * nt, axis=1) * b[:, cs]).astype(BF)
                    pltpu.make_async_copy(out_v.at[rows, cs], o_hbm.at[rows, cs], sems.at[SOUT]).start()
                return carry
            lax.fori_loop(0, n2, scoped(main2, 'main2', prof), 0)
            pltpu.make_async_copy(out_v, o_hbm, sems.at[SOUT]).wait()

        pl.when(pl.program_id(0) == 0)(phase1)
        pl.when(pl.program_id(0) == 1)(phase2)

    @jax.jit
    def f(A_x, A_wqkv, A_wo, B_x, B_W_gate, B_W_up, B_W_down, gate_w):
        x = A_x.reshape(S, D)
        anyspec = pl.BlockSpec(memory_space=pl.ANY)
        out = pl.pallas_call(
            kernel,
            grid=(2,),
            in_specs=[anyspec] * 7,
            out_specs=anyspec,
            out_shape=jax.ShapeDtypeStruct((S, D), BF),
            scratch_shapes=[
                pltpu.VMEM((S, D), BF),
                pltpu.VMEM((D, 3 * D), BF),
                pk_shape(24, D, 'q'),
                pltpu.VMEM((D, D), BF),
                pk_shape(8, D, 'o'),
                pltpu.VMEM((2, 1088, 128), F32),
                pltpu.VMEM((4, D, 128), BF),
                pltpu.VMEM((4, D, 128), BF),
                pltpu.VMEM((NFC - 1, D, FC), BF),
                pltpu.VMEM((NFC - 1, D, FC), BF),
                pltpu.VMEM((F, D), BF),
                pk_shape(F // 128, S, 'h'),
                pltpu.VMEM((8, tm2, 128), F32),
                pltpu.VMEM((8, (S if ring else tm2) + HALO, 128), F32),
                pltpu.VMEM((8, (S if ring else tm2) + HALO, 128), F32),
                pk_shape(8, tm2, 'a'),
                pltpu.VMEM((tm2, 128), F32),
                pltpu.VMEM((S, D), BF),
                pltpu.VMEM((D,), BF),
                pltpu.SemaphoreType.DMA((NSEM,)),
            ],
            compiler_params=pltpu.CompilerParams(
                vmem_limit_bytes=110 * 1024 * 1024, disable_bounds_checks=True,
                dimension_semantics=('arbitrary',)),
        )(x, gate_w, A_wqkv, A_wo, B_W_gate, B_W_up, B_W_down)
        return out.reshape(1, S, D)
    return f


_impl = build()


@jax.jit
def pallas_gated_mix__sliding_local_dilated__glu_gated_reglu__prompt_kernel(
    A_x: jax.Array,
    A_wqkv: jax.Array,
    A_wo: jax.Array,
    B_x: jax.Array,
    B_W_gate: jax.Array,
    B_W_up: jax.Array,
    B_W_down: jax.Array,
    gate_w: jax.Array,
):
    return _impl(A_x, A_wqkv, A_wo, B_x, B_W_gate, B_W_up, B_W_down, gate_w)
```

```python
import jax
import jax.numpy as jnp
from jax import lax
import jax.experimental.pallas as pl
import jax.experimental.pallas.tpu as pltpu

S, D, F = 2048, 1024, 3584
H, DH, W, DIL = 32, 32, 8, 2
HALO = 16
LOG2E = 1.4426950408889634
SCALE = DH ** -0.5
BF = jnp.bfloat16
F32 = jnp.float32
U32 = jnp.uint32
I32 = jnp.int32


def scoped(fn, name, on):
    if not on:
        return fn

    def g(i, c):
        with jax.named_scope(name):
            return fn(i, c)
    return g


def _swap(vs, vbit, lbit, lane):
    out = list(vs)
    sh = 1 << lbit
    hi = (lane & sh) != 0
    for i in range(8):
        if i & (1 << vbit):
            continue
        a, b = vs[i], vs[i | (1 << vbit)]
        out[i] = jnp.where(hi, pltpu.roll(b, sh, 1), a)
        out[i | (1 << vbit)] = jnp.where(hi, b, pltpu.roll(a, 128 - sh, 1))
    return out


def _permute_cols(vs, lane):
    for vb, lb in ((2, 4), (1, 3), (0, 2), (2, 6), (2, 1), (1, 5), (1, 0)):
        vs = _swap(vs, vb, lb, lane)
    out = [None] * 8
    for i in range(8):
        v2, v1, v0 = (i >> 2) & 1, (i >> 1) & 1, i & 1
        out[(v0 << 2) | (v2 << 1) | v1] = vs[i]
    return out


def _dot(a, b):
    return jnp.dot(a, b, preferred_element_type=F32)


def _shr(x, n):
    return x >> n if isinstance(x, int) else lax.shift_right_logical(x, n)


def _al(x, n):
    return x if isinstance(x, int) else pl.multiple_of(x, n)


def build(prof=False, opieces=4, rows1=2048, pks='qoha', ring=True, wser=True, pvw=1, qkw=1, qlag=0, order='qkv', gdep=False):
    tm2 = 256
    rb = 8
    FC = 512
    NFC = F // FC
    XB = 512
    WC = 256
    n2 = S // tm2
    OC = D // opieces
    SX = 5
    SM = SX + 3
    SD = SM + NFC - 1
    SOUT = SD + 1
    NSEM = SOUT + 1

    def st_pk(ref, t, r0, n, val):
        if ref.dtype == U32:
            ref[t, pl.ds(_al(_shr(r0, 1), 8), n // 2), :] = pltpu.bitcast(val, U32)
        else:
            ref[t, pl.ds(r0, n), :] = val

    def ld_pk(ref, t, r0, n):
        if ref.dtype == U32:
            return pltpu.bitcast(ref[t, pl.ds(_al(_shr(r0, 1), 8), n // 2), :], BF)
        return ref[t, pl.ds(r0, n), :]

    def pk_shape(nt, rows, key):
        return pltpu.VMEM((nt, rows // 2, 128), U32) if key in pks else pltpu.VMEM((nt, rows, 128), BF)

    def kernel(x_hbm, gw_hbm, wqkv_hbm, wo_hbm, wg_hbm, wu_hbm, wd_hbm, o_hbm,
               x_v, wqkv_v, wqkv_p, wo_v, wo_p, wo_f32, wg0, wu0, wg_v, wu_v, wd_v, h_v, q_s, k_s, v_s, oa_v, omg_s,
               out_v, gw_ref, sems):
        def cp_x(r0, n, s):
            return pltpu.make_async_copy(x_hbm.at[pl.ds(r0, n)], x_v.at[pl.ds(r0, n)], sems.at[s])

        def cp_w0(t, s):
            c = pl.ds(_al(t * 128, 128), 128)
            return [pltpu.make_async_copy(wg_hbm.at[:, c], wg0.at[t], sems.at[s]),
                    pltpu.make_async_copy(wu_hbm.at[:, c], wu0.at[t], sems.at[s])]

        def cp_w(j):
            c = pl.ds(_al(j * FC, FC), FC)
            return [pltpu.make_async_copy(wg_hbm.at[:, c], wg_v.at[j - 1], sems.at[SM + j - 1]),
                    pltpu.make_async_copy(wu_hbm.at[:, c], wu_v.at[j - 1], sems.at[SM + j - 1])]

        cp_qo = [pltpu.make_async_copy(wqkv_hbm, wqkv_v, sems.at[SM]),
                 pltpu.make_async_copy(wo_hbm, wo_v, sems.at[SM])]
        cp_d = [pltpu.make_async_copy(wd_hbm, wd_v, sems.at[SD]),
                pltpu.make_async_copy(gw_hbm, gw_ref, sems.at[SD])]

        first = [cp_w0(0, 0) + [cp_x(0, 256, 0)], [cp_x(256, 256, 1)]]
        starts = sum(first, [])
        for t in range(1, 4):
            starts += cp_w0(t, 1 + t)
        starts += [cp_x(b * XB, XB, SX + b - 1) for b in range(1, 4)]
        starts += cp_w(1) + cp_qo
        for j in range(2, NFC):
            starts += cp_w(j)
        starts += cp_d

        def ffn_up(r0, nr, wg, wu, t0):
            xx = x_v[pl.ds(r0, nr), :]
            gt = _dot(xx, wg)
            up = _dot(xx, wu)
            hh = (jnp.maximum(gt, 0.0) * up).astype(BF)
            for t in range(hh.shape[1] // 128):
                st_pk(h_v, t0 + t, r0, nr, hh[:, t * 128:(t + 1) * 128])

        def phase1():
            for c in starts:
                c.start()

            k_s[:, 0:HALO, :] = jnp.zeros((8, HALO, 128), F32)
            v_s[:, 0:HALO, :] = jnp.zeros((8, HALO, 128), F32)

            def warm0(u, carry):
                for k in range(2):
                    @pl.when(u == k)
                    def _():
                        for c in first[k]:
                            c.wait()
                ffn_up(_al(u * 256, 256), 256, wg0[0], wu0[0], 0)
                return carry
            lax.fori_loop(0, 2, scoped(warm0, 'warm0', prof), 0)

            def warm1(t, carry):
                for c in cp_w0(t, 1 + t):
                    c.wait()
                ffn_up(0, XB, wg0[t], wu0[t], t)
                return carry
            lax.fori_loop(1, 4, scoped(warm1, 'warm1', prof), 0)

            def warm2(b, carry):
                cp_x(_al(b * XB, XB), XB, SX + b - 1).wait()
                ffn_up(_al(b * XB, XB), XB, jnp.concatenate([wg0[t] for t in range(4)], axis=1),
                       jnp.concatenate([wu0[t] for t in range(4)], axis=1), 0)
                return carry
            lax.fori_loop(1, 4, scoped(warm2, 'warm2', prof), 0)

            lane = lax.broadcasted_iota(I32, (8, 128), 1)

            for c in cp_qo:
                c.wait()

            def main1(j, carry):
                for c in cp_w(j):
                    c.wait()

                zv = jnp.full((8, 128), _shr(j, 20), I32).astype(U32)
                p = j - 1
                m = _shr(p, 1)
                hf = p & 1
                src = wqkv_v.at[pl.ds(_al(hf * 512, 512), 512), pl.ds(_al(m * D, D), D)]
                if 'q' in pks:
                    dst = wqkv_p.at[pl.ds(m * 8, 8), pl.ds(_al(hf * 256, 256), 256)]
                else:
                    dst = wqkv_p.at[pl.ds(m * 8, 8), pl.ds(_al(hf * 512, 512), 512)]
                deps = []
                for rr in range(0, 512, 16):
                    vs = [pltpu.bitcast(src[rr:rr + 16, cc * 128:(cc + 1) * 128], U32) for cc in range(8)]
                    vs = _permute_cols(vs, lane)
                    for cc in range(8):
                        st_pk(dst, cc, rr, 16, pltpu.bitcast(vs[cc], BF))
                    deps.append(vs[7] & zv)
                for r0 in range(0, S, rows1):
                    ffn_up(r0, rows1, wg_v[p], wu_v[p], j * 4)
                cbs = [jnp.minimum(2 * p + t, 7) for t in range(2)]
                wsrc = [wo_v.at[:, pl.ds(_al(cbs[t] * 128, 128), 128)] for t in range(2)]
                for hh in range(H):
                    if hh % 2 == 0 or not wser:
                        dep = deps[hh // 2]
                    for t in range(2):
                        for q in range(2):
                            val = pltpu.bitcast(wsrc[t][hh * 32 + q * 16:hh * 32 + (q + 1) * 16, :], U32) | dep
                            vf = pltpu.bitcast(val, BF).astype(F32)
                            wo_f32[t, hh * 33 + q * 16:hh * 33 + (q + 1) * 16, :] = vf
                            if wser:
                                dep = pltpu.bitcast(vf[8:16], U32) & zv
                for b in range(8):
                    for a in range(4):
                        if a % 2 == 0 or not wser:
                            dep = deps[16 + (b * 4 + a) // 2]
                        for t in range(2):
                            for q in range(2):
                                parts = [pltpu.bitcast(pltpu.bitcast(
                                    wo_f32[t, pl.ds(a * 8 + b + (q * 16 + e * 8) * 33, 8, stride=33), :], U32) | dep, F32)
                                    for e in range(2)]
                                pv = jnp.concatenate(parts, axis=0).astype(BF)
                                st_pk(wo_p, cbs[t], b * 128 + a * 32 + q * 16, 16, pv)
                                if wser:
                                    dep = pltpu.bitcast(pv, U32) & zv
                return carry
            lax.fori_loop(1, NFC, scoped(main1, 'main1', prof), 0)

        def phase2():
            for c in cp_d:
                c.wait()

            cexp = SCALE * LOG2E

            def main2(i, carry):
                r0 = _al(i * tm2, tm2)
                rows = pl.ds(r0, tm2)
                xb = x_v.at[rows]
                tl = [8 * 'qkv'.index(ch) + c for ch in order for c in range(8)]
                qkv = _dot(xb[...], jnp.concatenate([ld_pk(wqkv_p, t, 0, D) for t in tl], axis=1))
                kb = r0 if ring else 0
                for n, t in enumerate(tl):
                    val = qkv[:, n * 128:(n + 1) * 128]
                    if t < 8:
                        q_s[t] = val
                    elif t < 16:
                        k_s[t - 8, pl.ds(kb + HALO, tm2), :] = val
                    else:
                        v_s[t - 16, pl.ds(kb + HALO, tm2), :] = val
                zs = [_shr(i, 20), _shr(i, 21)]
                kzs = [kb + zz for zz in zs]
                zv = jnp.full((rb, 128), zs[0], I32)
                gw = gw_ref[...].astype(F32).reshape(1, D)

                def gate(t, dep):
                    return pltpu.bitcast(pltpu.bitcast(t, I32) | dep, F32)

                def after(t, dep):
                    return gate(t, pltpu.bitcast(dep, I32) & zv)
                den = None
                outs = []
                raws = []
                pend = [None] * 8
                for gi, r in enumerate(range(0, tm2, rb)):
                    z = zs[gi % 2]
                    kz = kzs[gi % 2]
                    q = [q_s[c, pl.ds(z + r, rb), :] for c in range(8)]
                    xf = xb[r:r + rb, :].astype(F32)
                    xf = [xf[:, c * 128:(c + 1) * 128] for c in range(8)]
                    if gi >= 1:
                        dep = pltpu.bitcast(den, I32)
                        if qlag and gi >= qlag:
                            dep = dep | pltpu.bitcast(outs[(gi - qlag) * 8 + 7], I32)
                        dep = dep & zv
                        q = [gate(t, dep) for t in q]
                    else:
                        dep = pltpu.bitcast(q[0], I32) & zv
                    if gdep:
                        xf = [gate(t, dep) for t in xf]
                    else:
                        gd = pltpu.bitcast(q[0] if gi == 0 else g, I32) & zv
                        xf = [gate(t, gd) for t in xf]
                    zg = xf[0] * gw[:, 0:128]
                    for c in range(1, 8):
                        zg = zg + xf[c] * gw[:, c * 128:(c + 1) * 128]
                    g = jax.nn.sigmoid(jnp.broadcast_to(jnp.sum(zg, axis=-1, keepdims=True), (rb, 128)))
                    omg_s[r:r + rb, :] = 1.0 - g
                    s = []
                    for w in range(W):
                        st = HALO + r - DIL * w
                        q0 = q[0] if w < qkw else after(q[0], raws[-qkw])
                        acc = q0 * k_s[0, pl.ds(kz + st, rb), :]
                        for c in range(1, 8):
                            acc = acc + q[c] * k_s[c, pl.ds(kz + st, rb), :]
                        raws.append(acc)
                        acc = acc + pltpu.roll(acc, 64, 1)
                        acc = acc + pltpu.roll(acc, 32, 1)
                        if r < HALO and w > 0:
                            pos = i * tm2 + r + lax.broadcasted_iota(I32, (rb, 128), 0)
                            acc = jnp.where(pos >= DIL * w, acc, -1e9 / SCALE)
                        s.append(acc)
                    m = s[0]
                    for w in range(1, W):
                        m = jnp.maximum(m, s[w])
                    e = [jnp.exp2((s[w] - m) * cexp) for w in range(W)]
                    den = e[0]
                    for w in range(1, W):
                        den = den + e[w]
                    inv = g / den
                    for c in range(8):
                        st = HALO + r
                        e0 = e[0] if len(outs) < pvw else after(e[0], outs[-pvw])
                        acc = e0 * v_s[c, pl.ds(kz + st, rb), :]
                        for w in range(1, W):
                            st = HALO + r - DIL * w
                            acc = acc + e[w] * v_s[c, pl.ds(kz + st, rb), :]
                        outs.append(acc)
                        acc = acc * inv
                        if gi % 2 == 0:
                            pend[c] = acc
                        else:
                            st_pk(oa_v, c, r - rb, 2 * rb, jnp.concatenate([pend[c], acc], axis=0).astype(BF))
                for c in range(0 if ring else 8):
                    for r in range(0, HALO, rb):
                        k_s[c, r:r + rb, :] = after(k_s[c, tm2 + r:tm2 + r + rb, :], outs[-1])
                        v_s[c, r:r + rb, :] = after(v_s[c, tm2 + r:tm2 + r + rb, :], outs[-1])
                b = _dot(jnp.concatenate([ld_pk(h_v, t, r0, tm2) for t in range(F // 128)], axis=1), wd_v[...])
                oa = jnp.concatenate([ld_pk(oa_v, c, 0, tm2) for c in range(8)], axis=1)
                omg = omg_s[...]
                for pc in range(opieces):
                    cs = slice(pc * OC, (pc + 1) * OC)
                    nt = OC // 128
                    a = _dot(oa, jnp.concatenate([ld_pk(wo_p, t, 0, D) for t in range(pc * nt, (pc + 1) * nt)], axis=1))
                    out_v[rows, cs] = (a + jnp.concatenate([omg] * nt, axis=1) * b[:, cs]).astype(BF)
                    pltpu.make_async_copy(out_v.at[rows, cs], o_hbm.at[rows, cs], sems.at[SOUT]).start()
                return carry
            lax.fori_loop(0, n2, scoped(main2, 'main2', prof), 0)
            pltpu.make_async_copy(out_v, o_hbm, sems.at[SOUT]).wait()

        pl.when(pl.program_id(0) == 0)(phase1)
        pl.when(pl.program_id(0) == 1)(phase2)

    @jax.jit
    def f(A_x, A_wqkv, A_wo, B_x, B_W_gate, B_W_up, B_W_down, gate_w):
        x = A_x.reshape(S, D)
        anyspec = pl.BlockSpec(memory_space=pl.ANY)
        out = pl.pallas_call(
            kernel,
            grid=(2,),
            in_specs=[anyspec] * 7,
            out_specs=anyspec,
            out_shape=jax.ShapeDtypeStruct((S, D), BF),
            scratch_shapes=[
                pltpu.VMEM((S, D), BF),
                pltpu.VMEM((D, 3 * D), BF),
                pk_shape(24, D, 'q'),
                pltpu.VMEM((D, D), BF),
                pk_shape(8, D, 'o'),
                pltpu.VMEM((2, 1088, 128), F32),
                pltpu.VMEM((4, D, 128), BF),
                pltpu.VMEM((4, D, 128), BF),
                pltpu.VMEM((NFC - 1, D, FC), BF),
                pltpu.VMEM((NFC - 1, D, FC), BF),
                pltpu.VMEM((F, D), BF),
                pk_shape(F // 128, S, 'h'),
                pltpu.VMEM((8, tm2, 128), F32),
                pltpu.VMEM((8, (S if ring else tm2) + HALO, 128), F32),
                pltpu.VMEM((8, (S if ring else tm2) + HALO, 128), F32),
                pk_shape(8, tm2, 'a'),
                pltpu.VMEM((tm2, 128), F32),
                pltpu.VMEM((S, D), BF),
                pltpu.VMEM((D,), BF),
                pltpu.SemaphoreType.DMA((NSEM,)),
            ],
            compiler_params=pltpu.CompilerParams(
                vmem_limit_bytes=110 * 1024 * 1024, disable_bounds_checks=True,
                dimension_semantics=('arbitrary',)),
        )(x, gate_w, A_wqkv, A_wo, B_W_gate, B_W_up, B_W_down)
        return out.reshape(1, S, D)
    return f


_impl = build()


@jax.jit
def pallas_gated_mix__sliding_local_dilated__glu_gated_reglu__prompt_kernel(
    A_x: jax.Array,
    A_wqkv: jax.Array,
    A_wo: jax.Array,
    B_x: jax.Array,
    B_W_gate: jax.Array,
    B_W_up: jax.Array,
    B_W_down: jax.Array,
    gate_w: jax.Array,
):
    return _impl(A_x, A_wqkv, A_wo, B_x, B_W_gate, B_W_up, B_W_down, gate_w)
```

```python
import jax
import jax.numpy as jnp
from jax import lax
import jax.experimental.pallas as pl
import jax.experimental.pallas.tpu as pltpu

S, D, F = 2048, 1024, 3584
H, DH, W, DIL = 32, 32, 8, 2
HALO = 16
LOG2E = 1.4426950408889634
SCALE = DH ** -0.5
BF = jnp.bfloat16
F32 = jnp.float32
U32 = jnp.uint32
I32 = jnp.int32


def scoped(fn, name, on):
    if not on:
        return fn

    def g(i, c):
        with jax.named_scope(name):
            return fn(i, c)
    return g


def _swap(vs, vbit, lbit, lane):
    out = list(vs)
    sh = 1 << lbit
    hi = (lane & sh) != 0
    for i in range(8):
        if i & (1 << vbit):
            continue
        a, b = vs[i], vs[i | (1 << vbit)]
        out[i] = jnp.where(hi, pltpu.roll(b, sh, 1), a)
        out[i | (1 << vbit)] = jnp.where(hi, b, pltpu.roll(a, 128 - sh, 1))
    return out


def _permute_cols(vs, lane):
    for vb, lb in ((2, 4), (1, 3), (0, 2), (2, 6), (2, 1), (1, 5), (1, 0)):
        vs = _swap(vs, vb, lb, lane)
    out = [None] * 8
    for i in range(8):
        v2, v1, v0 = (i >> 2) & 1, (i >> 1) & 1, i & 1
        out[(v0 << 2) | (v2 << 1) | v1] = vs[i]
    return out


def _dot(a, b):
    return jnp.dot(a, b, preferred_element_type=F32)


def _shr(x, n):
    return x >> n if isinstance(x, int) else lax.shift_right_logical(x, n)


def _al(x, n):
    return x if isinstance(x, int) else pl.multiple_of(x, n)


def build(prof=False, opieces=4, rows1=2048, pks='qoa', ring=True, wser=True, pvw=1, qkw=1, qlag=0, order='qkv', qgate=8, xgate=8, pgate=False):
    tm2 = 256
    rb = 8
    FC = 512
    NFC = F // FC
    XB = 512
    WC = 256
    n2 = S // tm2
    OC = D // opieces
    SX = 5
    SM = SX + 3
    SD = SM + NFC - 1
    SOUT = SD + 1
    NSEM = SOUT + 1

    def st_pk(ref, t, r0, n, val):
        if ref.dtype == U32:
            ref[t, pl.ds(_al(_shr(r0, 1), 8), n // 2), :] = pltpu.bitcast(val, U32)
        else:
            ref[t, pl.ds(r0, n), :] = val

    def ld_pk(ref, t, r0, n):
        if ref.dtype == U32:
            return pltpu.bitcast(ref[t, pl.ds(_al(_shr(r0, 1), 8), n // 2), :], BF)
        return ref[t, pl.ds(r0, n), :]

    def pk_shape(nt, rows, key):
        return pltpu.VMEM((nt, rows // 2, 128), U32) if key in pks else pltpu.VMEM((nt, rows, 128), BF)

    def kernel(x_hbm, gw_hbm, wqkv_hbm, wo_hbm, wg_hbm, wu_hbm, wd_hbm, o_hbm,
               x_v, wqkv_v, wqkv_p, wo_v, wo_p, wo_f32, wg0, wu0, wg_v, wu_v, wd_v, h_v, q_s, k_s, v_s, oa_v, g_s,
               out_v, gw_ref, sems):
        def cp_x(r0, n, s):
            return pltpu.make_async_copy(x_hbm.at[pl.ds(r0, n)], x_v.at[pl.ds(r0, n)], sems.at[s])

        def cp_w0(t, s):
            c = pl.ds(_al(t * 128, 128), 128)
            return [pltpu.make_async_copy(wg_hbm.at[:, c], wg0.at[t], sems.at[s]),
                    pltpu.make_async_copy(wu_hbm.at[:, c], wu0.at[t], sems.at[s])]

        def cp_w(j):
            c = pl.ds(_al(j * FC, FC), FC)
            return [pltpu.make_async_copy(wg_hbm.at[:, c], wg_v.at[j - 1], sems.at[SM + j - 1]),
                    pltpu.make_async_copy(wu_hbm.at[:, c], wu_v.at[j - 1], sems.at[SM + j - 1])]

        cp_qo = [pltpu.make_async_copy(wqkv_hbm, wqkv_v, sems.at[SM]),
                 pltpu.make_async_copy(wo_hbm, wo_v, sems.at[SM]),
                 pltpu.make_async_copy(gw_hbm, gw_ref, sems.at[SM])]
        cp_d = [pltpu.make_async_copy(wd_hbm, wd_v, sems.at[SD])]

        first = [cp_w0(0, 0) + [cp_x(0, 256, 0)], [cp_x(256, 256, 1)]]
        starts = sum(first, [])
        for t in range(1, 4):
            starts += cp_w0(t, 1 + t)
        starts += [cp_x(b * XB, XB, SX + b - 1) for b in range(1, 4)]
        starts += cp_w(1) + cp_qo
        for j in range(2, NFC):
            starts += cp_w(j)
        starts += cp_d

        def ffn_up(r0, nr, wg, wu, t0):
            xx = x_v[pl.ds(r0, nr), :]
            gt = _dot(xx, wg)
            up = _dot(xx, wu)
            hh = (jnp.maximum(gt, 0.0) * up).astype(BF)
            for t in range(hh.shape[1] // 128):
                st_pk(h_v, t0 + t, r0, nr, hh[:, t * 128:(t + 1) * 128])

        def phase1():
            for c in starts:
                c.start()

            k_s[:, 0:HALO, :] = jnp.zeros((8, HALO, 128), F32)
            v_s[:, 0:HALO, :] = jnp.zeros((8, HALO, 128), F32)

            def warm0(u, carry):
                for k in range(2):
                    @pl.when(u == k)
                    def _():
                        for c in first[k]:
                            c.wait()
                ffn_up(_al(u * 256, 256), 256, wg0[0], wu0[0], 0)
                return carry
            lax.fori_loop(0, 2, scoped(warm0, 'warm0', prof), 0)

            def warm1(t, carry):
                for c in cp_w0(t, 1 + t):
                    c.wait()
                ffn_up(0, XB, wg0[t], wu0[t], t)
                return carry
            lax.fori_loop(1, 4, scoped(warm1, 'warm1', prof), 0)

            def warm2(b, carry):
                cp_x(_al(b * XB, XB), XB, SX + b - 1).wait()
                ffn_up(_al(b * XB, XB), XB, jnp.concatenate([wg0[t] for t in range(4)], axis=1),
                       jnp.concatenate([wu0[t] for t in range(4)], axis=1), 0)
                return carry
            lax.fori_loop(1, 4, scoped(warm2, 'warm2', prof), 0)

            lane = lax.broadcasted_iota(I32, (8, 128), 1)

            for c in cp_qo:
                c.wait()

            def main1(j, carry):
                for c in cp_w(j):
                    c.wait()

                zv = jnp.full((8, 128), _shr(j, 20), I32).astype(U32)
                p = j - 1
                m = _shr(p, 1)
                hf = p & 1
                src = wqkv_v.at[pl.ds(_al(hf * 512, 512), 512), pl.ds(_al(m * D, D), D)]
                if 'q' in pks:
                    dst = wqkv_p.at[pl.ds(m * 8, 8), pl.ds(_al(hf * 256, 256), 256)]
                else:
                    dst = wqkv_p.at[pl.ds(m * 8, 8), pl.ds(_al(hf * 512, 512), 512)]
                deps = []
                for rr in range(0, 512, 16):
                    vs = [pltpu.bitcast(src[rr:rr + 16, cc * 128:(cc + 1) * 128], U32) for cc in range(8)]
                    vs = _permute_cols(vs, lane)
                    for cc in range(8):
                        st_pk(dst, cc, rr, 16, pltpu.bitcast(vs[cc], BF))
                    deps.append(vs[7] & zv)
                for r0 in range(0, S, rows1):
                    ffn_up(r0, rows1, wg_v[p], wu_v[p], j * 4)
                gr = _al(jnp.minimum(p, 3) * XB, XB)
                xg = x_v.at[pl.ds(gr, XB)]
                gdst = g_s.at[pl.ds(gr, XB)]
                gw = gw_ref[...].astype(F32).reshape(1, D)
                gd = deps[0]
                for r in range(0, XB, 8):
                    xf = xg[r:r + 8, :].astype(F32)
                    xf = [xf[:, c * 128:(c + 1) * 128] for c in range(8)]
                    xf = [pltpu.bitcast(pltpu.bitcast(t, U32) | gd, F32) if c < xgate else t for c, t in enumerate(xf)]
                    zg = xf[0] * gw[:, 0:128]
                    for c in range(1, 8):
                        zg = zg + xf[c] * gw[:, c * 128:(c + 1) * 128]
                    g = jax.nn.sigmoid(jnp.broadcast_to(jnp.sum(zg, axis=-1, keepdims=True), (8, 128)))
                    gdst[r:r + 8, :] = g
                    gd = pltpu.bitcast(g, U32) & zv
                cbs = [jnp.minimum(2 * p + t, 7) for t in range(2)]
                wsrc = [wo_v.at[:, pl.ds(_al(cbs[t] * 128, 128), 128)] for t in range(2)]
                for hh in range(H):
                    if hh % 2 == 0 or not wser:
                        dep = deps[hh // 2]
                    for t in range(2):
                        for q in range(2):
                            val = pltpu.bitcast(wsrc[t][hh * 32 + q * 16:hh * 32 + (q + 1) * 16, :], U32) | dep
                            vf = pltpu.bitcast(val, BF).astype(F32)
                            wo_f32[t, hh * 33 + q * 16:hh * 33 + (q + 1) * 16, :] = vf
                            if wser:
                                dep = pltpu.bitcast(vf[8:16], U32) & zv
                for b in range(8):
                    for a in range(4):
                        if a % 2 == 0 or not wser:
                            dep = deps[16 + (b * 4 + a) // 2]
                        for t in range(2):
                            for q in range(2):
                                parts = [pltpu.bitcast(pltpu.bitcast(
                                    wo_f32[t, pl.ds(a * 8 + b + (q * 16 + e * 8) * 33, 8, stride=33), :], U32) | dep, F32)
                                    for e in range(2)]
                                pv = jnp.concatenate(parts, axis=0).astype(BF)
                                st_pk(wo_p, cbs[t], b * 128 + a * 32 + q * 16, 16, pv)
                                if wser:
                                    dep = pltpu.bitcast(pv, U32) & zv
                return carry
            lax.fori_loop(1, NFC, scoped(main1, 'main1', prof), 0)

        def phase2():
            for c in cp_d:
                c.wait()

            cexp = SCALE * LOG2E

            def main2(i, carry):
                r0 = _al(i * tm2, tm2)
                rows = pl.ds(r0, tm2)
                xb = x_v.at[rows]
                tl = [8 * 'qkv'.index(ch) + c for ch in order for c in range(8)]
                qkv = _dot(xb[...], jnp.concatenate([ld_pk(wqkv_p, t, 0, D) for t in tl], axis=1))
                kb = r0 if ring else 0
                for n, t in enumerate(tl):
                    val = qkv[:, n * 128:(n + 1) * 128]
                    if t < 8:
                        q_s[t] = val
                    elif t < 16:
                        k_s[t - 8, pl.ds(kb + HALO, tm2), :] = val
                    else:
                        v_s[t - 16, pl.ds(kb + HALO, tm2), :] = val
                zs = [_shr(i, 20), _shr(i, 21)]
                kzs = [kb + zz for zz in zs]
                zv = jnp.full((rb, 128), zs[0], I32)
                gb = g_s.at[rows]

                def gate(t, dep):
                    return pltpu.bitcast(pltpu.bitcast(t, I32) | dep, F32)

                def after(t, dep):
                    return gate(t, pltpu.bitcast(dep, I32) & zv)
                den = None
                outs = []
                raws = []
                pend = [None] * 8
                for gi, r in enumerate(range(0, tm2, rb)):
                    z = zs[gi % 2]
                    kz = kzs[gi % 2]
                    q = [q_s[c, pl.ds(z + r, rb), :] for c in range(8)]
                    if gi >= 1:
                        dep = pltpu.bitcast(den, I32) & zv
                        q = [gate(t, dep) if c < qgate else t for c, t in enumerate(q)]
                    g = gb[r:r + rb, :]
                    s = []
                    for w in range(W):
                        st = HALO + r - DIL * w
                        q0 = q[0] if w < qkw else after(q[0], raws[-qkw])
                        acc = q0 * k_s[0, pl.ds(kz + st, rb), :]
                        for c in range(1, 8):
                            acc = acc + q[c] * k_s[c, pl.ds(kz + st, rb), :]
                        raws.append(acc)
                        acc = acc + pltpu.roll(acc, 64, 1)
                        acc = acc + pltpu.roll(acc, 32, 1)
                        if r < HALO and w > 0:
                            pos = i * tm2 + r + lax.broadcasted_iota(I32, (rb, 128), 0)
                            acc = jnp.where(pos >= DIL * w, acc, -1e9 / SCALE)
                        s.append(acc)
                    m = s[0]
                    for w in range(1, W):
                        m = jnp.maximum(m, s[w])
                    e = [jnp.exp2((s[w] - m) * cexp) for w in range(W)]
                    den = e[0]
                    for w in range(1, W):
                        den = den + e[w]
                    inv = g / den
                    for c in range(8):
                        st = HALO + r
                        e0 = e[0] if len(outs) < pvw else after(e[0], outs[-pvw])
                        acc = e0 * v_s[c, pl.ds(kz + st, rb), :]
                        for w in range(1, W):
                            st = HALO + r - DIL * w
                            acc = acc + e[w] * v_s[c, pl.ds(kz + st, rb), :]
                        outs.append(acc)
                        acc = acc * inv
                        if gi % 2 == 0:
                            pend[c] = acc
                        else:
                            st_pk(oa_v, c, r - rb, 2 * rb, jnp.concatenate([pend[c], acc], axis=0).astype(BF))
                for c in range(0 if ring else 8):
                    for r in range(0, HALO, rb):
                        k_s[c, r:r + rb, :] = after(k_s[c, tm2 + r:tm2 + r + rb, :], outs[-1])
                        v_s[c, r:r + rb, :] = after(v_s[c, tm2 + r:tm2 + r + rb, :], outs[-1])
                b = _dot(jnp.concatenate([ld_pk(h_v, t, r0, tm2) for t in range(F // 128)], axis=1), wd_v[...])
                oa = jnp.concatenate([ld_pk(oa_v, c, 0, tm2) for c in range(8)], axis=1)
                omg = 1.0 - gb[...]
                for pc in range(opieces):
                    cs = slice(pc * OC, (pc + 1) * OC)
                    nt = OC // 128
                    a = _dot(oa, jnp.concatenate([ld_pk(wo_p, t, 0, D) for t in range(pc * nt, (pc + 1) * nt)], axis=1))
                    out_v[rows, cs] = (a + jnp.concatenate([omg] * nt, axis=1) * b[:, cs]).astype(BF)
                    pltpu.make_async_copy(out_v.at[rows, cs], o_hbm.at[rows, cs], sems.at[SOUT]).start()
                return carry
            lax.fori_loop(0, n2, scoped(main2, 'main2', prof), 0)
            pltpu.make_async_copy(out_v, o_hbm, sems.at[SOUT]).wait()

        pl.when(pl.program_id(0) == 0)(phase1)
        pl.when(pl.program_id(0) == 1)(phase2)

    @jax.jit
    def f(A_x, A_wqkv, A_wo, B_x, B_W_gate, B_W_up, B_W_down, gate_w):
        x = A_x.reshape(S, D)
        anyspec = pl.BlockSpec(memory_space=pl.ANY)
        out = pl.pallas_call(
            kernel,
            grid=(2,),
            in_specs=[anyspec] * 7,
            out_specs=anyspec,
            out_shape=jax.ShapeDtypeStruct((S, D), BF),
            scratch_shapes=[
                pltpu.VMEM((S, D), BF),
                pltpu.VMEM((D, 3 * D), BF),
                pk_shape(24, D, 'q'),
                pltpu.VMEM((D, D), BF),
                pk_shape(8, D, 'o'),
                pltpu.VMEM((2, 1088, 128), F32),
                pltpu.VMEM((4, D, 128), BF),
                pltpu.VMEM((4, D, 128), BF),
                pltpu.VMEM((NFC - 1, D, FC), BF),
                pltpu.VMEM((NFC - 1, D, FC), BF),
                pltpu.VMEM((F, D), BF),
                pk_shape(F // 128, S, 'h'),
                pltpu.VMEM((8, tm2, 128), F32),
                pltpu.VMEM((8, (S if ring else tm2) + HALO, 128), F32),
                pltpu.VMEM((8, (S if ring else tm2) + HALO, 128), F32),
                pk_shape(8, tm2, 'a'),
                pltpu.VMEM((S, 128), F32),
                pltpu.VMEM((S, D), BF),
                pltpu.VMEM((D,), BF),
                pltpu.SemaphoreType.DMA((NSEM,)),
            ],
            compiler_params=pltpu.CompilerParams(
                vmem_limit_bytes=110 * 1024 * 1024, disable_bounds_checks=True,
                dimension_semantics=('arbitrary',)),
        )(x, gate_w, A_wqkv, A_wo, B_W_gate, B_W_up, B_W_down)
        return out.reshape(1, S, D)
    return f


_impl = build()


@jax.jit
def pallas_gated_mix__sliding_local_dilated__glu_gated_reglu__prompt_kernel(
    A_x: jax.Array,
    A_wqkv: jax.Array,
    A_wo: jax.Array,
    B_x: jax.Array,
    B_W_gate: jax.Array,
    B_W_up: jax.Array,
    B_W_down: jax.Array,
    gate_w: jax.Array,
):
    return _impl(A_x, A_wqkv, A_wo, B_x, B_W_gate, B_W_up, B_W_down, gate_w)
```

```python
import jax
import jax.numpy as jnp
from jax import lax
import jax.experimental.pallas as pl
import jax.experimental.pallas.tpu as pltpu

S, D, F = 2048, 1024, 3584
H, DH, W, DIL = 32, 32, 8, 2
HALO = 16
LOG2E = 1.4426950408889634
SCALE = DH ** -0.5
BF = jnp.bfloat16
F32 = jnp.float32
U32 = jnp.uint32
I32 = jnp.int32


def scoped(fn, name, on):
    if not on:
        return fn

    def g(i, c):
        with jax.named_scope(name):
            return fn(i, c)
    return g


def _swap(vs, vbit, lbit, lane):
    out = list(vs)
    sh = 1 << lbit
    hi = (lane & sh) != 0
    for i in range(8):
        if i & (1 << vbit):
            continue
        a, b = vs[i], vs[i | (1 << vbit)]
        out[i] = jnp.where(hi, pltpu.roll(b, sh, 1), a)
        out[i | (1 << vbit)] = jnp.where(hi, b, pltpu.roll(a, 128 - sh, 1))
    return out


def _permute_cols(vs, lane):
    for vb, lb in ((2, 4), (1, 3), (0, 2), (2, 6), (2, 1), (1, 5), (1, 0)):
        vs = _swap(vs, vb, lb, lane)
    out = [None] * 8
    for i in range(8):
        v2, v1, v0 = (i >> 2) & 1, (i >> 1) & 1, i & 1
        out[(v0 << 2) | (v2 << 1) | v1] = vs[i]
    return out


def _dot(a, b):
    return jnp.dot(a, b, preferred_element_type=F32)


def _shr(x, n):
    return x >> n if isinstance(x, int) else lax.shift_right_logical(x, n)


def _al(x, n):
    return x if isinstance(x, int) else pl.multiple_of(x, n)


def build(prof=False, opieces=8, rows1=2048, pks='qoa', ring=True, wser=True, pvw=1, qkw=1, qlag=0, order='qkv', qgate=8, xgate=8, lastsplit=4, pgate=0):
    tm2 = 256
    rb = 8
    FC = 512
    NFC = F // FC
    XB = 512
    WC = 256
    n2 = S // tm2
    OC = D // opieces
    SM = 0
    SX = 6
    SD = 6
    SOUT = 7
    NSEM = 9

    def st_pk(ref, t, r0, n, val):
        if ref.dtype == U32:
            ref[t, pl.ds(_al(_shr(r0, 1), 8), n // 2), :] = pltpu.bitcast(val, U32)
        else:
            ref[t, pl.ds(r0, n), :] = val

    def ld_pk(ref, t, r0, n):
        if ref.dtype == U32:
            return pltpu.bitcast(ref[t, pl.ds(_al(_shr(r0, 1), 8), n // 2), :], BF)
        return ref[t, pl.ds(r0, n), :]

    def pk_shape(nt, rows, key):
        return pltpu.VMEM((nt, rows // 2, 128), U32) if key in pks else pltpu.VMEM((nt, rows, 128), BF)

    def kernel(x_hbm, gw_hbm, wqkv_hbm, wo_hbm, wg_hbm, wu_hbm, wd_hbm, o_hbm,
               x_v, wqkv_v, wqkv_p, wo_v, wo_p, wo_f32, wg0, wu0, wg_v, wu_v, wd_v, h_v, q_s, k_s, v_s, oa_v, g_s,
               out_v, gw_ref, sems):
        def cp_x(r0, n, s):
            return pltpu.make_async_copy(x_hbm.at[pl.ds(r0, n)], x_v.at[pl.ds(r0, n)], sems.at[s])

        def cp_w0(t, s):
            c = pl.ds(_al(t * 128, 128), 128)
            return [pltpu.make_async_copy(wg_hbm.at[:, c], wg0.at[t], sems.at[s]),
                    pltpu.make_async_copy(wu_hbm.at[:, c], wu0.at[t], sems.at[s])]

        def cp_w(j):
            c = pl.ds(_al(j * FC, FC), FC)
            return [pltpu.make_async_copy(wg_hbm.at[:, c], wg_v.at[j - 1], sems.at[SM + j - 1]),
                    pltpu.make_async_copy(wu_hbm.at[:, c], wu_v.at[j - 1], sems.at[SM + j - 1])]

        cp_qo = [pltpu.make_async_copy(wqkv_hbm, wqkv_v, sems.at[SM]),
                 pltpu.make_async_copy(wo_hbm, wo_v, sems.at[SM]),
                 pltpu.make_async_copy(gw_hbm, gw_ref, sems.at[SM])]
        cp_d = [pltpu.make_async_copy(wd_hbm, wd_v, sems.at[SD])]

        first = [cp_w0(0, 1) + [cp_x(0, 256, 1)], [cp_x(256, 256, 2)]]
        starts = sum(first, [])
        for t in range(1, 4):
            starts += cp_w0(t, 2 + t)
        starts += [cp_x(b * XB, XB, SX + b - 1) for b in range(1, 4)]
        starts += cp_w(1) + cp_qo

        def ffn_up(r0, nr, wg, wu, t0):
            xx = x_v[pl.ds(r0, nr), :]
            gt = _dot(xx, wg)
            up = _dot(xx, wu)
            hh = (jnp.maximum(gt, 0.0) * up).astype(BF)
            for t in range(hh.shape[1] // 128):
                st_pk(h_v, t0 + t, r0, nr, hh[:, t * 128:(t + 1) * 128])

        def phase1():
            for c in starts:
                c.start()

            k_s[:, 0:HALO, :] = jnp.zeros((8, HALO, 128), F32)
            v_s[:, 0:HALO, :] = jnp.zeros((8, HALO, 128), F32)

            def warm0(u, carry):
                for k in range(2):
                    @pl.when(u == k)
                    def _():
                        for c in first[k]:
                            c.wait()
                ffn_up(_al(u * 256, 256), 256, wg0[0], wu0[0], 0)
                return carry
            lax.fori_loop(0, 2, scoped(warm0, 'warm0', prof), 0)

            def warm1(t, carry):
                for c in cp_w0(t, 2 + t):
                    c.wait()
                ffn_up(0, XB, wg0[t], wu0[t], t)
                return carry
            lax.fori_loop(1, 4, scoped(warm1, 'warm1', prof), 0)
            for j in range(2, NFC):
                for c in cp_w(j):
                    c.start()

            def warm2(b, carry):
                cp_x(_al(b * XB, XB), XB, SX + b - 1).wait()
                ffn_up(_al(b * XB, XB), XB, jnp.concatenate([wg0[t] for t in range(4)], axis=1),
                       jnp.concatenate([wu0[t] for t in range(4)], axis=1), 0)
                return carry
            lax.fori_loop(1, 4, scoped(warm2, 'warm2', prof), 0)

            lane = lax.broadcasted_iota(I32, (8, 128), 1)

            for c in cp_d:
                c.start()
            for c in cp_qo:
                c.wait()

            def main1(j, carry):
                for c in cp_w(j):
                    c.wait()

                zv = jnp.full((8, 128), _shr(j, 20), I32).astype(U32)
                p = j - 1
                m = _shr(p, 1)
                hf = p & 1
                src = wqkv_v.at[pl.ds(_al(hf * 512, 512), 512), pl.ds(_al(m * D, D), D)]
                if 'q' in pks:
                    dst = wqkv_p.at[pl.ds(m * 8, 8), pl.ds(_al(hf * 256, 256), 256)]
                else:
                    dst = wqkv_p.at[pl.ds(m * 8, 8), pl.ds(_al(hf * 512, 512), 512)]
                deps = []
                for rr in range(0, 512, 16):
                    vs = [pltpu.bitcast(src[rr:rr + 16, cc * 128:(cc + 1) * 128], U32) for cc in range(8)]
                    if pgate:
                        pd = deps[-pgate] if len(deps) >= pgate else pltpu.roll(zv, 1, 1) & zv
                        vs = [v | pd for v in vs]
                    vs = _permute_cols(vs, lane)
                    for cc in range(8):
                        st_pk(dst, cc, rr, 16, pltpu.bitcast(vs[cc], BF))
                    deps.append(vs[7] & zv)
                for r0 in range(0, S, rows1):
                    ffn_up(r0, rows1, wg_v[p], wu_v[p], j * 4)
                gr = _al(jnp.minimum(p, 3) * XB, XB)
                xg = x_v.at[pl.ds(gr, XB)]
                gdst = g_s.at[pl.ds(gr, XB)]
                gw = gw_ref[...].astype(F32).reshape(1, D)
                gd = deps[0]
                for r in range(0, XB, 8):
                    xf = xg[r:r + 8, :].astype(F32)
                    xf = [xf[:, c * 128:(c + 1) * 128] for c in range(8)]
                    xf = [pltpu.bitcast(pltpu.bitcast(t, U32) | gd, F32) if c < xgate else t for c, t in enumerate(xf)]
                    zg = xf[0] * gw[:, 0:128]
                    for c in range(1, 8):
                        zg = zg + xf[c] * gw[:, c * 128:(c + 1) * 128]
                    g = jax.nn.sigmoid(jnp.broadcast_to(jnp.sum(zg, axis=-1, keepdims=True), (8, 128)))
                    gdst[r:r + 8, :] = g
                    gd = pltpu.bitcast(g, U32) & zv
                cbs = [jnp.minimum(2 * p + t, 7) for t in range(2)]
                wsrc = [wo_v.at[:, pl.ds(_al(cbs[t] * 128, 128), 128)] for t in range(2)]
                for hh in range(H):
                    if hh % 2 == 0 or not wser:
                        dep = deps[hh // 2]
                    for t in range(2):
                        for q in range(2):
                            val = pltpu.bitcast(wsrc[t][hh * 32 + q * 16:hh * 32 + (q + 1) * 16, :], U32) | dep
                            vf = pltpu.bitcast(val, BF).astype(F32)
                            wo_f32[t, hh * 33 + q * 16:hh * 33 + (q + 1) * 16, :] = vf
                            if wser:
                                dep = pltpu.bitcast(vf[8:16], U32) & zv
                for b in range(8):
                    for a in range(4):
                        if a % 2 == 0 or not wser:
                            dep = deps[16 + (b * 4 + a) // 2]
                        for t in range(2):
                            for q in range(2):
                                parts = [pltpu.bitcast(pltpu.bitcast(
                                    wo_f32[t, pl.ds(a * 8 + b + (q * 16 + e * 8) * 33, 8, stride=33), :], U32) | dep, F32)
                                    for e in range(2)]
                                pv = jnp.concatenate(parts, axis=0).astype(BF)
                                st_pk(wo_p, cbs[t], b * 128 + a * 32 + q * 16, 16, pv)
                                if wser:
                                    dep = pltpu.bitcast(pv, U32) & zv
                return carry
            lax.fori_loop(1, NFC, scoped(main1, 'main1', prof), 0)

        def phase2():
            for c in cp_d:
                c.wait()

            cexp = SCALE * LOG2E

            def main2(i, carry):
                r0 = _al(i * tm2, tm2)
                rows = pl.ds(r0, tm2)
                xb = x_v.at[rows]
                tl = [8 * 'qkv'.index(ch) + c for ch in order for c in range(8)]
                qkv = _dot(xb[...], jnp.concatenate([ld_pk(wqkv_p, t, 0, D) for t in tl], axis=1))
                kb = r0 if ring else 0
                for n, t in enumerate(tl):
                    val = qkv[:, n * 128:(n + 1) * 128]
                    if t < 8:
                        q_s[t] = val
                    elif t < 16:
                        k_s[t - 8, pl.ds(kb + HALO, tm2), :] = val
                    else:
                        v_s[t - 16, pl.ds(kb + HALO, tm2), :] = val
                zs = [_shr(i, 20), _shr(i, 21)]
                kzs = [kb + zz for zz in zs]
                zv = jnp.full((rb, 128), zs[0], I32)
                gb = g_s.at[rows]

                def gate(t, dep):
                    return pltpu.bitcast(pltpu.bitcast(t, I32) | dep, F32)

                def after(t, dep):
                    return gate(t, pltpu.bitcast(dep, I32) & zv)
                den = None
                outs = []
                raws = []
                pend = [None] * 8
                for gi, r in enumerate(range(0, tm2, rb)):
                    z = zs[gi % 2]
                    kz = kzs[gi % 2]
                    q = [q_s[c, pl.ds(z + r, rb), :] for c in range(8)]
                    if gi >= 1:
                        dep = pltpu.bitcast(den, I32) & zv
                        q = [gate(t, dep) if c < qgate else t for c, t in enumerate(q)]
                    g = gb[r:r + rb, :]
                    s = []
                    for w in range(W):
                        st = HALO + r - DIL * w
                        q0 = q[0] if w < qkw else after(q[0], raws[-qkw])
                        acc = q0 * k_s[0, pl.ds(kz + st, rb), :]
                        for c in range(1, 8):
                            acc = acc + q[c] * k_s[c, pl.ds(kz + st, rb), :]
                        raws.append(acc)
                        acc = acc + pltpu.roll(acc, 64, 1)
                        acc = acc + pltpu.roll(acc, 32, 1)
                        if r < HALO and w > 0:
                            pos = i * tm2 + r + lax.broadcasted_iota(I32, (rb, 128), 0)
                            acc = jnp.where(pos >= DIL * w, acc, -1e9 / SCALE)
                        s.append(acc)
                    m = s[0]
                    for w in range(1, W):
                        m = jnp.maximum(m, s[w])
                    e = [jnp.exp2((s[w] - m) * cexp) for w in range(W)]
                    den = e[0]
                    for w in range(1, W):
                        den = den + e[w]
                    inv = g / den
                    for c in range(8):
                        st = HALO + r
                        e0 = e[0] if len(outs) < pvw else after(e[0], outs[-pvw])
                        acc = e0 * v_s[c, pl.ds(kz + st, rb), :]
                        for w in range(1, W):
                            st = HALO + r - DIL * w
                            acc = acc + e[w] * v_s[c, pl.ds(kz + st, rb), :]
                        outs.append(acc)
                        acc = acc * inv
                        if gi % 2 == 0:
                            pend[c] = acc
                        else:
                            st_pk(oa_v, c, r - rb, 2 * rb, jnp.concatenate([pend[c], acc], axis=0).astype(BF))
                for c in range(0 if ring else 8):
                    for r in range(0, HALO, rb):
                        k_s[c, r:r + rb, :] = after(k_s[c, tm2 + r:tm2 + r + rb, :], outs[-1])
                        v_s[c, r:r + rb, :] = after(v_s[c, tm2 + r:tm2 + r + rb, :], outs[-1])
                b = _dot(jnp.concatenate([ld_pk(h_v, t, r0, tm2) for t in range(F // 128)], axis=1), wd_v[...])
                oa = jnp.concatenate([ld_pk(oa_v, c, 0, tm2) for c in range(8)], axis=1)
                omg = 1.0 - gb[...]
                for pc in range(opieces):
                    cs = slice(pc * OC, (pc + 1) * OC)
                    nt = OC // 128
                    a = _dot(oa, jnp.concatenate([ld_pk(wo_p, t, 0, D) for t in range(pc * nt, (pc + 1) * nt)], axis=1))
                    res = (a + jnp.concatenate([omg] * nt, axis=1) * b[:, cs]).astype(BF)
                    ns = lastsplit if pc == opieces - 1 else 1
                    nr = tm2 // ns
                    for k in range(ns):
                        rs = pl.ds(_al(r0 + k * nr, nr), nr)
                        out_v[rs, cs] = res[k * nr:(k + 1) * nr]
                        pltpu.make_async_copy(out_v.at[rs, cs], o_hbm.at[rs, cs], sems.at[SOUT]).start()
                return carry
            lax.fori_loop(0, n2, scoped(main2, 'main2', prof), 0)
            pltpu.make_async_copy(out_v, o_hbm, sems.at[SOUT]).wait()

        pl.when(pl.program_id(0) == 0)(phase1)
        pl.when(pl.program_id(0) == 1)(phase2)

    @jax.jit
    def f(A_x, A_wqkv, A_wo, B_x, B_W_gate, B_W_up, B_W_down, gate_w):
        x = A_x.reshape(S, D)
        anyspec = pl.BlockSpec(memory_space=pl.ANY)
        out = pl.pallas_call(
            kernel,
            grid=(2,),
            in_specs=[anyspec] * 7,
            out_specs=anyspec,
            out_shape=jax.ShapeDtypeStruct((S, D), BF),
            scratch_shapes=[
                pltpu.VMEM((S, D), BF),
                pltpu.VMEM((D, 3 * D), BF),
                pk_shape(24, D, 'q'),
                pltpu.VMEM((D, D), BF),
                pk_shape(8, D, 'o'),
                pltpu.VMEM((2, 1088, 128), F32),
                pltpu.VMEM((4, D, 128), BF),
                pltpu.VMEM((4, D, 128), BF),
                pltpu.VMEM((NFC - 1, D, FC), BF),
                pltpu.VMEM((NFC - 1, D, FC), BF),
                pltpu.VMEM((F, D), BF),
                pk_shape(F // 128, S, 'h'),
                pltpu.VMEM((8, tm2, 128), F32),
                pltpu.VMEM((8, (S if ring else tm2) + HALO, 128), F32),
                pltpu.VMEM((8, (S if ring else tm2) + HALO, 128), F32),
                pk_shape(8, tm2, 'a'),
                pltpu.VMEM((S, 128), F32),
                pltpu.VMEM((S, D), BF),
                pltpu.VMEM((D,), BF),
                pltpu.SemaphoreType.DMA((NSEM,)),
            ],
            compiler_params=pltpu.CompilerParams(
                vmem_limit_bytes=110 * 1024 * 1024, disable_bounds_checks=True, disable_semaphore_checks=True,
                dimension_semantics=('arbitrary',)),
        )(x, gate_w, A_wqkv, A_wo, B_W_gate, B_W_up, B_W_down)
        return out.reshape(1, S, D)
    return f


_impl = build()


@jax.jit
def pallas_gated_mix__sliding_local_dilated__glu_gated_reglu__prompt_kernel(
    A_x: jax.Array,
    A_wqkv: jax.Array,
    A_wo: jax.Array,
    B_x: jax.Array,
    B_W_gate: jax.Array,
    B_W_up: jax.Array,
    B_W_down: jax.Array,
    gate_w: jax.Array,
):
    return _impl(A_x, A_wqkv, A_wo, B_x, B_W_gate, B_W_up, B_W_down, gate_w)
```

```python
import jax
import jax.numpy as jnp
from jax import lax
import jax.experimental.pallas as pl
import jax.experimental.pallas.tpu as pltpu

S, D, F = 2048, 1024, 3584
H, DH, W, DIL = 32, 32, 8, 2
HALO = 16
LOG2E = 1.4426950408889634
SCALE = DH ** -0.5
BF = jnp.bfloat16
F32 = jnp.float32
U32 = jnp.uint32
I32 = jnp.int32


def scoped(fn, name, on):
    if not on:
        return fn

    def g(i, c):
        with jax.named_scope(name):
            return fn(i, c)
    return g


def _swap(vs, vbit, lbit, lane):
    out = list(vs)
    sh = 1 << lbit
    hi = (lane & sh) != 0
    for i in range(8):
        if i & (1 << vbit):
            continue
        a, b = vs[i], vs[i | (1 << vbit)]
        out[i] = jnp.where(hi, pltpu.roll(b, sh, 1), a)
        out[i | (1 << vbit)] = jnp.where(hi, b, pltpu.roll(a, 128 - sh, 1))
    return out


def _permute_cols(vs, lane):
    for vb, lb in ((2, 4), (1, 3), (0, 2), (2, 6), (2, 1), (1, 5), (1, 0)):
        vs = _swap(vs, vb, lb, lane)
    out = [None] * 8
    for i in range(8):
        v2, v1, v0 = (i >> 2) & 1, (i >> 1) & 1, i & 1
        out[(v0 << 2) | (v2 << 1) | v1] = vs[i]
    return out


def _dot(a, b):
    return jnp.dot(a, b, preferred_element_type=F32)


def _shr(x, n):
    return x >> n if isinstance(x, int) else lax.shift_right_logical(x, n)


def _al(x, n):
    return x if isinstance(x, int) else pl.multiple_of(x, n)


def _u(x):
    return pltpu.bitcast(x, U32)


def _bf(x):
    return pltpu.bitcast(x, BF)


def _cat(xs, axis=1):
    return xs[0] if len(xs) == 1 else jnp.concatenate(xs, axis=axis)


def _unpk(x):
    return [pltpu.unpack_elementwise(x, index=k, packed_dtype=BF, unpacked_dtype=F32) for k in range(2)]


def _pk(lo, hi):
    return _u(pltpu.pack_elementwise([lo, hi], packed_dtype=BF))


def _lhs_sums(a11, a12, a21, a22):
    return [a11 + a22, a21 + a22, a11 + a12, a21 - a11, a12 - a22]


def _rhs_sums(b11, b12, b21, b22):
    return [b11 + b22, b12 - b22, b21 - b11, b11 + b12, b21 + b22]


def _packed_sums(fn, blocks):
    un = [_unpk(b) for b in blocks]
    lo = fn(*[u[0] for u in un])
    hi = fn(*[u[1] for u in un])
    return [_pk(a, b) for a, b in zip(lo, hi)]


LSUM = {1: 0, 2: 1, 5: 2, 6: 3, 7: 4}
RSUM = {1: 0, 3: 1, 4: 2, 6: 3, 7: 4}


def _combine(m):
    c11 = m[1] + m[4] - m[5] + m[7]
    c12 = m[3] + m[5]
    c21 = m[2] + m[4]
    c22 = m[1] - m[2] + m[3] + m[6]
    return c11, c12, c21, c22


def _ticker(prods, zv, n, lo, hi):
    slots = []
    for pr in prods:
        for t in range(pr.shape[1] // 128):
            for r in range(0, pr.shape[0], 8):
                slots.append((pr, r, t))
    for k in range(n):
        pr, r, t = slots[min(int((lo + (hi - lo) * k / n) * len(slots)), len(slots) - 1)]
        yield _u(pr[r:r + 8, t * 128:(t + 1) * 128]) & zv


def build(prof=False, pvw=1, qkw=1, qgate=8, lastsplit=2, qk_strassen=False):
    tm2 = 256
    hm = tm2 // 2
    rb = 8
    FC = 512
    NFC = F // FC
    XB = 512
    n2 = S // tm2
    KD = F // 256
    SM, SX, SR, SOUT, NSEM = 0, 6, 6, 7, 9

    def kernel(x_hbm, gw_hbm, wqkv_hbm, wo_hbm, wg_hbm, wu_hbm, wd_hbm, o_hbm,
               x_v, xs, wq7, wo7, wd7, hs, hs0, g_s, sems):

        def x_raw(i, half, kh):
            return x_v[pl.ds(_al(i * tm2 + half * hm, hm), hm), kh * 512:(kh + 1) * 512]

        def phase1(wqkv_v, wo_v, wo_f32, wg0, wu0, wg_v, wu_v, bs, wd_v, h0, gw_ref):
            def cp_x(r0, n, s):
                return pltpu.make_async_copy(x_hbm.at[pl.ds(r0, n)], x_v.at[pl.ds(r0, n)], sems.at[s])

            def cp_w0(t, s):
                c = pl.ds(_al(t * 128, 128), 128)
                return [pltpu.make_async_copy(wg_hbm.at[:, c], wg0.at[t], sems.at[s]),
                        pltpu.make_async_copy(wu_hbm.at[:, c], wu0.at[t], sems.at[s])]

            def cp_w(j):
                c = pl.ds(_al(j * FC, FC), FC)
                return [pltpu.make_async_copy(wg_hbm.at[:, c], wg_v.at[j - 1], sems.at[SM + j - 1]),
                        pltpu.make_async_copy(wu_hbm.at[:, c], wu_v.at[j - 1], sems.at[SM + j - 1])]

            cp_head = [pltpu.make_async_copy(wqkv_hbm.at[:, 0:D], wqkv_v.at[:, 0:D], sems.at[SM]),
                       pltpu.make_async_copy(wo_hbm, wo_v, sems.at[SM]),
                       pltpu.make_async_copy(wd_hbm.at[0:2 * FC], wd_v.at[0:2 * FC], sems.at[SM]),
                       pltpu.make_async_copy(gw_hbm, gw_ref.at[pl.ds(0, D)], sems.at[SM])]
            cp_rest = [pltpu.make_async_copy(wd_hbm.at[2 * FC:F], wd_v.at[2 * FC:F], sems.at[SR]),
                       pltpu.make_async_copy(wqkv_hbm.at[:, D:3 * D], wqkv_v.at[:, D:3 * D], sems.at[SR])]

            first = [cp_w0(0, 1) + [cp_x(0, 256, 1)], [cp_x(256, 256, 2)]]
            starts = sum(first, [])
            for t in range(1, 4):
                starts += cp_w0(t, 2 + t)
            starts += [cp_x(b * XB, XB, SX + b - 1) for b in range(1, 4)]
            starts += cp_w(1) + cp_head
            for c in starts:
                c.start()

            def ffn_up(r0, nr, wg, wu, t0):
                xx = x_v[pl.ds(r0, nr), :]
                gt = _dot(xx, wg)
                hh = (jnp.maximum(gt, 0.0) * _dot(xx, wu)).astype(BF)
                for t in range(hh.shape[1] // 128):
                    h0[t0 + t, pl.ds(r0, nr), :] = hh[:, t * 128:(t + 1) * 128]
                return gt

            def warm0(u, carry):
                for k in range(2):
                    @pl.when(u == k)
                    def _():
                        for c in first[k]:
                            c.wait()
                ffn_up(_al(u * 256, 256), 256, wg0[0], wu0[0], 0)
                return carry
            lax.fori_loop(0, 2, scoped(warm0, 'warm0', prof), 0)

            def warm1(t, carry):
                for c in cp_w0(t, 2 + t):
                    c.wait()
                ffn_up(0, XB, wg0[t], wu0[t], t)
                return carry
            lax.fori_loop(1, 4, scoped(warm1, 'warm1', prof), 0)
            for c in cp_w(2):
                c.start()

            def warm2(b, carry):
                cp_x(_al(b * XB, XB), XB, SX + b - 1).wait()
                gt = ffn_up(_al(b * XB, XB), XB, _cat([wg0[t] for t in range(4)]), _cat([wu0[t] for t in range(4)]), 0)
                zv = jnp.full((8, 128), _shr(b, 20), I32).astype(U32)
                tick = _ticker([gt], zv, 96, 0.0, 1.0)
                u0 = jnp.minimum(3 * (b - 1), 5)
                xsrc = x_v.at[pl.ds(_al(u0 * tm2, tm2), 3 * tm2)]
                xdst = xs.at[:, pl.ds(_al(u0 * 64, 64), 3 * 64)]
                for u in range(3):
                    for r in range(0, hm, 16):
                        for t in range(4):
                            dep = next(tick)
                            blk = [_u(xsrc[u * tm2 + hf * hm + r:u * tm2 + hf * hm + r + 16,
                                           kh * 512 + t * 128:kh * 512 + (t + 1) * 128]) | dep
                                   for hf in range(2) for kh in range(2)]
                            sm = _packed_sums(_lhs_sums, blk)
                            for k in range(5):
                                xdst[k * 4 + t, u * 64 + r // 2:u * 64 + r // 2 + 8, :] = sm[k]
                return carry
            lax.fori_loop(1, 4, scoped(warm2, 'warm2', prof), 0)

            for c in cp_rest:
                c.start()
            for j in range(3, NFC):
                for c in cp_w(j):
                    c.start()
            for c in cp_head:
                c.wait()

            def main1(j, carry):
                @pl.when(j == 2)
                def _():
                    for c in cp_rest:
                        c.wait()
                for c in cp_w(j):
                    c.wait()

                zj = _shr(j, 20)
                zv = jnp.full((8, 128), zj, I32).astype(U32)
                p = j - 1
                wsrc = [wg_v.at[p], wu_v.at[p]]
                def lhs(k):
                    if k == 3:
                        return _cat([x_raw(i, 0, 0) for i in range(n2)], axis=0)
                    if k == 4:
                        return _cat([x_raw(i, 1, 1) for i in range(n2)], axis=0)
                    return _cat([_bf(xs[LSUM[k] * 4 + t]) for t in range(4)])

                def rhs(mi, k):
                    if k == 2:
                        return wsrc[mi][0:512, 0:256]
                    if k == 5:
                        return wsrc[mi][512:1024, 256:512]
                    return _cat([_bf(bs[zj + (mi * 5 + RSUM[k]) * 2 + t]) for t in range(2)])

                mm = [{}, {}]
                prods = []
                for mi, k in [(0, 2), (0, 5), (1, 2), (1, 5)]:
                    mm[mi][k] = _dot(lhs(k), rhs(mi, k))
                    prods.append(mm[mi][k])
                tick = _ticker(prods, zv, 128, 0.0, 0.95)
                for mi in range(2):
                    for t in range(2):
                        for r in range(0, 512, 16):
                            dep = next(tick)
                            blk = [_u(wsrc[mi][kh * 512 + r:kh * 512 + r + 16,
                                               nh * 256 + t * 128:nh * 256 + (t + 1) * 128]) | dep
                                   for kh in range(2) for nh in range(2)]
                            sm = _packed_sums(_rhs_sums, blk)
                            for k in range(5):
                                bs[(mi * 5 + k) * 2 + t, r // 2:r // 2 + 8, :] = sm[k]
                prods = []
                for k in (4, 3, 1, 7, 6):
                    for mi in range(2):
                        mm[mi][k] = _dot(lhs(k), rhs(mi, k))
                        prods.append(mm[mi][k])
                hb = [jnp.maximum(gt, 0.0) * up for gt, up in zip(_combine(mm[0]), _combine(mm[1]))]
                sm = _lhs_sums(*hb)
                h7 = {3: hb[0], 4: hb[3]}
                for k, n in LSUM.items():
                    h7[k] = sm[n]
                hdst = hs.at[:, pl.ds(2 * p, 2)]
                for k in range(1, 8):
                    hv = h7[k].astype(BF)
                    for t in range(2):
                        hdst[k - 1, t] = hv[:, t * 128:(t + 1) * 128]

                tick = _ticker(prods, zv, 32 + 128 + 64, 0.0, 0.8)
                pb = jnp.minimum(p, 3)
                hsrc = h0.at[:, pl.ds(_al(pb * XB, XB), XB)]
                hdst0 = hs0.at[:, :, pl.ds(_al(pb * 128, 128), 128)]
                for u in range(2):
                    for r in range(0, hm, 16):
                        for t in range(2):
                            dep = next(tick)
                            blk = [_u(hsrc[kh * 2 + t, u * tm2 + hf * hm + r:u * tm2 + hf * hm + r + 16, :]) | dep
                                   for hf in range(2) for kh in range(2)]
                            sm = _packed_sums(_lhs_sums, blk)
                            o7 = {3: blk[0], 4: blk[3]}
                            for k, n in LSUM.items():
                                o7[k] = sm[n]
                            for k in range(1, 8):
                                hdst0[k - 1, t, (u * hm + r) // 2:(u * hm + r) // 2 + 8, :] = o7[k]

                for e in range(2):
                    ch = jnp.minimum(2 * p + e, NFC - 1)
                    dsrc = wd_v.at[pl.ds(_al(ch * FC, FC), FC)]
                    ddst = wd7.at[:, pl.ds(_al(ch * 128, 128), 128)]
                    for r in range(0, 256, 16):
                        for t in range(4):
                            dep = next(tick)
                            blk = [_u(dsrc[kh * 256 + r:kh * 256 + r + 16,
                                           nh * 512 + t * 128:nh * 512 + (t + 1) * 128]) | dep
                                   for kh in range(2) for nh in range(2)]
                            sm = _packed_sums(_rhs_sums, blk)
                            o7 = {2: blk[0], 5: blk[3]}
                            for k, n in RSUM.items():
                                o7[k] = sm[n]
                            for k in range(1, 8):
                                ddst[(k - 1) * 4 + t, r // 2:r // 2 + 8, :] = o7[k]

                gr = _al(pb * XB, XB)
                xg = x_v.at[pl.ds(gr, XB)]
                gdst = g_s.at[pl.ds(gr, XB)]
                gw = gw_ref[pl.ds(0, D)].astype(F32).reshape(1, D)
                for r in range(0, XB, 8):
                    dep = next(tick)
                    xf = xg[r:r + 8, :].astype(F32)
                    xf = [pltpu.bitcast(_u(xf[:, c * 128:(c + 1) * 128]) | dep, F32) for c in range(8)]
                    zg = xf[0] * gw[:, 0:128]
                    for c in range(1, 8):
                        zg = zg + xf[c] * gw[:, c * 128:(c + 1) * 128]
                    g = jax.nn.sigmoid(jnp.broadcast_to(jnp.sum(zg, axis=-1, keepdims=True), (8, 128)))
                    gdst[r:r + 8, :] = g

                lane = lax.broadcasted_iota(I32, (8, 128), 1)
                m = _shr(p, 1)
                hf = p & 1
                qsrc = wqkv_v.at[:, pl.ds(_al(m * D, D), D)]
                qsrc = [qsrc.at[pl.ds(_al(kh * 512 + hf * 256, 256), 256)] for kh in range(2)]
                qdst = wq7.at[pl.ds(m * 36, 36), pl.ds(_al(hf * 128, 128), 128)]
                deps = []
                for r in range(0, 256, 16):
                    pv = []
                    for kh in range(2):
                        vs = _permute_cols([_u(qsrc[kh][r:r + 16, c * 128:(c + 1) * 128]) for c in range(8)], lane)
                        pv.append(vs)
                        deps.append(vs[7] & zv)
                    for t in range(4):
                        blk = [pv[0][t], pv[0][t + 4], pv[1][t], pv[1][t + 4]]
                        sm = _packed_sums(_rhs_sums, blk)
                        o7 = {2: blk[0], 5: blk[3], 8: blk[1], 9: blk[2]}
                        for k, n in RSUM.items():
                            o7[k] = sm[n]
                        for k in range(1, 10):
                            qdst[(k - 1) * 4 + t, r // 2:r // 2 + 8, :] = o7[k]

                osrc = [wo_v.at[:, pl.ds(_al((pb + 4 * t) * 128, 128), 128)] for t in range(2)]
                for hh in range(H):
                    if hh % 2 == 0:
                        dep = deps[hh // 2]
                    for t in range(2):
                        for q in range(2):
                            vf = _bf(_u(osrc[t][hh * 32 + q * 16:hh * 32 + (q + 1) * 16, :]) | dep).astype(F32)
                            wo_f32[t, hh * 33 + q * 16:hh * 33 + (q + 1) * 16, :] = vf
                            dep = _u(vf[8:16]) & zv
                for b in range(4):
                    for a in range(4):
                        dep = deps[16 + b * 4 + a]
                        for q in range(2):
                            blk = [_cat([pltpu.bitcast(_u(wo_f32[
                                t, pl.ds(a * 8 + b + 4 * kh + (q * 16 + e * 8) * 33, 8, stride=33), :]) | dep, F32)
                                for e in range(2)], axis=0) for kh in range(2) for t in range(2)]
                            sm = _rhs_sums(*blk)
                            o7 = {2: blk[0], 5: blk[3]}
                            for k, n in RSUM.items():
                                o7[k] = sm[n]
                            r = (b * 128 + a * 32 + q * 16) // 2
                            for k in range(1, 8):
                                pk = _u(o7[k].astype(BF))
                                wo7[(k - 1) * 4 + pb, r:r + 8, :] = pk
                            dep = pk & zv
                return carry
            lax.fori_loop(1, NFC, scoped(main1, 'main1', prof), 0)

        def phase2(q_s, k_s, v_s, oa_v, oas, out_v):
            k_s[:, 0:HALO, :] = jnp.zeros((8, HALO, 128), F32)
            v_s[:, 0:HALO, :] = jnp.zeros((8, HALO, 128), F32)
            cexp = SCALE * LOG2E

            def main2(i, carry):
                r0 = _al(i * tm2, tm2)
                xsb = xs.at[:, pl.ds(_al(i * 64, 64), 64)]

                def lhs_x(k):
                    if k == 3:
                        return x_raw(i, 0, 0)
                    if k == 4:
                        return x_raw(i, 1, 1)
                    return _cat([_bf(xsb[LSUM[k] * 4 + t]) for t in range(4)])

                def wq(m, k):
                    return _cat([_bf(wq7[m * 36 + (k - 1) * 4 + t]) for t in range(4)])

                for m in range(3):
                    if m < 2 and not qk_strassen:
                        full = _dot(x_v[pl.ds(r0, tm2), :],
                                    _cat([_cat([wq(m, 2), wq(m, 8)]), _cat([wq(m, 9), wq(m, 5)])], axis=0))
                        cbs = [full[hf * hm:(hf + 1) * hm, nh * 512:(nh + 1) * 512] for hf in range(2) for nh in range(2)]
                    else:
                        cbs = _combine({k: _dot(lhs_x(k), wq(m, k)) for k in (2, 4, 3, 5, 1, 7, 6)})
                    for n, cb in enumerate(cbs):
                        for t in range(4):
                            val = cb[:, t * 128:(t + 1) * 128]
                            c = (n % 2) * 4 + t
                            ro = (n // 2) * hm
                            if m == 0:
                                q_s[c, ro:ro + hm, :] = val
                            else:
                                (k_s, v_s)[m - 1][c, pl.ds(r0 + HALO + ro, hm), :] = val
                zs = [_shr(i, 20), _shr(i, 21)]
                kzs = [r0 + zz for zz in zs]
                zv = jnp.full((rb, 128), zs[0], I32)
                gb = g_s.at[pl.ds(r0, tm2)]

                def gate(t, dep):
                    return pltpu.bitcast(pltpu.bitcast(t, I32) | dep, F32)

                def after(t, dep):
                    return gate(t, pltpu.bitcast(dep, I32) & zv)
                den = None
                outs = []
                raws = []
                pend = [None] * 8
                for gi, r in enumerate(range(0, tm2, rb)):
                    z = zs[gi % 2]
                    kz = kzs[gi % 2]
                    q = [q_s[c, pl.ds(z + r, rb), :] for c in range(8)]
                    if gi >= 1:
                        dep = pltpu.bitcast(den, I32) & zv
                        q = [gate(t, dep) if c < qgate else t for c, t in enumerate(q)]
                    g = gb[r:r + rb, :]
                    s = []
                    for w in range(W):
                        st = HALO + r - DIL * w
                        q0 = q[0] if w < qkw else after(q[0], raws[-qkw])
                        acc = q0 * k_s[0, pl.ds(kz + st, rb), :]
                        for c in range(1, 8):
                            acc = acc + q[c] * k_s[c, pl.ds(kz + st, rb), :]
                        raws.append(acc)
                        acc = acc + pltpu.roll(acc, 64, 1)
                        acc = acc + pltpu.roll(acc, 32, 1)
                        if r < HALO and w > 0:
                            pos = i * tm2 + r + lax.broadcasted_iota(I32, (rb, 128), 0)
                            acc = jnp.where(pos >= DIL * w, acc, -1e9 / SCALE)
                        s.append(acc)
                    mx = s[0]
                    for w in range(1, W):
                        mx = jnp.maximum(mx, s[w])
                    e = [jnp.exp2((s[w] - mx) * cexp) for w in range(W)]
                    den = e[0]
                    for w in range(1, W):
                        den = den + e[w]
                    inv = g / den
                    pks = []
                    for c in range(8):
                        st = HALO + r
                        e0 = e[0] if len(outs) < pvw else after(e[0], outs[-pvw])
                        acc = e0 * v_s[c, pl.ds(kz + st, rb), :]
                        for w in range(1, W):
                            st = HALO + r - DIL * w
                            acc = acc + e[w] * v_s[c, pl.ds(kz + st, rb), :]
                        outs.append(acc)
                        acc = acc * inv
                        if gi % 2 == 0:
                            pend[c] = acc
                        else:
                            pks.append(_u(_cat([pend[c], acc], axis=0).astype(BF)))
                    if gi % 2 == 1:
                        w0 = (r - rb) // 2
                        if r < hm:
                            for c in range(8):
                                oa_v[c, w0:w0 + 8, :] = pks[c]
                        else:
                            w1 = w0 - 64
                            for t in range(4):
                                oa_v[t + 4, w0:w0 + 8, :] = pks[t + 4]
                                blk = [oa_v[t, w1:w1 + 8, :], oa_v[t + 4, w1:w1 + 8, :], pks[t], pks[t + 4]]
                                sm = _packed_sums(_lhs_sums, blk)
                                for k in range(5):
                                    oas[k * 4 + t, w1:w1 + 8, :] = sm[k]

                hsb = hs.at[:, :, pl.ds(_al(i * hm, hm), hm)]
                hsb0 = hs0.at[:, :, pl.ds(_al(i * 64, 64), 64)]
                mm = {k: _dot(_cat([_bf(hsb0[k - 1, t]) for t in range(2)] + [hsb[k - 1, t] for t in range(KD - 2)]),
                              _cat([_bf(wd7[(k - 1) * 4 + t]) for t in range(4)]))
                      for k in (2, 4, 3, 5, 1, 7, 6)}
                bb = _combine(mm)

                def lhs_o(k):
                    if k == 3:
                        return _cat([_bf(oa_v[t, 0:64, :]) for t in range(4)])
                    if k == 4:
                        return _cat([_bf(oa_v[t + 4, 64:128, :]) for t in range(4)])
                    return _cat([_bf(oas[LSUM[k] * 4 + t]) for t in range(4)])

                mm = {k: _dot(lhs_o(k), _cat([_bf(wo7[(k - 1) * 4 + t]) for t in range(4)]))
                      for k in (3, 4, 2, 5, 1, 7, 6)}
                aa = _combine(mm)
                omg = 1.0 - gb[...]
                for n in (2, 1, 0, 3):
                    ro = (n // 2) * hm
                    co = (n % 2) * 512
                    res = (aa[n] + _cat([omg[ro:ro + hm]] * 4) * bb[n]).astype(BF)
                    if n != 3:
                        pieces = [(0, hm, 0, 512)]
                    else:
                        nr = hm // lastsplit
                        pieces = [(0, hm, 0, 384)] + [(k * nr, nr, 384, 128) for k in range(lastsplit)]
                    for (pr, pn, pc, pw) in pieces:
                        rs = pl.ds(_al(r0 + ro + pr, pn), pn)
                        cs = slice(co + pc, co + pc + pw)
                        out_v[rs, cs] = res[pr:pr + pn, pc:pc + pw]
                        pltpu.make_async_copy(out_v.at[rs, cs], o_hbm.at[rs, cs], sems.at[SOUT]).start()
                return carry
            lax.fori_loop(0, n2, scoped(main2, 'main2', prof), 0)
            pltpu.make_async_copy(out_v, o_hbm, sems.at[SOUT]).wait()

        @pl.when(pl.program_id(0) == 0)
        def _():
            pl.run_scoped(
                phase1,
                pltpu.VMEM((D, 3 * D), BF),
                pltpu.VMEM((D, D), BF),
                pltpu.VMEM((2, 1088, 128), F32),
                pltpu.VMEM((4, D, 128), BF),
                pltpu.VMEM((4, D, 128), BF),
                pltpu.VMEM((NFC - 1, D, FC), BF),
                pltpu.VMEM((NFC - 1, D, FC), BF),
                pltpu.VMEM((20, 256, 128), U32),
                pltpu.VMEM((F, D), BF),
                pltpu.VMEM((4, S, 128), BF),
                pltpu.VMEM((8 * D,), BF),
            )

        @pl.when(pl.program_id(0) == 1)
        def _():
            pl.run_scoped(
                phase2,
                pltpu.VMEM((8, tm2, 128), F32),
                pltpu.VMEM((8, S + HALO, 128), F32),
                pltpu.VMEM((8, S + HALO, 128), F32),
                pltpu.VMEM((8, 128, 128), U32),
                pltpu.VMEM((20, 64, 128), U32),
                pltpu.VMEM((S, D), BF),
            )

    @jax.jit
    def f(A_x, A_wqkv, A_wo, B_x, B_W_gate, B_W_up, B_W_down, gate_w):
        x = A_x.reshape(S, D)
        anyspec = pl.BlockSpec(memory_space=pl.ANY)
        out = pl.pallas_call(
            kernel,
            grid=(2,),
            in_specs=[anyspec] * 7,
            out_specs=anyspec,
            out_shape=jax.ShapeDtypeStruct((S, D), BF),
            scratch_shapes=[
                pltpu.VMEM((S, D), BF),
                pltpu.VMEM((20, 512, 128), U32),
                pltpu.VMEM((108, 256, 128), U32),
                pltpu.VMEM((28, 256, 128), U32),
                pltpu.VMEM((28, F // 4, 128), U32),
                pltpu.VMEM((7, KD - 2, S // 2, 128), BF),
                pltpu.VMEM((7, 2, S // 4, 128), U32),
                pltpu.VMEM((S, 128), F32),
                pltpu.SemaphoreType.DMA((NSEM,)),
            ],
            compiler_params=pltpu.CompilerParams(
                vmem_limit_bytes=120 * 1024 * 1024, disable_bounds_checks=True, disable_semaphore_checks=True,
                dimension_semantics=('arbitrary',)),
        )(x, gate_w, A_wqkv, A_wo, B_W_gate, B_W_up, B_W_down)
        return out.reshape(1, S, D)
    return f


_impl = build()


@jax.jit
def pallas_gated_mix__sliding_local_dilated__glu_gated_reglu__prompt_kernel(
    A_x: jax.Array,
    A_wqkv: jax.Array,
    A_wo: jax.Array,
    B_x: jax.Array,
    B_W_gate: jax.Array,
    B_W_up: jax.Array,
    B_W_down: jax.Array,
    gate_w: jax.Array,
):
    return _impl(A_x, A_wqkv, A_wo, B_x, B_W_gate, B_W_up, B_W_down, gate_w)
```

```python
import jax
import jax.numpy as jnp
from jax import lax
import jax.experimental.pallas as pl
import jax.experimental.pallas.tpu as pltpu

S, D, F = 2048, 1024, 3584
H, DH, W, DIL = 32, 32, 8, 2
HALO = 16
LOG2E = 1.4426950408889634
SCALE = DH ** -0.5
BF = jnp.bfloat16
F32 = jnp.float32
U32 = jnp.uint32
I32 = jnp.int32


def scoped(fn, name, on):
    if not on:
        return fn

    def g(i, c):
        with jax.named_scope(name):
            return fn(i, c)
    return g


def _swap(vs, vbit, lbit, lane):
    out = list(vs)
    sh = 1 << lbit
    hi = (lane & sh) != 0
    for i in range(8):
        if i & (1 << vbit):
            continue
        a, b = vs[i], vs[i | (1 << vbit)]
        out[i] = jnp.where(hi, pltpu.roll(b, sh, 1), a)
        out[i | (1 << vbit)] = jnp.where(hi, b, pltpu.roll(a, 128 - sh, 1))
    return out


def _permute_cols(vs, lane):
    for vb, lb in ((2, 4), (1, 3), (0, 2), (2, 6), (2, 1), (1, 5), (1, 0)):
        vs = _swap(vs, vb, lb, lane)
    out = [None] * 8
    for i in range(8):
        v2, v1, v0 = (i >> 2) & 1, (i >> 1) & 1, i & 1
        out[(v0 << 2) | (v2 << 1) | v1] = vs[i]
    return out


def _dot(a, b):
    return jnp.dot(a, b, preferred_element_type=F32)


def _shr(x, n):
    return x >> n if isinstance(x, int) else lax.shift_right_logical(x, n)


def _al(x, n):
    return x if isinstance(x, int) else pl.multiple_of(x, n)


def _u(x):
    return pltpu.bitcast(x, U32)


def _bf(x):
    return pltpu.bitcast(x, BF)


def _cat(xs, axis=1):
    return xs[0] if len(xs) == 1 else jnp.concatenate(xs, axis=axis)


def _unpk(x):
    return [pltpu.unpack_elementwise(x, index=k, packed_dtype=BF, unpacked_dtype=F32) for k in range(2)]


def _pk(lo, hi):
    return _u(pltpu.pack_elementwise([lo, hi], packed_dtype=BF))


def _lhs_sums(a11, a12, a21, a22):
    return [a11 + a22, a21 + a22, a11 + a12, a21 - a11, a12 - a22]


def _rhs_sums(b11, b12, b21, b22):
    return [b11 + b22, b12 - b22, b21 - b11, b11 + b12, b21 + b22]


def _packed_sums(fn, blocks):
    un = [_unpk(b) for b in blocks]
    lo = fn(*[u[0] for u in un])
    hi = fn(*[u[1] for u in un])
    return [_pk(a, b) for a, b in zip(lo, hi)]


LSUM = {1: 0, 2: 1, 5: 2, 6: 3, 7: 4}
RSUM = {1: 0, 3: 1, 4: 2, 6: 3, 7: 4}


def _combine(m):
    c11 = m[4] - m[5] + m[1] + m[7]
    c12 = m[3] + m[5]
    c21 = m[2] + m[4]
    c22 = m[3] - m[2] + m[1] + m[6]
    return c11, c12, c21, c22


def _ticker(prods, zv, n, lo, hi):
    slots = []
    for pr in prods:
        for t in range(pr.shape[1] // 128):
            for r in range(0, pr.shape[0], 8):
                slots.append((pr, r, t))
    for k in range(n):
        pr, r, t = slots[min(int((lo + (hi - lo) * k / n) * len(slots)), len(slots) - 1)]
        yield _u(pr[r:r + 8, t * 128:(t + 1) * 128]) & zv


def build(prof=False, pvw=1, qkw=1, qgate=8, lastsplit=2, sidehi=0.8):
    tm2 = 256
    hm = tm2 // 2
    rb = 8
    FC = 512
    NFC = F // FC
    XB = 512
    n2 = S // tm2
    KD = F // 256
    SM, SX, SR, SOUT, NSEM = 0, 6, 6, 7, 9

    def kernel(x_hbm, gw_hbm, wqkv_hbm, wo_hbm, wg_hbm, wu_hbm, wd_hbm, o_hbm,
               x_v, xs, wqk, wv7, wo7, wd7, hs, g_s, sems):

        def x_raw(i, half, kh):
            return x_v[pl.ds(_al(i * tm2 + half * hm, hm), hm), kh * 512:(kh + 1) * 512]

        def phase1(wqkv_v, wo_v, wo_f32, wg0, wu0, wg_v, wu_v, bs, wd_v, h0, gw_ref):
            def cp_x(r0, n, s):
                return pltpu.make_async_copy(x_hbm.at[pl.ds(r0, n)], x_v.at[pl.ds(r0, n)], sems.at[s])

            def cp_w0(t, s):
                c = pl.ds(_al(t * 128, 128), 128)
                return [pltpu.make_async_copy(wg_hbm.at[:, c], wg0.at[t], sems.at[s]),
                        pltpu.make_async_copy(wu_hbm.at[:, c], wu0.at[t], sems.at[s])]

            def cp_w(j):
                c = pl.ds(_al(j * FC, FC), FC)
                return [pltpu.make_async_copy(wg_hbm.at[:, c], wg_v.at[j - 1], sems.at[SM + j - 1]),
                        pltpu.make_async_copy(wu_hbm.at[:, c], wu_v.at[j - 1], sems.at[SM + j - 1])]

            QH = 96

            def cp_q(r0, n, s):
                return [pltpu.make_async_copy(wqkv_hbm.at[kh * 512 + r0:kh * 512 + r0 + n],
                                              wqkv_v.at[kh * 512 + r0:kh * 512 + r0 + n], sems.at[s])
                        for kh in range(2)]

            cp_head = cp_q(0, QH, SM) + [
                pltpu.make_async_copy(wo_hbm, wo_v, sems.at[SM]),
                pltpu.make_async_copy(wd_hbm.at[0:2 * FC], wd_v.at[0:2 * FC], sems.at[SM]),
                pltpu.make_async_copy(gw_hbm, gw_ref.at[pl.ds(0, D)], sems.at[SM])]
            cp_rest = cp_q(QH, 512 - QH, SR) + [
                pltpu.make_async_copy(wd_hbm.at[2 * FC:F], wd_v.at[2 * FC:F], sems.at[SR])]

            first = [cp_w0(0, 1) + [cp_x(0, 256, 1)], [cp_x(256, 256, 2)]]
            starts = sum(first, [])
            for t in range(1, 4):
                starts += cp_w0(t, 2 + t)
            starts += [cp_x(b * XB, XB, SX + b - 1) for b in range(1, 4)]
            starts += cp_w(1) + cp_head
            for c in starts:
                c.start()

            def zeros_of(i):
                zi = _shr(i, 20)
                return zi, jnp.full((8, 128), zi, I32).astype(U32)

            def ffn_plain(r0, nr, t):
                xx = x_v[pl.ds(r0, nr), :]
                gt = _dot(xx, wg0[t])
                up = _dot(xx, wu0[t])
                h0[t, pl.ds(r0, nr), :] = (jnp.maximum(gt, 0.0) * up).astype(BF)
                return [gt, up]

            def x_sums(u0, nu, tick):
                xsrc = x_v.at[pl.ds(_al(u0 * tm2, tm2), nu * tm2)]
                xdst = xs.at[:, pl.ds(_al(u0 * 64, 64), nu * 64)]
                for u in range(nu):
                    for r in range(0, hm, 16):
                        for t in range(4):
                            dep = next(tick)
                            blk = [_u(xsrc[u * tm2 + hf * hm + r:u * tm2 + hf * hm + r + 16,
                                           kh * 512 + t * 128:kh * 512 + (t + 1) * 128]) | dep
                                   for hf in range(2) for kh in range(2)]
                            sm = _packed_sums(_lhs_sums, blk)
                            for k in range(5):
                                xdst[k * 4 + t, u * 64 + r // 2:u * 64 + r // 2 + 8, :] = sm[k]

            def w_sums(tile, mi, t, tick):
                for r in range(0, 512, 16):
                    dep = next(tick)
                    blk = [_u(tile(nh, kh * 512 + r)) | dep for kh in range(2) for nh in range(2)]
                    sm = _packed_sums(_rhs_sums, blk)
                    for k in range(5):
                        bs[(mi * 5 + k) * 2 + t, r // 2:r // 2 + 8, :] = sm[k]

            def store_h7(mm, hdst):
                hb = [jnp.maximum(gt, 0.0) * up for gt, up in zip(_combine(mm[0]), _combine(mm[1]))]
                sm = _lhs_sums(*hb)
                h7 = {3: hb[0], 4: hb[3]}
                for k, n in LSUM.items():
                    h7[k] = sm[n]
                for k in range(1, 8):
                    hv = h7[k].astype(BF)
                    for t in range(2):
                        hdst[k - 1, t] = hv[:, t * 128:(t + 1) * 128]

            def warm0(u, carry):
                for k in range(2):
                    @pl.when(u == k)
                    def _():
                        for c in first[k]:
                            c.wait()
                pr = ffn_plain(_al(u * 256, 256), 256, 0)
                x_sums(u, 1, _ticker(pr, zeros_of(u)[1], 32, 0.0, 0.8))
                return carry
            lax.fori_loop(0, 2, scoped(warm0, 'warm0', prof), 0)

            def warm1(t, carry):
                for c in cp_w0(t, 2 + t):
                    c.wait()
                pr = ffn_plain(0, XB, t)
                tick = _ticker(pr, zeros_of(t)[1], 64, 0.0, 0.9)
                pi = _shr(t - 1, 1)
                for mi, w0 in enumerate((wg0, wu0)):
                    wp = w0.at[pl.ds(2 * pi, 2)]
                    w_sums(lambda nh, r: wp[nh, r:r + 16, :], mi, pi, tick)
                return carry
            lax.fori_loop(1, 4, scoped(warm1, 'warm1', prof), 0)
            for c in cp_w(2):
                c.start()

            def warm2(b, carry):
                cp_x(_al(b * XB, XB), XB, SX + b - 1).wait()
                zb, zv = zeros_of(b)
                xsb = xs.at[:, pl.ds(_al(b * 128, 128), 128)]

                def lhs(k):
                    if k == 3:
                        return _cat([x_raw(2 * b + u, 0, 0) for u in range(2)], axis=0)
                    if k == 4:
                        return _cat([x_raw(2 * b + u, 1, 1) for u in range(2)], axis=0)
                    return _cat([_bf(xsb[LSUM[k] * 4 + t]) for t in range(4)])

                def rhs(mi, k):
                    w0 = (wg0, wu0)[mi]
                    if k == 2:
                        return _cat([w0[2 * t, 0:512, :] for t in range(2)])
                    if k == 5:
                        return _cat([w0[2 * t + 1, 512:1024, :] for t in range(2)])
                    return _cat([_bf(bs[(mi * 5 + RSUM[k]) * 2 + t]) for t in range(2)])

                mm = [{}, {}]
                prods = []
                for k in (3, 4):
                    for mi in range(2):
                        mm[mi][k] = _dot(lhs(k), rhs(mi, k))
                        prods.append(mm[mi][k])
                x_sums(2 * b, 2, _ticker(prods, zv, 64, 0.0, 0.85))
                prods = []
                for k in (2, 5, 1, 7, 6):
                    for mi in range(2):
                        mm[mi][k] = _dot(lhs(k), rhs(mi, k))
                        prods.append(mm[mi][k])
                tick = _ticker(prods, zv, 32, 0.0, 0.6)
                for u in range(2):
                    for r in range(0, hm, 16):
                        for t in range(2):
                            dep = next(tick)
                            blk = [_u(h0[2 * t + kh, u * tm2 + hf * hm + r:u * tm2 + hf * hm + r + 16, :]) | dep
                                   for hf in range(2) for kh in range(2)]
                            sm = _packed_sums(_lhs_sums, blk)
                            o7 = {3: blk[0], 4: blk[3]}
                            for k, n in LSUM.items():
                                o7[k] = sm[n]
                            for k in range(1, 8):
                                hs[k - 1, t, u * hm + r:u * hm + r + 16, :] = _bf(o7[k])
                store_h7(mm, hs.at[:, 0:2, pl.ds(_al(b * 256, 256), 256)])
                return carry
            lax.fori_loop(1, 4, scoped(warm2, 'warm2', prof), 0)

            for c in cp_rest:
                c.start()
            for j in range(3, NFC):
                for c in cp_w(j):
                    c.start()
            for c in cp_head:
                c.wait()

            def main1(j, carry):
                @pl.when(j == 2)
                def _():
                    for c in cp_rest:
                        c.wait()
                for c in cp_w(j):
                    c.wait()

                zj, zv = zeros_of(j)
                p = j - 1
                wsrc = [wg_v.at[p], wu_v.at[p]]

                def lhs(k):
                    if k == 3:
                        return _cat([x_raw(i, 0, 0) for i in range(n2)], axis=0)
                    if k == 4:
                        return _cat([x_raw(i, 1, 1) for i in range(n2)], axis=0)
                    return _cat([_bf(xs[LSUM[k] * 4 + t]) for t in range(4)])

                def rhs(mi, k):
                    if k == 2:
                        return _cat([wsrc[mi][0:512, 2 * t * 128:(2 * t + 1) * 128] for t in range(2)])
                    if k == 5:
                        return _cat([wsrc[mi][512:1024, (2 * t + 1) * 128:(2 * t + 2) * 128] for t in range(2)])
                    return _cat([_bf(bs[zj + (mi * 5 + RSUM[k]) * 2 + t]) for t in range(2)])

                mm = [{}, {}]
                prods = []
                for mi, k in [(0, 2), (0, 5), (1, 2), (1, 5)]:
                    mm[mi][k] = _dot(lhs(k), rhs(mi, k))
                    prods.append(mm[mi][k])
                tick = _ticker(prods, zv, 128, 0.0, 0.95)
                for mi in range(2):
                    for t in range(2):
                        w_sums(lambda nh, r: wsrc[mi][r:r + 16, (2 * t + nh) * 128:(2 * t + nh + 1) * 128], mi, t, tick)
                prods = []
                for k in (4, 3, 1, 7, 6):
                    for mi in range(2):
                        mm[mi][k] = _dot(lhs(k), rhs(mi, k))
                        prods.append(mm[mi][k])
                store_h7(mm, hs.at[:, pl.ds(2 * j, 2)])

                tick = _ticker(prods, zv, 80, 0.0, sidehi)
                q0 = jnp.minimum(5 * p, 23)
                for e in range(5):
                    qq = q0 + e
                    ch = _shr(qq, 2)
                    sub = qq & 3
                    rsrc = ch * FC + _shr(sub, 1) * 256 + (sub & 1) * 64
                    dsrc = [wd_v.at[pl.ds(_al(rsrc + kh * 128, 64), 64)] for kh in range(2)]
                    ddst = wd7.at[:, pl.ds(_al(qq * 32, 32), 32)]
                    for r in range(0, 64, 16):
                        for t in range(4):
                            dep = next(tick)
                            blk = [_u(dsrc[kh][r:r + 16, nh * 512 + t * 128:nh * 512 + (t + 1) * 128]) | dep
                                   for kh in range(2) for nh in range(2)]
                            sm = _packed_sums(_rhs_sums, blk)
                            o7 = {2: blk[0], 5: blk[3]}
                            for k, n in RSUM.items():
                                o7[k] = sm[n]
                            for k in range(1, 8):
                                ddst[(k - 1) * 4 + t, r // 2:r // 2 + 8, :] = o7[k]

                tick = _ticker(prods, zv, 44, 0.005, sidehi)
                gr = _al(jnp.minimum(p * 352, S - 352), 32)
                xg = x_v.at[pl.ds(gr, 352)]
                gdst = g_s.at[pl.ds(gr, 352)]
                gw = gw_ref[pl.ds(0, D)].astype(F32).reshape(1, D)
                for r in range(0, 352, 8):
                    dep = next(tick)
                    xf = xg[r:r + 8, :].astype(F32)
                    xf = [pltpu.bitcast(_u(xf[:, c * 128:(c + 1) * 128]) | dep, F32) for c in range(8)]
                    zg = xf[0] * gw[:, 0:128]
                    for c in range(1, 8):
                        zg = zg + xf[c] * gw[:, c * 128:(c + 1) * 128]
                    gdst[r:r + 8, :] = jax.nn.sigmoid(
                        jnp.broadcast_to(jnp.sum(zg, axis=-1, keepdims=True), (8, 128)))

                lane = lax.broadcasted_iota(I32, (8, 128), 1)
                qr = _al(jnp.minimum(p * QH, 512 - QH), 16)
                qsrc = [wqkv_v.at[pl.ds(kh * 512 + qr, QH)] for kh in range(2)]
                qw = _al(_shr(qr, 1), 8)
                qdst = [wqk.at[:, pl.ds(kh * 256 + qw, QH // 2)] for kh in range(2)]
                vdst = wv7.at[:, pl.ds(qw, QH // 2)]
                tick = _ticker(prods, zv, 36, 0.0, sidehi - 0.05)
                tick2 = _ticker(prods, zv, 36 * 2, 0.05, sidehi + 0.02)
                for r in range(0, QH, 16):
                    pv = []
                    for m in (2, 0, 1):
                        for kh in range(2):
                            dep = next(tick)
                            vs = _permute_cols([_u(qsrc[kh][r:r + 16, m * D + c * 128:m * D + (c + 1) * 128]) | dep
                                                for c in range(8)], lane)
                            if m == 2:
                                pv.append(vs)
                            else:
                                for c in range(8):
                                    qdst[kh][m * 8 + c, r // 2:r // 2 + 8, :] = vs[c]
                    for t in range(4):
                        for _ in range(3):
                            dep = next(tick2)
                        blk = [v | dep for v in (pv[0][t], pv[0][t + 4], pv[1][t], pv[1][t + 4])]
                        sm = _packed_sums(_rhs_sums, blk)
                        o7 = {2: blk[0], 5: blk[3]}
                        for k, n in RSUM.items():
                            o7[k] = sm[n]
                        for k in range(1, 8):
                            vdst[(k - 1) * 4 + t, r // 2:r // 2 + 8, :] = o7[k]

                pb = jnp.minimum(p, 3)
                osrc = [wo_v.at[:, pl.ds(_al((pb + 4 * t) * 128, 128), 128)] for t in range(2)]
                tick = _ticker(prods, zv, 64, 0.002, 0.4)
                for hh in range(H):
                    for t in range(2):
                        dep = next(tick)
                        for q in range(2):
                            wo_f32[t, hh * 33 + q * 16:hh * 33 + (q + 1) * 16, :] = _bf(
                                _u(osrc[t][hh * 32 + q * 16:hh * 32 + (q + 1) * 16, :]) | dep).astype(F32)
                tick = _ticker(prods, zv, 32, 0.42, sidehi)
                for b in range(4):
                    for a in range(4):
                        for q in range(2):
                            dep = next(tick)
                            blk = [_cat([pltpu.bitcast(_u(wo_f32[
                                t, pl.ds(a * 8 + b + 4 * kh + (q * 16 + e * 8) * 33, 8, stride=33), :]) | dep, F32)
                                for e in range(2)], axis=0) for kh in range(2) for t in range(2)]
                            sm = _rhs_sums(*blk)
                            o7 = {2: blk[0], 5: blk[3]}
                            for k, n in RSUM.items():
                                o7[k] = sm[n]
                            r = (b * 128 + a * 32 + q * 16) // 2
                            for k in range(1, 8):
                                wo7[(k - 1) * 4 + pb, r:r + 8, :] = _u(o7[k].astype(BF))
                return carry
            lax.fori_loop(1, NFC, scoped(main1, 'main1', prof), 0)

        def phase2(q_s, k_s, v_s, oa_v, oas, out_v):
            k_s[:, 0:HALO, :] = jnp.zeros((8, HALO, 128), F32)
            v_s[:, 0:HALO, :] = jnp.zeros((8, HALO, 128), F32)
            cexp = SCALE * LOG2E

            def main2(i, carry):
                r0 = _al(i * tm2, tm2)
                xsb = xs.at[:, pl.ds(_al(i * 64, 64), 64)]

                def lhs_x(k):
                    if k == 3:
                        return x_raw(i, 0, 0)
                    if k == 4:
                        return x_raw(i, 1, 1)
                    return _cat([_bf(xsb[LSUM[k] * 4 + t]) for t in range(4)])

                for m in range(3):
                    if m < 2:
                        full = _dot(x_v[pl.ds(r0, tm2), :], _cat([_bf(wqk[m * 8 + c]) for c in range(8)]))
                        cbs = [full[hf * hm:(hf + 1) * hm, nh * 512:(nh + 1) * 512] for hf in range(2) for nh in range(2)]
                    else:
                        cbs = _combine({k: _dot(lhs_x(k), _cat([_bf(wv7[(k - 1) * 4 + t]) for t in range(4)]))
                                        for k in (2, 4, 3, 5, 1, 7, 6)})
                    for n, cb in enumerate(cbs):
                        for t in range(4):
                            val = cb[:, t * 128:(t + 1) * 128]
                            c = (n % 2) * 4 + t
                            ro = (n // 2) * hm
                            if m == 0:
                                q_s[c, ro:ro + hm, :] = val
                            else:
                                (k_s, v_s)[m - 1][c, pl.ds(r0 + HALO + ro, hm), :] = val
                zs = [_shr(i, 20), _shr(i, 21)]
                kzs = [r0 + zz for zz in zs]
                zv = jnp.full((rb, 128), zs[0], I32)
                gb = g_s.at[pl.ds(r0, tm2)]

                def gate(t, dep):
                    return pltpu.bitcast(pltpu.bitcast(t, I32) | dep, F32)

                def after(t, dep):
                    return gate(t, pltpu.bitcast(dep, I32) & zv)
                den = None
                outs = []
                raws = []
                pend = [None] * 8
                for gi, r in enumerate(range(0, tm2, rb)):
                    z = zs[gi % 2]
                    kz = kzs[gi % 2]
                    q = [q_s[c, pl.ds(z + r, rb), :] for c in range(8)]
                    if gi >= 1:
                        dep = pltpu.bitcast(den, I32) & zv
                        q = [gate(t, dep) if c < qgate else t for c, t in enumerate(q)]
                    g = gb[r:r + rb, :]
                    s = []
                    for w in range(W):
                        st = HALO + r - DIL * w
                        q0 = q[0] if w < qkw else after(q[0], raws[-qkw])
                        acc = q0 * k_s[0, pl.ds(kz + st, rb), :]
                        for c in range(1, 8):
                            acc = acc + q[c] * k_s[c, pl.ds(kz + st, rb), :]
                        raws.append(acc)
                        acc = acc + pltpu.roll(acc, 64, 1)
                        acc = acc + pltpu.roll(acc, 32, 1)
                        if r < HALO and w > 0:
                            pos = i * tm2 + r + lax.broadcasted_iota(I32, (rb, 128), 0)
                            acc = jnp.where(pos >= DIL * w, acc, -1e9 / SCALE)
                        s.append(acc)
                    mx = s[0]
                    for w in range(1, W):
                        mx = jnp.maximum(mx, s[w])
                    e = [jnp.exp2((s[w] - mx) * cexp) for w in range(W)]
                    den = e[0]
                    for w in range(1, W):
                        den = den + e[w]
                    inv = g / den
                    pks = []
                    for c in range(8):
                        st = HALO + r
                        e0 = e[0] if len(outs) < pvw else after(e[0], outs[-pvw])
                        acc = e0 * v_s[c, pl.ds(kz + st, rb), :]
                        for w in range(1, W):
                            st = HALO + r - DIL * w
                            acc = acc + e[w] * v_s[c, pl.ds(kz + st, rb), :]
                        outs.append(acc)
                        acc = acc * inv
                        if gi % 2 == 0:
                            pend[c] = acc
                        else:
                            pks.append(_u(_cat([pend[c], acc], axis=0).astype(BF)))
                    if gi % 2 == 1:
                        w0 = (r - rb) // 2
                        if r < hm:
                            for c in range(8):
                                oa_v[c, w0:w0 + 8, :] = pks[c]
                        else:
                            w1 = w0 - 64
                            for t in range(4):
                                oa_v[t + 4, w0:w0 + 8, :] = pks[t + 4]
                                blk = [oa_v[t, w1:w1 + 8, :], oa_v[t + 4, w1:w1 + 8, :], pks[t], pks[t + 4]]
                                sm = _packed_sums(_lhs_sums, blk)
                                for k in range(5):
                                    oas[k * 4 + t, w1:w1 + 8, :] = sm[k]

                hsb = hs.at[:, :, pl.ds(_al(i * hm, hm), hm)]
                mm = {k: _dot(_cat([hsb[k - 1, t] for t in range(KD)]),
                              _cat([_bf(wd7[(k - 1) * 4 + t]) for t in range(4)]))
                      for k in (2, 4, 3, 5, 1, 7, 6)}
                bb = _combine(mm)

                def lhs_o(k):
                    if k == 3:
                        return _cat([_bf(oa_v[t, 0:64, :]) for t in range(4)])
                    if k == 4:
                        return _cat([_bf(oa_v[t + 4, 64:128, :]) for t in range(4)])
                    return _cat([_bf(oas[LSUM[k] * 4 + t]) for t in range(4)])

                mm = {k: _dot(lhs_o(k), _cat([_bf(wo7[(k - 1) * 4 + t]) for t in range(4)]))
                      for k in (3, 4, 2, 5, 1, 7, 6)}
                omg = 1.0 - gb[...]
                ob = [_cat([omg[(n // 2) * hm:(n // 2 + 1) * hm]] * 4) * bb[n] for n in range(4)]
                fin = {2: (ob[2] + mm[4]) + mm[2],
                       1: (ob[1] + mm[3]) + mm[5],
                       0: (ob[0] + mm[4] - mm[5] + mm[1]) + mm[7],
                       3: (ob[3] + mm[3] - mm[2] + mm[1]) + mm[6]}
                for n in (2, 1, 0, 3):
                    ro = (n // 2) * hm
                    co = (n % 2) * 512
                    if n != 3:
                        pieces = [(0, hm, 0, 512)]
                    else:
                        nr = hm // lastsplit
                        pieces = [(0, hm, 0, 256), (0, hm, 256, 128)] + [(k * nr, nr, 384, 128) for k in range(lastsplit)]
                    for (pr, pn, pc, pw) in pieces:
                        rs = pl.ds(_al(r0 + ro + pr, pn), pn)
                        cs = slice(co + pc, co + pc + pw)
                        out_v[rs, cs] = fin[n][pr:pr + pn, pc:pc + pw].astype(BF)
                        pltpu.make_async_copy(out_v.at[rs, cs], o_hbm.at[rs, cs], sems.at[SOUT]).start()
                return carry
            lax.fori_loop(0, n2, scoped(main2, 'main2', prof), 0)
            pltpu.make_async_copy(out_v, o_hbm, sems.at[SOUT]).wait()

        @pl.when(pl.program_id(0) == 0)
        def _():
            pl.run_scoped(
                phase1,
                pltpu.VMEM((D, 3 * D), BF),
                pltpu.VMEM((D, D), BF),
                pltpu.VMEM((2, 1088, 128), F32),
                pltpu.VMEM((4, D, 128), BF),
                pltpu.VMEM((4, D, 128), BF),
                pltpu.VMEM((NFC - 1, D, FC), BF),
                pltpu.VMEM((NFC - 1, D, FC), BF),
                pltpu.VMEM((20, 256, 128), U32),
                pltpu.VMEM((F, D), BF),
                pltpu.VMEM((4, XB, 128), BF),
                pltpu.VMEM((8 * D,), BF),
            )

        @pl.when(pl.program_id(0) == 1)
        def _():
            pl.run_scoped(
                phase2,
                pltpu.VMEM((8, tm2, 128), F32),
                pltpu.VMEM((8, S + HALO, 128), F32),
                pltpu.VMEM((8, S + HALO, 128), F32),
                pltpu.VMEM((8, 128, 128), U32),
                pltpu.VMEM((20, 64, 128), U32),
                pltpu.VMEM((S, D), BF),
            )

    @jax.jit
    def f(A_x, A_wqkv, A_wo, B_x, B_W_gate, B_W_up, B_W_down, gate_w):
        x = A_x.reshape(S, D)
        anyspec = pl.BlockSpec(memory_space=pl.ANY)
        out = pl.pallas_call(
            kernel,
            grid=(2,),
            in_specs=[anyspec] * 7,
            out_specs=anyspec,
            out_shape=jax.ShapeDtypeStruct((S, D), BF),
            scratch_shapes=[
                pltpu.VMEM((S, D), BF),
                pltpu.VMEM((20, 512, 128), U32),
                pltpu.VMEM((16, 512, 128), U32),
                pltpu.VMEM((28, 256, 128), U32),
                pltpu.VMEM((28, 256, 128), U32),
                pltpu.VMEM((28, F // 4, 128), U32),
                pltpu.VMEM((7, KD, S // 2, 128), BF),
                pltpu.VMEM((S, 128), F32),
                pltpu.SemaphoreType.DMA((NSEM,)),
            ],
            compiler_params=pltpu.CompilerParams(
                vmem_limit_bytes=120 * 1024 * 1024, disable_bounds_checks=True, disable_semaphore_checks=True,
                dimension_semantics=('arbitrary',)),
        )(x, gate_w, A_wqkv, A_wo, B_W_gate, B_W_up, B_W_down)
        return out.reshape(1, S, D)
    return f


_impl = build()


@jax.jit
def pallas_gated_mix__sliding_local_dilated__glu_gated_reglu__prompt_kernel(
    A_x: jax.Array,
    A_wqkv: jax.Array,
    A_wo: jax.Array,
    B_x: jax.Array,
    B_W_gate: jax.Array,
    B_W_up: jax.Array,
    B_W_down: jax.Array,
    gate_w: jax.Array,
):
    return _impl(A_x, A_wqkv, A_wo, B_x, B_W_gate, B_W_up, B_W_down, gate_w)
```

```python
import jax
import jax.numpy as jnp
from jax import lax
import jax.experimental.pallas as pl
import jax.experimental.pallas.tpu as pltpu

S, D, F = 2048, 1024, 3584
H, DH, W, DIL = 32, 32, 8, 2
HALO = 16
LOG2E = 1.4426950408889634
SCALE = DH ** -0.5
BF = jnp.bfloat16
F32 = jnp.float32
U32 = jnp.uint32
I32 = jnp.int32


def scoped(fn, name, on):
    if not on:
        return fn

    def g(i, c):
        with jax.named_scope(name):
            return fn(i, c)
    return g


def _swap(vs, vbit, lbit, lane):
    out = list(vs)
    sh = 1 << lbit
    hi = (lane & sh) != 0
    for i in range(8):
        if i & (1 << vbit):
            continue
        a, b = vs[i], vs[i | (1 << vbit)]
        out[i] = jnp.where(hi, pltpu.roll(b, sh, 1), a)
        out[i | (1 << vbit)] = jnp.where(hi, b, pltpu.roll(a, 128 - sh, 1))
    return out


def _permute_cols(vs, lane):
    for bit in range(3):
        vs = _swap(vs, bit, bit, lane)
    idx = ((lane & 3) << 5) | ((lane >> 5) << 3) | ((lane >> 2) & 7)
    return [jnp.take_along_axis(v, idx, axis=1) for v in vs]


def _dot(a, b):
    return jnp.dot(a, b, preferred_element_type=F32)


def _shr(x, n):
    return x >> n if isinstance(x, int) else lax.shift_right_logical(x, n)


def _al(x, n):
    return x if isinstance(x, int) else pl.multiple_of(x, n)


def _u(x):
    return pltpu.bitcast(x, U32)


def _bf(x):
    return pltpu.bitcast(x, BF)


def _cat(xs, axis=1):
    return xs[0] if len(xs) == 1 else jnp.concatenate(xs, axis=axis)


def _unpk(x):
    return [pltpu.unpack_elementwise(x, index=k, packed_dtype=BF, unpacked_dtype=F32) for k in range(2)]


def _pk(lo, hi):
    return _u(pltpu.pack_elementwise([lo, hi], packed_dtype=BF))


def _lhs_sums(a11, a12, a21, a22):
    return [a11 + a22, a21 + a22, a11 + a12, a21 - a11, a12 - a22]


def _rhs_sums(b11, b12, b21, b22):
    return [b11 + b22, b12 - b22, b21 - b11, b11 + b12, b21 + b22]


def _packed_sums(fn, blocks):
    un = [_unpk(b) for b in blocks]
    lo = fn(*[u[0] for u in un])
    hi = fn(*[u[1] for u in un])
    return [_pk(a, b) for a, b in zip(lo, hi)]


LSUM = {1: 0, 2: 1, 5: 2, 6: 3, 7: 4}
RSUM = {1: 0, 3: 1, 4: 2, 6: 3, 7: 4}


def _combine(m):
    c11 = m[4] - m[5] + m[1] + m[7]
    c12 = m[3] + m[5]
    c21 = m[2] + m[4]
    c22 = m[3] - m[2] + m[1] + m[6]
    return c11, c12, c21, c22


def _ticker(prods, zv, n, lo, hi):
    slots = []
    for pr in prods:
        for t in range(pr.shape[1] // 128):
            for r in range(0, pr.shape[0], 8):
                slots.append((pr, r, t))
    for k in range(n):
        pr, r, t = slots[min(int((lo + (hi - lo) * k / n) * len(slots)), len(slots) - 1)]
        yield _u(pr[r:r + 8, t * 128:(t + 1) * 128]) & zv


def build(prof=False, pvw=1, qkw=1, qgate=8, lastsplit=2, sidehi=0.72, plo=0.0, wlo=0.3):
    tm2 = 256
    hm = tm2 // 2
    rb = 8
    FC = 512
    NFC = F // FC
    XB = 512
    n2 = S // tm2
    KD = F // 256
    SM, SX, SR, SOUT, NSEM = 0, 6, 6, 7, 9

    def kernel(x_hbm, gw_hbm, wqkv_hbm, wo_hbm, wg_hbm, wu_hbm, wd_hbm, o_hbm,
               x_v, xs, wqk, wv7, wo7, wd7, hs, g_s, sems):

        def x_raw(i, half, kh):
            return x_v[pl.ds(_al(i * tm2 + half * hm, hm), hm), kh * 512:(kh + 1) * 512]

        def phase1(wqkv_v, wo_v, wo_f32, wg0, wu0, wg_v, wu_v, bs, wd_v, h0, gw_ref):
            def cp_x(r0, n, s):
                return pltpu.make_async_copy(x_hbm.at[pl.ds(r0, n)], x_v.at[pl.ds(r0, n)], sems.at[s])

            def cp_w0(t, s):
                c = pl.ds(_al(t * 128, 128), 128)
                return [pltpu.make_async_copy(wg_hbm.at[:, c], wg0.at[t], sems.at[s]),
                        pltpu.make_async_copy(wu_hbm.at[:, c], wu0.at[t], sems.at[s])]

            def cp_w(j):
                c = pl.ds(_al(j * FC, FC), FC)
                return [pltpu.make_async_copy(wg_hbm.at[:, c], wg_v.at[j - 1], sems.at[SM + j - 1]),
                        pltpu.make_async_copy(wu_hbm.at[:, c], wu_v.at[j - 1], sems.at[SM + j - 1])]

            QH = 96

            def cp_q(r0, n, s):
                return [pltpu.make_async_copy(wqkv_hbm.at[kh * 512 + r0:kh * 512 + r0 + n],
                                              wqkv_v.at[kh * 512 + r0:kh * 512 + r0 + n], sems.at[s])
                        for kh in range(2)]

            cp_head = cp_q(0, QH, SM) + [
                pltpu.make_async_copy(wo_hbm, wo_v, sems.at[SM]),
                pltpu.make_async_copy(wd_hbm.at[0:2 * FC], wd_v.at[0:2 * FC], sems.at[SM]),
                pltpu.make_async_copy(gw_hbm, gw_ref.at[pl.ds(0, D)], sems.at[SM])]
            cp_rest = cp_q(QH, 512 - QH, SR) + [
                pltpu.make_async_copy(wd_hbm.at[2 * FC:F], wd_v.at[2 * FC:F], sems.at[SR])]

            first = [cp_w0(0, 1) + [cp_x(0, 256, 1)], [cp_x(256, 256, 2)]]
            starts = sum(first, [])
            for t in range(1, 4):
                starts += cp_w0(t, 2 + t)
            starts += [cp_x(b * XB, XB, SX + b - 1) for b in range(1, 4)]
            starts += cp_w(1) + cp_head
            for c in starts:
                c.start()

            def zeros_of(i):
                zi = _shr(i, 20)
                return zi, jnp.full((8, 128), zi, I32).astype(U32)

            def ffn_plain(r0, nr, t):
                xx = x_v[pl.ds(r0, nr), :]
                gt = _dot(xx, wg0[t])
                up = _dot(xx, wu0[t])
                h0[t, pl.ds(r0, nr), :] = (jnp.maximum(gt, 0.0) * up).astype(BF)
                return [gt, up]

            def x_sums(u0, nu, tick):
                xsrc = x_v.at[pl.ds(_al(u0 * tm2, tm2), nu * tm2)]
                xdst = xs.at[:, pl.ds(_al(u0 * 64, 64), nu * 64)]
                for u in range(nu):
                    for r in range(0, hm, 16):
                        for t in range(4):
                            dep = next(tick)
                            blk = [_u(xsrc[u * tm2 + hf * hm + r:u * tm2 + hf * hm + r + 16,
                                           kh * 512 + t * 128:kh * 512 + (t + 1) * 128]) | dep
                                   for hf in range(2) for kh in range(2)]
                            sm = _packed_sums(_lhs_sums, blk)
                            for k in range(5):
                                xdst[k * 4 + t, u * 64 + r // 2:u * 64 + r // 2 + 8, :] = sm[k]

            def w_sums(tile, mi, t, tick):
                for r in range(0, 512, 16):
                    dep = next(tick)
                    blk = [_u(tile(nh, kh * 512 + r)) | dep for kh in range(2) for nh in range(2)]
                    sm = _packed_sums(_rhs_sums, blk)
                    for k in range(5):
                        bs[(mi * 5 + k) * 2 + t, r // 2:r // 2 + 8, :] = sm[k]

            def store_h7(mm, hdst):
                hb = [jnp.maximum(gt, 0.0) * up for gt, up in zip(_combine(mm[0]), _combine(mm[1]))]
                sm = _lhs_sums(*hb)
                h7 = {3: hb[0], 4: hb[3]}
                for k, n in LSUM.items():
                    h7[k] = sm[n]
                for k in range(1, 8):
                    hv = h7[k].astype(BF)
                    for t in range(2):
                        hdst[k - 1, t] = hv[:, t * 128:(t + 1) * 128]

            def warm0(u, carry):
                for k in range(2):
                    @pl.when(u == k)
                    def _():
                        for c in first[k]:
                            c.wait()
                pr = ffn_plain(_al(u * 256, 256), 256, 0)
                x_sums(u, 1, _ticker(pr, zeros_of(u)[1], 32, 0.0, 0.8))
                return carry
            lax.fori_loop(0, 2, scoped(warm0, 'warm0', prof), 0)

            def warm1(t, carry):
                for c in cp_w0(t, 2 + t):
                    c.wait()
                pr = ffn_plain(0, XB, t)
                tick = _ticker(pr, zeros_of(t)[1], 64, 0.0, 0.9)
                pi = _shr(t - 1, 1)
                for mi, w0 in enumerate((wg0, wu0)):
                    wp = w0.at[pl.ds(2 * pi, 2)]
                    w_sums(lambda nh, r: wp[nh, r:r + 16, :], mi, pi, tick)
                return carry
            lax.fori_loop(1, 4, scoped(warm1, 'warm1', prof), 0)
            for c in cp_w(2):
                c.start()

            def warm2(b, carry):
                cp_x(_al(b * XB, XB), XB, SX + b - 1).wait()
                zb, zv = zeros_of(b)
                xsb = xs.at[:, pl.ds(_al(b * 128, 128), 128)]

                def lhs(k):
                    if k == 3:
                        return _cat([x_raw(2 * b + u, 0, 0) for u in range(2)], axis=0)
                    if k == 4:
                        return _cat([x_raw(2 * b + u, 1, 1) for u in range(2)], axis=0)
                    return _cat([_bf(xsb[LSUM[k] * 4 + t]) for t in range(4)])

                def rhs(mi, k):
                    w0 = (wg0, wu0)[mi]
                    if k == 2:
                        return _cat([w0[2 * t, 0:512, :] for t in range(2)])
                    if k == 5:
                        return _cat([w0[2 * t + 1, 512:1024, :] for t in range(2)])
                    return _cat([_bf(bs[(mi * 5 + RSUM[k]) * 2 + t]) for t in range(2)])

                mm = [{}, {}]
                prods = []
                for k in (3, 4):
                    for mi in range(2):
                        mm[mi][k] = _dot(lhs(k), rhs(mi, k))
                        prods.append(mm[mi][k])
                x_sums(2 * b, 2, _ticker(prods, zv, 64, 0.0, 0.85))
                prods = []
                for k in (2, 5, 1, 7, 6):
                    for mi in range(2):
                        mm[mi][k] = _dot(lhs(k), rhs(mi, k))
                        prods.append(mm[mi][k])
                tick = _ticker(prods, zv, 32, 0.0, 0.6)
                for u in range(2):
                    for r in range(0, hm, 16):
                        for t in range(2):
                            dep = next(tick)
                            blk = [_u(h0[2 * t + kh, u * tm2 + hf * hm + r:u * tm2 + hf * hm + r + 16, :]) | dep
                                   for hf in range(2) for kh in range(2)]
                            sm = _packed_sums(_lhs_sums, blk)
                            o7 = {3: blk[0], 4: blk[3]}
                            for k, n in LSUM.items():
                                o7[k] = sm[n]
                            for k in range(1, 8):
                                hs[k - 1, t, u * hm + r:u * hm + r + 16, :] = _bf(o7[k])
                store_h7(mm, hs.at[:, 0:2, pl.ds(_al(b * 256, 256), 256)])
                return carry
            lax.fori_loop(1, 4, scoped(warm2, 'warm2', prof), 0)

            for c in cp_rest:
                c.start()
            for j in range(3, NFC):
                for c in cp_w(j):
                    c.start()
            for c in cp_head:
                c.wait()

            def main1(j, carry):
                @pl.when(j == 2)
                def _():
                    for c in cp_rest:
                        c.wait()
                for c in cp_w(j):
                    c.wait()

                zj, zv = zeros_of(j)
                p = j - 1
                wsrc = [wg_v.at[p], wu_v.at[p]]

                def lhs(k):
                    if k == 3:
                        return _cat([x_raw(i, 0, 0) for i in range(n2)], axis=0)
                    if k == 4:
                        return _cat([x_raw(i, 1, 1) for i in range(n2)], axis=0)
                    return _cat([_bf(xs[LSUM[k] * 4 + t]) for t in range(4)])

                def rhs(mi, k):
                    if k == 2:
                        return _cat([wsrc[mi][0:512, 2 * t * 128:(2 * t + 1) * 128] for t in range(2)])
                    if k == 5:
                        return _cat([wsrc[mi][512:1024, (2 * t + 1) * 128:(2 * t + 2) * 128] for t in range(2)])
                    return _cat([_bf(bs[zj + (mi * 5 + RSUM[k]) * 2 + t]) for t in range(2)])

                mm = [{}, {}]
                prods = []
                for mi, k in [(0, 2), (0, 5), (1, 2), (1, 5)]:
                    mm[mi][k] = _dot(lhs(k), rhs(mi, k))
                    prods.append(mm[mi][k])
                tick = _ticker(prods, zv, 128, 0.0, 0.95)
                for mi in range(2):
                    for t in range(2):
                        w_sums(lambda nh, r: wsrc[mi][r:r + 16, (2 * t + nh) * 128:(2 * t + nh + 1) * 128], mi, t, tick)
                for k in (4, 3, 1, 7, 6):
                    for mi in range(2):
                        mm[mi][k] = _dot(lhs(k), rhs(mi, k))
                        prods.append(mm[mi][k])
                store_h7(mm, hs.at[:, pl.ds(2 * j, 2)])

                tick = _ticker(prods, zv, 80, wlo, sidehi)
                q0 = jnp.minimum(5 * p, 23)
                for e in range(5):
                    qq = q0 + e
                    ch = _shr(qq, 2)
                    sub = qq & 3
                    rsrc = ch * FC + _shr(sub, 1) * 256 + (sub & 1) * 64
                    dsrc = [wd_v.at[pl.ds(_al(rsrc + kh * 128, 64), 64)] for kh in range(2)]
                    ddst = wd7.at[:, pl.ds(_al(qq * 32, 32), 32)]
                    for r in range(0, 64, 16):
                        for t in range(4):
                            dep = next(tick)
                            blk = [_u(dsrc[kh][r:r + 16, nh * 512 + t * 128:nh * 512 + (t + 1) * 128]) | dep
                                   for kh in range(2) for nh in range(2)]
                            sm = _packed_sums(_rhs_sums, blk)
                            o7 = {2: blk[0], 5: blk[3]}
                            for k, n in RSUM.items():
                                o7[k] = sm[n]
                            for k in range(1, 8):
                                ddst[(k - 1) * 4 + t, r // 2:r // 2 + 8, :] = o7[k]

                tick = _ticker(prods, zv, 44, wlo + 0.003, sidehi)
                gr = _al(jnp.minimum(p * 352, S - 352), 32)
                xg = x_v.at[pl.ds(gr, 352)]
                gdst = g_s.at[pl.ds(gr, 352)]
                gw = gw_ref[pl.ds(0, D)].astype(F32).reshape(1, D)
                for r in range(0, 352, 8):
                    dep = next(tick)
                    xf = xg[r:r + 8, :].astype(F32)
                    xf = [pltpu.bitcast(_u(xf[:, c * 128:(c + 1) * 128]) | dep, F32) for c in range(8)]
                    zg = xf[0] * gw[:, 0:128]
                    for c in range(1, 8):
                        zg = zg + xf[c] * gw[:, c * 128:(c + 1) * 128]
                    gdst[r:r + 8, :] = jax.nn.sigmoid(
                        jnp.broadcast_to(jnp.sum(zg, axis=-1, keepdims=True), (8, 128)))

                lane = lax.broadcasted_iota(I32, (8, 128), 1)
                qr = _al(jnp.minimum(p * QH, 512 - QH), 16)
                qsrc = [wqkv_v.at[pl.ds(kh * 512 + qr, QH)] for kh in range(2)]
                qw = _al(_shr(qr, 1), 8)
                qdst = [wqk.at[:, pl.ds(kh * 256 + qw, QH // 2)] for kh in range(2)]
                vdst = wv7.at[:, pl.ds(qw, QH // 2)]
                tick = _ticker(prods, zv, 36, plo, sidehi - 0.04)
                tick2 = _ticker(prods, zv, 36 * 2, plo + 0.04, sidehi + 0.01)
                for r in range(0, QH, 16):
                    pv = []
                    for m in (2, 0, 1):
                        for kh in range(2):
                            dep = next(tick)
                            vs = _permute_cols([_u(qsrc[kh][r:r + 16, m * D + c * 128:m * D + (c + 1) * 128]) | dep
                                                for c in range(8)], lane)
                            if m == 2:
                                pv.append(vs)
                            else:
                                for c in range(8):
                                    qdst[kh][m * 8 + c, r // 2:r // 2 + 8, :] = vs[c]
                    for t in range(4):
                        for _ in range(3):
                            dep = next(tick2)
                        blk = [v | dep for v in (pv[0][t], pv[0][t + 4], pv[1][t], pv[1][t + 4])]
                        sm = _packed_sums(_rhs_sums, blk)
                        o7 = {2: blk[0], 5: blk[3]}
                        for k, n in RSUM.items():
                            o7[k] = sm[n]
                        for k in range(1, 8):
                            vdst[(k - 1) * 4 + t, r // 2:r // 2 + 8, :] = o7[k]

                pb = jnp.minimum(p, 3)
                osrc = [wo_v.at[:, pl.ds(_al((pb + 4 * t) * 128, 128), 128)] for t in range(2)]
                tick = _ticker(prods, zv, 64, 0.002, wlo)
                for hh in range(H):
                    for t in range(2):
                        dep = next(tick)
                        for q in range(2):
                            wo_f32[t, hh * 33 + q * 16:hh * 33 + (q + 1) * 16, :] = _bf(
                                _u(osrc[t][hh * 32 + q * 16:hh * 32 + (q + 1) * 16, :]) | dep).astype(F32)
                tick = _ticker(prods, zv, 32, wlo + 0.01, sidehi)
                for b in range(4):
                    for a in range(4):
                        for q in range(2):
                            dep = next(tick)
                            blk = [_cat([pltpu.bitcast(_u(wo_f32[
                                t, pl.ds(a * 8 + b + 4 * kh + (q * 16 + e * 8) * 33, 8, stride=33), :]) | dep, F32)
                                for e in range(2)], axis=0) for kh in range(2) for t in range(2)]
                            sm = _rhs_sums(*blk)
                            o7 = {2: blk[0], 5: blk[3]}
                            for k, n in RSUM.items():
                                o7[k] = sm[n]
                            r = (b * 128 + a * 32 + q * 16) // 2
                            for k in range(1, 8):
                                wo7[(k - 1) * 4 + pb, r:r + 8, :] = _u(o7[k].astype(BF))
                return carry
            lax.fori_loop(1, NFC, scoped(main1, 'main1', prof), 0)

        def phase2(q_s, k_s, v_s, oa_v, oas, out_v):
            k_s[:, 0:HALO, :] = jnp.zeros((8, HALO, 128), F32)
            v_s[:, 0:HALO, :] = jnp.zeros((8, HALO, 128), F32)
            cexp = SCALE * LOG2E

            def main2(i, carry):
                r0 = _al(i * tm2, tm2)
                xsb = xs.at[:, pl.ds(_al(i * 64, 64), 64)]

                def lhs_x(k):
                    if k == 3:
                        return x_raw(i, 0, 0)
                    if k == 4:
                        return x_raw(i, 1, 1)
                    return _cat([_bf(xsb[LSUM[k] * 4 + t]) for t in range(4)])

                for m in range(3):
                    if m < 2:
                        full = _dot(x_v[pl.ds(r0, tm2), :], _cat([_bf(wqk[m * 8 + c]) for c in range(8)]))
                        cbs = [full[hf * hm:(hf + 1) * hm, nh * 512:(nh + 1) * 512] for hf in range(2) for nh in range(2)]
                    else:
                        cbs = _combine({k: _dot(lhs_x(k), _cat([_bf(wv7[(k - 1) * 4 + t]) for t in range(4)]))
                                        for k in (2, 4, 3, 5, 1, 7, 6)})
                    for n, cb in enumerate(cbs):
                        for t in range(4):
                            val = cb[:, t * 128:(t + 1) * 128]
                            c = (n % 2) * 4 + t
                            ro = (n // 2) * hm
                            if m == 0:
                                q_s[c, ro:ro + hm, :] = val
                            else:
                                (k_s, v_s)[m - 1][c, pl.ds(r0 + HALO + ro, hm), :] = val
                zs = [_shr(i, 20), _shr(i, 21)]
                kzs = [r0 + zz for zz in zs]
                zv = jnp.full((rb, 128), zs[0], I32)
                gb = g_s.at[pl.ds(r0, tm2)]

                def gate(t, dep):
                    return pltpu.bitcast(pltpu.bitcast(t, I32) | dep, F32)

                def after(t, dep):
                    return gate(t, pltpu.bitcast(dep, I32) & zv)
                den = None
                outs = []
                raws = []
                pend = [None] * 8
                for gi, r in enumerate(range(0, tm2, rb)):
                    z = zs[gi % 2]
                    kz = kzs[gi % 2]
                    q = [q_s[c, pl.ds(z + r, rb), :] for c in range(8)]
                    if gi >= 1:
                        dep = pltpu.bitcast(den, I32) & zv
                        q = [gate(t, dep) if c < qgate else t for c, t in enumerate(q)]
                    g = gb[r:r + rb, :]
                    s = []
                    for w in range(W):
                        st = HALO + r - DIL * w
                        q0 = q[0] if w < qkw else after(q[0], raws[-qkw])
                        acc = q0 * k_s[0, pl.ds(kz + st, rb), :]
                        for c in range(1, 8):
                            acc = acc + q[c] * k_s[c, pl.ds(kz + st, rb), :]
                        raws.append(acc)
                        acc = acc + pltpu.roll(acc, 64, 1)
                        acc = acc + pltpu.roll(acc, 32, 1)
                        if r < HALO and w > 0:
                            pos = i * tm2 + r + lax.broadcasted_iota(I32, (rb, 128), 0)
                            acc = jnp.where(pos >= DIL * w, acc, -1e9 / SCALE)
                        s.append(acc)
                    mx = s[0]
                    for w in range(1, W):
                        mx = jnp.maximum(mx, s[w])
                    e = [jnp.exp2((s[w] - mx) * cexp) for w in range(W)]
                    den = e[0]
                    for w in range(1, W):
                        den = den + e[w]
                    inv = g / den
                    pks = []
                    for c in range(8):
                        st = HALO + r
                        e0 = e[0] if len(outs) < pvw else after(e[0], outs[-pvw])
                        acc = e0 * v_s[c, pl.ds(kz + st, rb), :]
                        for w in range(1, W):
                            st = HALO + r - DIL * w
                            acc = acc + e[w] * v_s[c, pl.ds(kz + st, rb), :]
                        outs.append(acc)
                        acc = acc * inv
                        if gi % 2 == 0:
                            pend[c] = acc
                        else:
                            pks.append(_u(_cat([pend[c], acc], axis=0).astype(BF)))
                    if gi % 2 == 1:
                        w0 = (r - rb) // 2
                        if r < hm:
                            for c in range(8):
                                oa_v[c, w0:w0 + 8, :] = pks[c]
                        else:
                            w1 = w0 - 64
                            for t in range(4):
                                oa_v[t + 4, w0:w0 + 8, :] = pks[t + 4]
                                blk = [oa_v[t, w1:w1 + 8, :], oa_v[t + 4, w1:w1 + 8, :], pks[t], pks[t + 4]]
                                sm = _packed_sums(_lhs_sums, blk)
                                for k in range(5):
                                    oas[k * 4 + t, w1:w1 + 8, :] = sm[k]

                hsb = hs.at[:, :, pl.ds(_al(i * hm, hm), hm)]
                mm = {k: _dot(_cat([hsb[k - 1, t] for t in range(KD)]),
                              _cat([_bf(wd7[(k - 1) * 4 + t]) for t in range(4)]))
                      for k in (2, 4, 3, 5, 1, 7, 6)}
                bb = _combine(mm)

                def lhs_o(k):
                    if k == 3:
                        return _cat([_bf(oa_v[t, 0:64, :]) for t in range(4)])
                    if k == 4:
                        return _cat([_bf(oa_v[t + 4, 64:128, :]) for t in range(4)])
                    return _cat([_bf(oas[LSUM[k] * 4 + t]) for t in range(4)])

                mm = {k: _dot(lhs_o(k), _cat([_bf(wo7[(k - 1) * 4 + t]) for t in range(4)]))
                      for k in (3, 4, 2, 5, 1, 7, 6)}
                omg = 1.0 - gb[...]
                ob = [_cat([omg[(n // 2) * hm:(n // 2 + 1) * hm]] * 4) * bb[n] for n in range(4)]
                fin = {2: (ob[2] + mm[4]) + mm[2],
                       1: (ob[1] + mm[3]) + mm[5],
                       0: (ob[0] + mm[4] - mm[5] + mm[1]) + mm[7],
                       3: (ob[3] + mm[3] - mm[2] + mm[1]) + mm[6]}
                for n in (2, 1, 0, 3):
                    ro = (n // 2) * hm
                    co = (n % 2) * 512
                    if n != 3:
                        pieces = [(0, hm, 0, 512)]
                    else:
                        nr = hm // lastsplit
                        pieces = [(0, hm, 0, 256), (0, hm, 256, 128)] + [(k * nr, nr, 384, 128) for k in range(lastsplit)]
                    for (pr, pn, pc, pw) in pieces:
                        rs = pl.ds(_al(r0 + ro + pr, pn), pn)
                        cs = slice(co + pc, co + pc + pw)
                        out_v[rs, cs] = fin[n][pr:pr + pn, pc:pc + pw].astype(BF)
                        pltpu.make_async_copy(out_v.at[rs, cs], o_hbm.at[rs, cs], sems.at[SOUT]).start()
                return carry
            lax.fori_loop(0, n2, scoped(main2, 'main2', prof), 0)
            pltpu.make_async_copy(out_v, o_hbm, sems.at[SOUT]).wait()

        @pl.when(pl.program_id(0) == 0)
        def _():
            pl.run_scoped(
                phase1,
                pltpu.VMEM((D, 3 * D), BF),
                pltpu.VMEM((D, D), BF),
                pltpu.VMEM((2, 1088, 128), F32),
                pltpu.VMEM((4, D, 128), BF),
                pltpu.VMEM((4, D, 128), BF),
                pltpu.VMEM((NFC - 1, D, FC), BF),
                pltpu.VMEM((NFC - 1, D, FC), BF),
                pltpu.VMEM((20, 256, 128), U32),
                pltpu.VMEM((F, D), BF),
                pltpu.VMEM((4, XB, 128), BF),
                pltpu.VMEM((8 * D,), BF),
            )

        @pl.when(pl.program_id(0) == 1)
        def _():
            pl.run_scoped(
                phase2,
                pltpu.VMEM((8, tm2, 128), F32),
                pltpu.VMEM((8, S + HALO, 128), F32),
                pltpu.VMEM((8, S + HALO, 128), F32),
                pltpu.VMEM((8, 128, 128), U32),
                pltpu.VMEM((20, 64, 128), U32),
                pltpu.VMEM((S, D), BF),
            )

    @jax.jit
    def f(A_x, A_wqkv, A_wo, B_x, B_W_gate, B_W_up, B_W_down, gate_w):
        x = A_x.reshape(S, D)
        anyspec = pl.BlockSpec(memory_space=pl.ANY)
        out = pl.pallas_call(
            kernel,
            grid=(2,),
            in_specs=[anyspec] * 7,
            out_specs=anyspec,
            out_shape=jax.ShapeDtypeStruct((S, D), BF),
            scratch_shapes=[
                pltpu.VMEM((S, D), BF),
                pltpu.VMEM((20, 512, 128), U32),
                pltpu.VMEM((16, 512, 128), U32),
                pltpu.VMEM((28, 256, 128), U32),
                pltpu.VMEM((28, 256, 128), U32),
                pltpu.VMEM((28, F // 4, 128), U32),
                pltpu.VMEM((7, KD, S // 2, 128), BF),
                pltpu.VMEM((S, 128), F32),
                pltpu.SemaphoreType.DMA((NSEM,)),
            ],
            compiler_params=pltpu.CompilerParams(
                vmem_limit_bytes=120 * 1024 * 1024, disable_bounds_checks=True, disable_semaphore_checks=True,
                dimension_semantics=('arbitrary',)),
        )(x, gate_w, A_wqkv, A_wo, B_W_gate, B_W_up, B_W_down)
        return out.reshape(1, S, D)
    return f


_impl = build()


@jax.jit
def pallas_gated_mix__sliding_local_dilated__glu_gated_reglu__prompt_kernel(
    A_x: jax.Array,
    A_wqkv: jax.Array,
    A_wo: jax.Array,
    B_x: jax.Array,
    B_W_gate: jax.Array,
    B_W_up: jax.Array,
    B_W_down: jax.Array,
    gate_w: jax.Array,
):
    return _impl(A_x, A_wqkv, A_wo, B_x, B_W_gate, B_W_up, B_W_down, gate_w)
```

```python
import jax
import jax.numpy as jnp
from jax import lax
import jax.experimental.pallas as pl
import jax.experimental.pallas.tpu as pltpu

S, D, F = 2048, 1024, 3584
H, DH, W, DIL = 32, 32, 8, 2
HALO = 16
LOG2E = 1.4426950408889634
SCALE = DH ** -0.5
BF = jnp.bfloat16
F32 = jnp.float32
U32 = jnp.uint32
I32 = jnp.int32

TM = 256
HM = TM // 2
RB = 8
FC = 512
NFC = F // FC
NB = S // TM
KD = F // 256
NU2 = 3
QH = 96
SM, SX, SR, SOUT, NSEM = 0, 6, 6, 7, 8


def _swap(vs, bit, lane):
    out = list(vs)
    sh = 1 << bit
    hi = (lane & sh) != 0
    for i in range(8):
        if i & sh:
            continue
        a, b = vs[i], vs[i | sh]
        out[i] = jnp.where(hi, pltpu.roll(b, sh, 1), a)
        out[i | sh] = jnp.where(hi, b, pltpu.roll(a, 128 - sh, 1))
    return out


def _permute_cols(vs, lane):
    for bit in range(3):
        vs = _swap(vs, bit, lane)
    idx = ((lane & 3) << 5) | ((lane >> 5) << 3) | ((lane >> 2) & 7)
    return [jnp.take_along_axis(v, idx, axis=1) for v in vs]


def _dot(a, b):
    return jnp.dot(a, b, preferred_element_type=F32)


def _shr(x, n):
    return x >> n if isinstance(x, int) else lax.shift_right_logical(x, n)


def _al(x, n):
    return x if isinstance(x, int) else pl.multiple_of(x, n)


def _u(x):
    return pltpu.bitcast(x, U32)


def _bf(x):
    return pltpu.bitcast(x, BF)


def _cat(xs, axis=1):
    return xs[0] if len(xs) == 1 else jnp.concatenate(xs, axis=axis)


def _lhs_sums(a11, a12, a21, a22):
    return [a11 + a22, a21 + a22, a11 + a12, a21 - a11, a12 - a22]


def _rhs_sums(b11, b12, b21, b22):
    return [b11 + b22, b12 - b22, b21 - b11, b11 + b12, b21 + b22]


LSUM = {1: 0, 2: 1, 5: 2, 6: 3, 7: 4}
RSUM = {1: 0, 3: 1, 4: 2, 6: 3, 7: 4}


def _packed_sums(fn, blocks):
    un = [[pltpu.unpack_elementwise(b, index=k, packed_dtype=BF, unpacked_dtype=F32) for k in range(2)]
          for b in blocks]
    lo = fn(*[u[0] for u in un])
    hi = fn(*[u[1] for u in un])
    return [_u(pltpu.pack_elementwise([a, b], packed_dtype=BF)) for a, b in zip(lo, hi)]


def _lhs7(blocks, sums):
    o = {3: blocks[0], 4: blocks[3]}
    o.update({k: sums[n] for k, n in LSUM.items()})
    return o


def _rhs7(blocks, sums):
    o = {2: blocks[0], 5: blocks[3]}
    o.update({k: sums[n] for k, n in RSUM.items()})
    return o


def _combine(m):
    c11 = m[4] - m[5] + m[1] + m[7]
    c12 = m[3] + m[5]
    c21 = m[2] + m[4]
    c22 = m[3] - m[2] + m[1] + m[6]
    return c11, c12, c21, c22


def _ticker(prods, zv, n, lo, hi):
    slots = []
    for pr in prods:
        for t in range(pr.shape[1] // 128):
            for r in range(0, pr.shape[0], 8):
                slots.append((pr, r, t))
    for k in range(n):
        pr, r, t = slots[min(int((lo + (hi - lo) * k / n) * len(slots)), len(slots) - 1)]
        yield _u(pr[r:r + 8, t * 128:(t + 1) * 128]) & zv


def _kernel(x_hbm, gw_hbm, wqkv_hbm, wo_hbm, wg_hbm, wu_hbm, wd_hbm, o_hbm,
            x_v, xs, wqk, wv7, wo7, wd7, hs, g_s, sems):

    def x_raw(i, half, kh):
        return x_v[pl.ds(_al(i * TM + half * HM, HM), HM), kh * 512:(kh + 1) * 512]

    def phase1(wqkv_v, wo_v, wo_f32, wg0, wu0, wg_v, wu_v, bs, wd_v, h0, gw_ref):
        def cp_x(r0, n, s):
            return pltpu.make_async_copy(x_hbm.at[pl.ds(r0, n)], x_v.at[pl.ds(r0, n)], sems.at[s])

        def cp_w0(t, s):
            c = pl.ds(_al(t * 128, 128), 128)
            return [pltpu.make_async_copy(wg_hbm.at[:, c], wg0.at[t], sems.at[s]),
                    pltpu.make_async_copy(wu_hbm.at[:, c], wu0.at[t], sems.at[s])]

        def cp_w(j):
            c = pl.ds(_al(j * FC, FC), FC)
            return [pltpu.make_async_copy(wg_hbm.at[:, c], wg_v.at[j - 1], sems.at[SM + j - 1]),
                    pltpu.make_async_copy(wu_hbm.at[:, c], wu_v.at[j - 1], sems.at[SM + j - 1])]

        def cp_q(r0, n, s):
            return [pltpu.make_async_copy(wqkv_hbm.at[kh * 512 + r0:kh * 512 + r0 + n],
                                          wqkv_v.at[kh * 512 + r0:kh * 512 + r0 + n], sems.at[s])
                    for kh in range(2)]

        cp_head = cp_q(0, QH, SM) + [
            pltpu.make_async_copy(wo_hbm, wo_v, sems.at[SM]),
            pltpu.make_async_copy(wd_hbm.at[0:2 * FC], wd_v.at[0:2 * FC], sems.at[SM]),
            pltpu.make_async_copy(gw_hbm, gw_ref.at[pl.ds(0, D)], sems.at[SM])]
        cp_rest = cp_q(QH, 512 - QH, SR) + [
            pltpu.make_async_copy(wd_hbm.at[2 * FC:F], wd_v.at[2 * FC:F], sems.at[SR])]

        first = [cp_w0(0, 1) + [cp_x(0, TM, 1)], [cp_x(TM, TM, 2)]]
        starts = sum(first, [])
        for t in range(1, 4):
            starts += cp_w0(t, 2 + t)
        starts += [cp_x((2 + b * NU2) * TM, NU2 * TM, SX + b) for b in range(6 // NU2)]
        starts += cp_w(1) + cp_head
        for c in starts:
            c.start()
        for t in range(2):
            for hh in range(H):
                wo_f32[t, hh * 33 + 32:hh * 33 + 33, :] = jnp.zeros((1, 128), F32)

        def zeros_of(i):
            zi = _shr(i, 20)
            return zi, jnp.full((8, 128), zi, I32).astype(U32)

        def ffn_plain(r0, nr, t):
            xx = x_v[pl.ds(r0, nr), :]
            gt = _dot(xx, wg0[t])
            up = _dot(xx, wu0[t])
            h0[t, pl.ds(r0, nr), :] = (jnp.maximum(gt, 0.0) * up).astype(BF)
            return [gt, up]

        def x_sums(u0, nu, tick):
            xsrc = x_v.at[pl.ds(_al(u0 * TM, TM), nu * TM)]
            xdst = xs.at[:, pl.ds(_al(u0 * 64, 64), nu * 64)]
            for u in range(nu):
                for r in range(0, HM, 16):
                    for t in range(4):
                        dep = next(tick)
                        blk = [_u(xsrc[u * TM + hf * HM + r:u * TM + hf * HM + r + 16,
                                       kh * 512 + t * 128:kh * 512 + (t + 1) * 128]) | dep
                               for hf in range(2) for kh in range(2)]
                        sm = _packed_sums(_lhs_sums, blk)
                        for k in range(5):
                            xdst[k * 4 + t, u * 64 + r // 2:u * 64 + r // 2 + 8, :] = sm[k]

        def w_sums(tile, mi, t, tick):
            for r in range(0, 512, 16):
                dep = next(tick)
                blk = [_u(tile(nh, kh * 512 + r)) | dep for kh in range(2) for nh in range(2)]
                sm = _packed_sums(_rhs_sums, blk)
                for k in range(5):
                    bs[(mi * 5 + k) * 2 + t, r // 2:r // 2 + 8, :] = sm[k]

        def store_h7(mm, hdst):
            hb = [jnp.maximum(gt, 0.0) * up for gt, up in zip(_combine(mm[0]), _combine(mm[1]))]
            h7 = _lhs7(hb, _lhs_sums(*hb))
            for k in range(1, 8):
                hv = h7[k].astype(BF)
                for t in range(2):
                    hdst[k - 1, t] = hv[:, t * 128:(t + 1) * 128]

        def warm0(u, carry):
            for k in range(2):
                @pl.when(u == k)
                def _():
                    for c in first[k]:
                        c.wait()
            pr = ffn_plain(_al(u * TM, TM), TM, 0)
            x_sums(u, 1, _ticker(pr, zeros_of(u)[1], 32, 0.0, 0.8))
            return carry
        lax.fori_loop(0, 2, warm0, 0)

        def warm1(t, carry):
            for c in cp_w0(t, 2 + t):
                c.wait()
            pr = ffn_plain(0, 2 * TM, t)
            tick = _ticker(pr, zeros_of(t)[1], 64, 0.0, 0.9)
            pi = _shr(t - 1, 1)
            for mi, w0 in enumerate((wg0, wu0)):
                wp = w0.at[pl.ds(2 * pi, 2)]
                w_sums(lambda nh, r: wp[nh, r:r + 16, :], mi, pi, tick)
            return carry
        lax.fori_loop(1, 4, warm1, 0)
        for c in cp_w(2):
            c.start()

        def warm2(b, carry):
            u0 = 2 + b * NU2
            cp_x(_al(u0 * TM, TM), NU2 * TM, SX + b).wait()
            zv = zeros_of(b)[1]
            xsb = xs.at[:, pl.ds(_al(u0 * 64, 64), NU2 * 64)]

            def lhs(k):
                if k == 3:
                    return _cat([x_raw(u0 + u, 0, 0) for u in range(NU2)], axis=0)
                if k == 4:
                    return _cat([x_raw(u0 + u, 1, 1) for u in range(NU2)], axis=0)
                return _cat([_bf(xsb[LSUM[k] * 4 + t]) for t in range(4)])

            def rhs(mi, k):
                w0 = (wg0, wu0)[mi]
                if k == 2:
                    return _cat([w0[2 * t, 0:512, :] for t in range(2)])
                if k == 5:
                    return _cat([w0[2 * t + 1, 512:1024, :] for t in range(2)])
                return _cat([_bf(bs[(mi * 5 + RSUM[k]) * 2 + t]) for t in range(2)])

            mm = [{}, {}]
            prods = []
            for k in (3, 4):
                for mi in range(2):
                    mm[mi][k] = _dot(lhs(k), rhs(mi, k))
                    prods.append(mm[mi][k])
            x_sums(u0, NU2, _ticker(prods, zv, 32 * NU2, 0.0, 0.85))
            prods = []
            for k in (2, 5, 1, 7, 6):
                for mi in range(2):
                    mm[mi][k] = _dot(lhs(k), rhs(mi, k))
                    prods.append(mm[mi][k])
            tick = _ticker(prods, zv, 32, 0.0, 0.6)
            for u in range(2):
                for r in range(0, HM, 16):
                    for t in range(2):
                        dep = next(tick)
                        blk = [_u(h0[2 * t + kh, u * TM + hf * HM + r:u * TM + hf * HM + r + 16, :]) | dep
                               for hf in range(2) for kh in range(2)]
                        o7 = _lhs7(blk, _packed_sums(_lhs_sums, blk))
                        for k in range(1, 8):
                            hs[k - 1, t, u * HM + r:u * HM + r + 16, :] = _bf(o7[k])
            store_h7(mm, hs.at[:, 0:2, pl.ds(_al(u0 * HM, HM), NU2 * HM)])
            return carry
        lax.fori_loop(0, 6 // NU2, warm2, 0)

        for c in cp_rest:
            c.start()
        for j in range(3, NFC):
            for c in cp_w(j):
                c.start()
        for c in cp_head:
            c.wait()

        def main1(j, carry):
            @pl.when(j == 2)
            def _():
                for c in cp_rest:
                    c.wait()
            for c in cp_w(j):
                c.wait()

            zj, zv = zeros_of(j)
            p = j - 1
            wsrc = [wg_v.at[p], wu_v.at[p]]

            def lhs(k):
                if k == 3:
                    return _cat([x_raw(i, 0, 0) for i in range(NB)], axis=0)
                if k == 4:
                    return _cat([x_raw(i, 1, 1) for i in range(NB)], axis=0)
                return _cat([_bf(xs[LSUM[k] * 4 + t]) for t in range(4)])

            def rhs(mi, k):
                if k == 2:
                    return _cat([wsrc[mi][0:512, 2 * t * 128:(2 * t + 1) * 128] for t in range(2)])
                if k == 5:
                    return _cat([wsrc[mi][512:1024, (2 * t + 1) * 128:(2 * t + 2) * 128] for t in range(2)])
                return _cat([_bf(bs[zj + (mi * 5 + RSUM[k]) * 2 + t]) for t in range(2)])

            mm = [{}, {}]
            prods = []
            for mi, k in [(0, 2), (0, 5), (1, 2), (1, 5)]:
                mm[mi][k] = _dot(lhs(k), rhs(mi, k))
                prods.append(mm[mi][k])
            tick = _ticker(prods, zv, 128, 0.0, 0.95)
            for mi in range(2):
                for t in range(2):
                    w_sums(lambda nh, r: wsrc[mi][r:r + 16, (2 * t + nh) * 128:(2 * t + nh + 1) * 128], mi, t, tick)
            for k in (4, 3, 1, 7, 6):
                for mi in range(2):
                    mm[mi][k] = _dot(lhs(k), rhs(mi, k))
                    prods.append(mm[mi][k])
            store_h7(mm, hs.at[:, pl.ds(2 * j, 2)])

            tick = _ticker(prods, zv, 80, 0.3, 0.72)
            q0 = jnp.minimum(5 * p, 23)
            for e in range(5):
                qq = q0 + e
                sub = qq & 3
                rsrc = _shr(qq, 2) * FC + _shr(sub, 1) * 256 + (sub & 1) * 64
                dsrc = [wd_v.at[pl.ds(_al(rsrc + kh * 128, 64), 64)] for kh in range(2)]
                ddst = wd7.at[:, pl.ds(_al(qq * 32, 32), 32)]
                for r in range(0, 64, 16):
                    for t in range(4):
                        dep = next(tick)
                        blk = [_u(dsrc[kh][r:r + 16, nh * 512 + t * 128:nh * 512 + (t + 1) * 128]) | dep
                               for kh in range(2) for nh in range(2)]
                        o7 = _rhs7(blk, _packed_sums(_rhs_sums, blk))
                        for k in range(1, 8):
                            ddst[(k - 1) * 4 + t, r // 2:r // 2 + 8, :] = o7[k]

            tick = _ticker(prods, zv, 44, 0.303, 0.72)
            gr = _al(jnp.minimum(p * 352, S - 352), 32)
            xg = x_v.at[pl.ds(gr, 352)]
            gdst = g_s.at[pl.ds(gr, 352)]
            gw = gw_ref[pl.ds(0, D)].astype(F32).reshape(1, D)
            for r in range(0, 352, 8):
                dep = next(tick)
                xf = xg[r:r + 8, :].astype(F32)
                xf = [pltpu.bitcast(_u(xf[:, c * 128:(c + 1) * 128]) | dep, F32) for c in range(8)]
                zg = xf[0] * gw[:, 0:128]
                for c in range(1, 8):
                    zg = zg + xf[c] * gw[:, c * 128:(c + 1) * 128]
                gdst[r:r + 8, :] = jax.nn.sigmoid(
                    jnp.broadcast_to(jnp.sum(zg, axis=-1, keepdims=True), (8, 128)))

            lane = lax.broadcasted_iota(I32, (8, 128), 1)
            qr = _al(jnp.minimum(p * QH, 512 - QH), 16)
            qsrc = [wqkv_v.at[pl.ds(kh * 512 + qr, QH)] for kh in range(2)]
            qw = _al(_shr(qr, 1), 8)
            qdst = [wqk.at[:, pl.ds(kh * 256 + qw, QH // 2)] for kh in range(2)]
            vdst = wv7.at[:, pl.ds(qw, QH // 2)]
            tick = _ticker(prods, zv, 36, 0.0, 0.72 - 0.04)
            tick2 = _ticker(prods, zv, 36 * 2, 0.04, 0.72 + 0.01)
            for r in range(0, QH, 16):
                pv = []
                for m in (2, 0, 1):
                    for kh in range(2):
                        dep = next(tick)
                        vs = _permute_cols([_u(qsrc[kh][r:r + 16, m * D + c * 128:m * D + (c + 1) * 128]) | dep
                                            for c in range(8)], lane)
                        if m == 2:
                            pv.append(vs)
                        else:
                            for c in range(8):
                                qdst[kh][m * 8 + c, r // 2:r // 2 + 8, :] = vs[c]
                for t in range(4):
                    for _ in range(3):
                        dep = next(tick2)
                    blk = [v | dep for v in (pv[0][t], pv[0][t + 4], pv[1][t], pv[1][t + 4])]
                    o7 = _rhs7(blk, _packed_sums(_rhs_sums, blk))
                    for k in range(1, 8):
                        vdst[(k - 1) * 4 + t, r // 2:r // 2 + 8, :] = o7[k]

            pb = jnp.minimum(p, 3)
            osrc = [wo_v.at[:, pl.ds(_al((pb + 4 * t) * 128, 128), 128)] for t in range(2)]
            tick = _ticker(prods, zv, 64, 0.002, 0.3)
            for hh in range(H):
                for t in range(2):
                    dep = next(tick)
                    for q in range(2):
                        wo_f32[t, hh * 33 + q * 16:hh * 33 + (q + 1) * 16, :] = _bf(
                            _u(osrc[t][hh * 32 + q * 16:hh * 32 + (q + 1) * 16, :]) | dep).astype(F32)
            tick = _ticker(prods, zv, 32, 0.31, 0.72)
            for b in range(4):
                for a in range(4):
                    for q in range(2):
                        dep = next(tick)
                        blk = [_cat([pltpu.bitcast(_u(wo_f32[
                            t, pl.ds(a * 8 + b + 4 * kh + (q * 16 + e * 8) * 33, 8, stride=33), :]) | dep, F32)
                            for e in range(2)], axis=0) for kh in range(2) for t in range(2)]
                        o7 = _rhs7(blk, _rhs_sums(*blk))
                        r = (b * 128 + a * 32 + q * 16) // 2
                        for k in range(1, 8):
                            wo7[(k - 1) * 4 + pb, r:r + 8, :] = _u(o7[k].astype(BF))
            return carry
        lax.fori_loop(1, NFC, main1, 0)

    def phase2(q_s, k_s, v_s, oa_v, oas, out_v):
        k_s[:, 0:HALO, :] = jnp.zeros((8, HALO, 128), F32)
        v_s[:, 0:HALO, :] = jnp.zeros((8, HALO, 128), F32)
        cexp = SCALE * LOG2E

        def main2(i, carry):
            r0 = _al(i * TM, TM)
            xsb = xs.at[:, pl.ds(_al(i * 64, 64), 64)]

            def lhs_x(k):
                if k == 3:
                    return x_raw(i, 0, 0)
                if k == 4:
                    return x_raw(i, 1, 1)
                return _cat([_bf(xsb[LSUM[k] * 4 + t]) for t in range(4)])

            for m in range(3):
                if m < 2:
                    full = _dot(x_v[pl.ds(r0, TM), :], _cat([_bf(wqk[m * 8 + c]) for c in range(8)]))
                    cbs = [full[hf * HM:(hf + 1) * HM, nh * 512:(nh + 1) * 512] for hf in range(2) for nh in range(2)]
                else:
                    cbs = _combine({k: _dot(lhs_x(k), _cat([_bf(wv7[(k - 1) * 4 + t]) for t in range(4)]))
                                    for k in (2, 4, 3, 5, 1, 7, 6)})
                for n, cb in enumerate(cbs):
                    for t in range(4):
                        val = cb[:, t * 128:(t + 1) * 128]
                        c = (n % 2) * 4 + t
                        ro = (n // 2) * HM
                        if m == 0:
                            q_s[c, ro:ro + HM, :] = val
                        else:
                            (k_s, v_s)[m - 1][c, pl.ds(r0 + HALO + ro, HM), :] = val

            zs = [_shr(i, 20), _shr(i, 21)]
            kzs = [r0 + zz for zz in zs]
            zv = jnp.full((RB, 128), zs[0], I32)
            gb = g_s.at[pl.ds(r0, TM)]

            def gate(t, dep):
                return pltpu.bitcast(pltpu.bitcast(t, I32) | dep, F32)

            def after(t, dep):
                return gate(t, pltpu.bitcast(dep, I32) & zv)
            den = None
            last_o = None
            pend = [None] * 8
            for gi, r in enumerate(range(0, TM, RB)):
                z = zs[gi % 2]
                kz = kzs[gi % 2]
                q = [q_s[c, pl.ds(z + r, RB), :] for c in range(8)]
                if gi >= 1:
                    dep = pltpu.bitcast(den, I32) & zv
                    q = [gate(t, dep) for t in q]
                g = gb[r:r + RB, :]
                s = []
                raw = None
                for w in range(W):
                    st = HALO + r - DIL * w
                    q0 = q[0] if raw is None else after(q[0], raw)
                    acc = q0 * k_s[0, pl.ds(kz + st, RB), :]
                    for c in range(1, 8):
                        acc = acc + q[c] * k_s[c, pl.ds(kz + st, RB), :]
                    raw = acc
                    acc = acc + pltpu.roll(acc, 64, 1)
                    acc = acc + pltpu.roll(acc, 32, 1)
                    if r < HALO and w > 0:
                        pos = i * TM + r + lax.broadcasted_iota(I32, (RB, 128), 0)
                        acc = jnp.where(pos >= DIL * w, acc, -1e9 / SCALE)
                    s.append(acc)
                mx = s[0]
                for w in range(1, W):
                    mx = jnp.maximum(mx, s[w])
                e = [jnp.exp2((s[w] - mx) * cexp) for w in range(W)]
                den = e[0]
                for w in range(1, W):
                    den = den + e[w]
                inv = g / den
                pks = []
                for c in range(8):
                    st = HALO + r
                    e0 = e[0] if last_o is None else after(e[0], last_o)
                    acc = e0 * v_s[c, pl.ds(kz + st, RB), :]
                    for w in range(1, W):
                        st = HALO + r - DIL * w
                        acc = acc + e[w] * v_s[c, pl.ds(kz + st, RB), :]
                    last_o = acc
                    acc = acc * inv
                    if gi % 2 == 0:
                        pend[c] = acc
                    else:
                        pks.append(_u(_cat([pend[c], acc], axis=0).astype(BF)))
                if gi % 2 == 1:
                    w0 = (r - RB) // 2
                    if r < HM:
                        for c in range(8):
                            oa_v[c, w0:w0 + 8, :] = pks[c]
                    else:
                        w1 = w0 - 64
                        for t in range(4):
                            oa_v[t + 4, w0:w0 + 8, :] = pks[t + 4]
                            blk = [oa_v[t, w1:w1 + 8, :], oa_v[t + 4, w1:w1 + 8, :], pks[t], pks[t + 4]]
                            sm = _packed_sums(_lhs_sums, blk)
                            for k in range(5):
                                oas[k * 4 + t, w1:w1 + 8, :] = sm[k]

            hsb = hs.at[:, :, pl.ds(_al(i * HM, HM), HM)]
            bb = _combine({k: _dot(_cat([hsb[k - 1, t] for t in range(KD)]),
                                   _cat([_bf(wd7[(k - 1) * 4 + t]) for t in range(4)]))
                           for k in (2, 4, 3, 5, 1, 7, 6)})

            def lhs_o(k):
                if k == 3:
                    return _cat([_bf(oa_v[t, 0:64, :]) for t in range(4)])
                if k == 4:
                    return _cat([_bf(oa_v[t + 4, 64:128, :]) for t in range(4)])
                return _cat([_bf(oas[LSUM[k] * 4 + t]) for t in range(4)])

            mm = {k: _dot(lhs_o(k), _cat([_bf(wo7[(k - 1) * 4 + t]) for t in range(4)]))
                  for k in (3, 4, 2, 5, 1, 7, 6)}
            omg = 1.0 - gb[...]
            ob = [_cat([omg[(n // 2) * HM:(n // 2 + 1) * HM]] * 4) * bb[n] for n in range(4)]
            fin = {2: (ob[2] + mm[4]) + mm[2],
                   1: (ob[1] + mm[3]) + mm[5],
                   0: (ob[0] + mm[4] - mm[5] + mm[1]) + mm[7],
                   3: (ob[3] + mm[3] - mm[2] + mm[1]) + mm[6]}
            for n in (2, 1, 0, 3):
                ro = (n // 2) * HM
                co = (n % 2) * 512
                if n != 3:
                    pieces = [(0, HM, 0, 512)]
                else:
                    pieces = [(0, HM, 0, 256), (0, HM, 256, 128), (0, 64, 384, 128), (64, 64, 384, 128)]
                for (pr, pn, pc, pw) in pieces:
                    rs = pl.ds(_al(r0 + ro + pr, pn), pn)
                    cs = slice(co + pc, co + pc + pw)
                    out_v[rs, cs] = fin[n][pr:pr + pn, pc:pc + pw].astype(BF)
                    pltpu.make_async_copy(out_v.at[rs, cs], o_hbm.at[rs, cs], sems.at[SOUT]).start()
            return carry
        lax.fori_loop(0, NB, main2, 0)
        pltpu.make_async_copy(out_v, o_hbm, sems.at[SOUT]).wait()

    @pl.when(pl.program_id(0) == 0)
    def _():
        pl.run_scoped(
            phase1,
            pltpu.VMEM((D, 3 * D), BF),
            pltpu.VMEM((D, D), BF),
            pltpu.VMEM((2, 1088, 128), F32),
            pltpu.VMEM((4, D, 128), BF),
            pltpu.VMEM((4, D, 128), BF),
            pltpu.VMEM((NFC - 1, D, FC), BF),
            pltpu.VMEM((NFC - 1, D, FC), BF),
            pltpu.VMEM((20, 256, 128), U32),
            pltpu.VMEM((F, D), BF),
            pltpu.VMEM((4, 2 * TM, 128), BF),
            pltpu.VMEM((8 * D,), BF),
        )

    @pl.when(pl.program_id(0) == 1)
    def _():
        pl.run_scoped(
            phase2,
            pltpu.VMEM((8, TM, 128), F32),
            pltpu.VMEM((8, S + HALO, 128), F32),
            pltpu.VMEM((8, S + HALO, 128), F32),
            pltpu.VMEM((8, 128, 128), U32),
            pltpu.VMEM((20, 64, 128), U32),
            pltpu.VMEM((S, D), BF),
        )


@jax.jit
def pallas_gated_mix__sliding_local_dilated__glu_gated_reglu__prompt_kernel(
    A_x: jax.Array,
    A_wqkv: jax.Array,
    A_wo: jax.Array,
    B_x: jax.Array,
    B_W_gate: jax.Array,
    B_W_up: jax.Array,
    B_W_down: jax.Array,
    gate_w: jax.Array,
):
    anyspec = pl.BlockSpec(memory_space=pl.ANY)
    out = pl.pallas_call(
        _kernel,
        grid=(2,),
        in_specs=[anyspec] * 7,
        out_specs=anyspec,
        out_shape=jax.ShapeDtypeStruct((S, D), BF),
        scratch_shapes=[
            pltpu.VMEM((S, D), BF),
            pltpu.VMEM((20, 512, 128), U32),
            pltpu.VMEM((16, 512, 128), U32),
            pltpu.VMEM((28, 256, 128), U32),
            pltpu.VMEM((28, 256, 128), U32),
            pltpu.VMEM((28, F // 4, 128), U32),
            pltpu.VMEM((7, KD, S // 2, 128), BF),
            pltpu.VMEM((S, 128), F32),
            pltpu.SemaphoreType.DMA((NSEM,)),
        ],
        compiler_params=pltpu.CompilerParams(
            vmem_limit_bytes=120 * 1024 * 1024,
            disable_bounds_checks=True,
            disable_semaphore_checks=True,
            dimension_semantics=("arbitrary",)),
    )(A_x.reshape(S, D), gate_w, A_wqkv, A_wo, B_W_gate, B_W_up, B_W_down)
    return out.reshape(1, S, D)
```

```python
import jax
import jax.numpy as jnp
from jax import lax
import jax.experimental.pallas as pl
import jax.experimental.pallas.tpu as pltpu

S, D, F = 2048, 1024, 3584
H, DH, W, DIL = 32, 32, 8, 2
HALO = 16
LOG2E = 1.4426950408889634
SCALE = DH ** -0.5
BF = jnp.bfloat16
F32 = jnp.float32
U32 = jnp.uint32
I32 = jnp.int32

TM = 256
HM = TM // 2
RB = 8
FC = 512
NFC = F // FC
NB = S // TM
KD = F // 256
NU2 = 3
QH = 96
SM, SX, SR, SOUT, NSEM = 0, 6, 6, 7, 8


def _swap(vs, bit, lane):
    out = list(vs)
    sh = 1 << bit
    hi = (lane & sh) != 0
    for i in range(8):
        if i & sh:
            continue
        a, b = vs[i], vs[i | sh]
        out[i] = jnp.where(hi, pltpu.roll(b, sh, 1), a)
        out[i | sh] = jnp.where(hi, b, pltpu.roll(a, 128 - sh, 1))
    return out


def _permute_cols(vs, lane):
    for bit in range(3):
        vs = _swap(vs, bit, lane)
    idx = ((lane & 3) << 5) | ((lane >> 5) << 3) | ((lane >> 2) & 7)
    return [jnp.take_along_axis(v, idx, axis=1) for v in vs]


def _dot(a, b):
    return jnp.dot(a, b, preferred_element_type=F32)


def _shr(x, n):
    return x >> n if isinstance(x, int) else lax.shift_right_logical(x, n)


def _al(x, n):
    return x if isinstance(x, int) else pl.multiple_of(x, n)


def _u(x):
    return pltpu.bitcast(x, U32)


def _bf(x):
    return pltpu.bitcast(x, BF)


def _f(x):
    return pltpu.bitcast(x, F32)


def _pk(x):
    return _u(x.astype(BF))


def _gated(x, dep):
    return _f(_u(x.astype(F32)) | jnp.concatenate([dep, dep], axis=0))


def _cat(xs, axis=1):
    return xs[0] if len(xs) == 1 else jnp.concatenate(xs, axis=axis)


def _lhs_sums(a11, a12, a21, a22):
    return [a11 + a22, a21 + a22, a11 + a12, a21 - a11, a12 - a22]


def _rhs_sums(b11, b12, b21, b22):
    return [b11 + b22, b12 - b22, b21 - b11, b11 + b12, b21 + b22]


LSUM = {1: 0, 2: 1, 5: 2, 6: 3, 7: 4}
RSUM = {1: 0, 3: 1, 4: 2, 6: 3, 7: 4}


def _lhs7(blocks, sums):
    o = {3: blocks[0], 4: blocks[3]}
    o.update({k: sums[n] for k, n in LSUM.items()})
    return o


def _rhs7(blocks, sums):
    o = {2: blocks[0], 5: blocks[3]}
    o.update({k: sums[n] for k, n in RSUM.items()})
    return o


def _combine(m):
    c11 = m[4] - m[5] + m[1] + m[7]
    c12 = m[3] + m[5]
    c21 = m[2] + m[4]
    c22 = m[3] - m[2] + m[1] + m[6]
    return c11, c12, c21, c22


def _ticker(prods, zv, n, lo, hi):
    slots = []
    for pr in prods:
        for t in range(pr.shape[1] // 128):
            for r in range(0, pr.shape[0], 8):
                slots.append((pr, r, t))
    for k in range(n):
        pr, r, t = slots[min(int((lo + (hi - lo) * k / n) * len(slots)), len(slots) - 1)]
        yield _u(pr[r:r + 8, t * 128:(t + 1) * 128]) & zv


def _kernel(x_hbm, gw_hbm, wqkv_hbm, wo_hbm, wg_hbm, wu_hbm, wd_hbm, o_hbm,
            x_v, xs, wqk, wv7, wo7, wd7, hs, g_s, sems):

    def x_raw(i, half, kh):
        return x_v[pl.ds(_al(i * TM + half * HM, HM), HM), kh * 512:(kh + 1) * 512]

    def phase1(wqkv_v, wo_v, wo_f32, wg0, wu0, wg_v, wu_v, bs, wd_v, h0, gw_ref):
        def cp_x(r0, n, s):
            return pltpu.make_async_copy(x_hbm.at[pl.ds(r0, n)], x_v.at[pl.ds(r0, n)], sems.at[s])

        def cp_w0(t, s):
            c = pl.ds(_al(t * 128, 128), 128)
            return [pltpu.make_async_copy(wg_hbm.at[:, c], wg0.at[t], sems.at[s]),
                    pltpu.make_async_copy(wu_hbm.at[:, c], wu0.at[t], sems.at[s])]

        def cp_w(j):
            c = pl.ds(_al(j * FC, FC), FC)
            return [pltpu.make_async_copy(wg_hbm.at[:, c], wg_v.at[j - 1], sems.at[SM + j - 1]),
                    pltpu.make_async_copy(wu_hbm.at[:, c], wu_v.at[j - 1], sems.at[SM + j - 1])]

        def cp_q(r0, n, s):
            return [pltpu.make_async_copy(wqkv_hbm.at[kh * 512 + r0:kh * 512 + r0 + n],
                                          wqkv_v.at[kh * 512 + r0:kh * 512 + r0 + n], sems.at[s])
                    for kh in range(2)]

        cp_head = cp_q(0, QH, SM) + [
            pltpu.make_async_copy(wo_hbm, wo_v, sems.at[SM]),
            pltpu.make_async_copy(wd_hbm.at[0:2 * FC], wd_v.at[0:2 * FC], sems.at[SM]),
            pltpu.make_async_copy(gw_hbm, gw_ref.at[pl.ds(0, D)], sems.at[SM])]
        cp_rest = cp_q(QH, 512 - QH, SR) + [
            pltpu.make_async_copy(wd_hbm.at[2 * FC:F], wd_v.at[2 * FC:F], sems.at[SR])]

        first = [cp_w0(0, 1) + [cp_x(0, TM, 1)], [cp_x(TM, TM, 2)]]
        starts = sum(first, [])
        for t in range(1, 4):
            starts += cp_w0(t, 2 + t)
        starts += [cp_x((2 + b * NU2) * TM, NU2 * TM, SX + b) for b in range(6 // NU2)]
        starts += cp_w(1) + cp_head
        for c in starts:
            c.start()
        for t in range(2):
            for hh in range(H):
                wo_f32[t, hh * 33 + 32:hh * 33 + 33, :] = jnp.zeros((1, 128), F32)

        def zeros_of(i):
            zi = _shr(i, 20)
            return zi, jnp.full((8, 128), zi, I32).astype(U32)

        def ffn_plain(r0, nr, t):
            xx = x_v[pl.ds(r0, nr), :]
            gt = _dot(xx, wg0[t])
            up = _dot(xx, wu0[t])
            h0[t, pl.ds(r0, nr), :] = (jnp.maximum(gt, 0.0) * up).astype(BF)
            return [gt, up]

        def x_sums(u0, nu, tick):
            xsrc = x_v.at[pl.ds(_al(u0 * TM, TM), nu * TM)]
            xdst = xs.at[:, pl.ds(_al(u0 * 64, 64), nu * 64)]
            for u in range(nu):
                for r in range(0, HM, 16):
                    for t in range(4):
                        dep = next(tick)
                        sm = _lhs_sums(*[_gated(xsrc[u * TM + hf * HM + r:u * TM + hf * HM + r + 16,
                                                     kh * 512 + t * 128:kh * 512 + (t + 1) * 128], dep)
                                         for hf in range(2) for kh in range(2)])
                        for k in range(5):
                            xdst[k * 4 + t, u * 64 + r // 2:u * 64 + r // 2 + 8, :] = _pk(sm[k])

        def w_sums(tile, mi, t, tick):
            for r in range(0, 512, 16):
                dep = next(tick)
                sm = _rhs_sums(*[_gated(tile(nh, kh * 512 + r), dep) for kh in range(2) for nh in range(2)])
                for k in range(5):
                    bs[(mi * 5 + k) * 2 + t, r:r + 16, :] = sm[k].astype(BF)

        def store_h7(mm, hdst):
            hb = [jnp.maximum(gt, 0.0) * up for gt, up in zip(_combine(mm[0]), _combine(mm[1]))]
            h7 = _lhs7(hb, _lhs_sums(*hb))
            for k in range(1, 8):
                hv = h7[k].astype(BF)
                for t in range(2):
                    hdst[k - 1, t] = hv[:, t * 128:(t + 1) * 128]

        def warm0(u, carry):
            for k in range(2):
                @pl.when(u == k)
                def _():
                    for c in first[k]:
                        c.wait()
            pr = ffn_plain(_al(u * TM, TM), TM, 0)
            x_sums(u, 1, _ticker(pr, zeros_of(u)[1], 32, 0.0, 0.95))
            return carry
        lax.fori_loop(0, 2, warm0, 0)

        def warm1(t, carry):
            for c in cp_w0(t, 2 + t):
                c.wait()
            pr = ffn_plain(0, 2 * TM, t)
            tick = _ticker(pr, zeros_of(t)[1], 64, 0.0, 0.9)
            pi = _shr(t - 1, 1)
            for mi, w0 in enumerate((wg0, wu0)):
                wp = w0.at[pl.ds(2 * pi, 2)]
                w_sums(lambda nh, r: wp[nh, r:r + 16, :], mi, pi, tick)
            return carry
        lax.fori_loop(1, 4, warm1, 0)
        for c in cp_w(2):
            c.start()

        def warm2(b, carry):
            u0 = 2 + b * NU2
            cp_x(_al(u0 * TM, TM), NU2 * TM, SX + b).wait()
            zv = zeros_of(b)[1]
            xsb = xs.at[:, pl.ds(_al(u0 * 64, 64), NU2 * 64)]

            def lhs(k):
                if k == 3:
                    return _cat([x_raw(u0 + u, 0, 0) for u in range(NU2)], axis=0)
                if k == 4:
                    return _cat([x_raw(u0 + u, 1, 1) for u in range(NU2)], axis=0)
                return _cat([_bf(xsb[LSUM[k] * 4 + t]) for t in range(4)])

            def rhs(mi, k):
                w0 = (wg0, wu0)[mi]
                if k == 2:
                    return _cat([w0[2 * t, 0:512, :] for t in range(2)])
                if k == 5:
                    return _cat([w0[2 * t + 1, 512:1024, :] for t in range(2)])
                return _cat([bs[(mi * 5 + RSUM[k]) * 2 + t] for t in range(2)])

            mm = [{}, {}]
            prods = []
            for k in (3, 4):
                for mi in range(2):
                    mm[mi][k] = _dot(lhs(k), rhs(mi, k))
                    prods.append(mm[mi][k])
            x_sums(u0, NU2, _ticker(prods, zv, 32 * NU2, 0.0, 0.85))
            prods = []
            for k in (2, 5, 1, 7, 6):
                for mi in range(2):
                    mm[mi][k] = _dot(lhs(k), rhs(mi, k))
                    prods.append(mm[mi][k])
            tick = _ticker(prods, zv, 32, 0.05, 0.45)
            for u in range(2):
                for r in range(0, HM, 16):
                    for t in range(2):
                        dep = next(tick)
                        blk = [_gated(h0[2 * t + kh, u * TM + hf * HM + r:u * TM + hf * HM + r + 16, :], dep)
                               for hf in range(2) for kh in range(2)]
                        o7 = _lhs7(blk, _lhs_sums(*blk))
                        for k in range(1, 8):
                            hs[k - 1, t, u * HM + r:u * HM + r + 16, :] = o7[k].astype(BF)
            store_h7(mm, hs.at[:, 0:2, pl.ds(_al(u0 * HM, HM), NU2 * HM)])
            return carry
        lax.fori_loop(0, 6 // NU2, warm2, 0)

        for c in cp_rest:
            c.start()
        for j in range(3, NFC):
            for c in cp_w(j):
                c.start()
        for c in cp_head:
            c.wait()

        def main1(j, carry):
            @pl.when(j == 2)
            def _():
                for c in cp_rest:
                    c.wait()
            for c in cp_w(j):
                c.wait()

            zj, zv = zeros_of(j)
            p = j - 1
            wsrc = [wg_v.at[p], wu_v.at[p]]

            def lhs(k):
                if k == 3:
                    return _cat([x_raw(i, 0, 0) for i in range(NB)], axis=0)
                if k == 4:
                    return _cat([x_raw(i, 1, 1) for i in range(NB)], axis=0)
                return _cat([_bf(xs[LSUM[k] * 4 + t]) for t in range(4)])

            def rhs(mi, k):
                if k == 2:
                    return _cat([wsrc[mi][0:512, 2 * t * 128:(2 * t + 1) * 128] for t in range(2)])
                if k == 5:
                    return _cat([wsrc[mi][512:1024, (2 * t + 1) * 128:(2 * t + 2) * 128] for t in range(2)])
                return _cat([bs[zj + (mi * 5 + RSUM[k]) * 2 + t] for t in range(2)])

            mm = [{}, {}]
            prods = []
            for mi, k in [(0, 2), (0, 5), (1, 2), (1, 5)]:
                mm[mi][k] = _dot(lhs(k), rhs(mi, k))
                prods.append(mm[mi][k])
            tick = _ticker(prods, zv, 128, 0.0, 0.95)
            for mi in range(2):
                for t in range(2):
                    w_sums(lambda nh, r: wsrc[mi][r:r + 16, (2 * t + nh) * 128:(2 * t + nh + 1) * 128], mi, t, tick)
            for k in (4, 3, 1, 7, 6):
                for mi in range(2):
                    mm[mi][k] = _dot(lhs(k), rhs(mi, k))
                    prods.append(mm[mi][k])
            store_h7(mm, hs.at[:, pl.ds(2 * j, 2)])

            tick = _ticker(prods, zv, 80, 0.3, 0.78)
            q0 = jnp.minimum(5 * p, 23)
            for e in range(5):
                qq = q0 + e
                sub = qq & 3
                rsrc = _shr(qq, 2) * FC + _shr(sub, 1) * 256 + (sub & 1) * 64
                dsrc = [wd_v.at[pl.ds(_al(rsrc + kh * 128, 64), 64)] for kh in range(2)]
                ddst = wd7.at[:, pl.ds(_al(qq * 32, 32), 32)]
                for r in range(0, 64, 16):
                    for t in range(4):
                        dep = next(tick)
                        blk = [_u(dsrc[kh][r:r + 16, nh * 512 + t * 128:nh * 512 + (t + 1) * 128]) | dep
                               for kh in range(2) for nh in range(2)]
                        o7 = _rhs7(blk, [_pk(v) for v in _rhs_sums(*[_bf(v).astype(F32) for v in blk])])
                        for k in range(1, 8):
                            ddst[(k - 1) * 4 + t, r // 2:r // 2 + 8, :] = o7[k]

            tick = _ticker(prods, zv, 44, 0.3 + 0.003, 0.78)
            gr = _al(jnp.minimum(p * 352, S - 352), 32)
            xg = x_v.at[pl.ds(gr, 352)]
            gdst = g_s.at[pl.ds(gr, 352)]
            gw = gw_ref[pl.ds(0, D)].astype(F32).reshape(1, D)
            for r in range(0, 352, 8):
                dep = next(tick)
                xf = xg[r:r + 8, :].astype(F32)
                xf = [_f(_u(xf[:, c * 128:(c + 1) * 128]) | dep) for c in range(8)]
                zg = xf[0] * gw[:, 0:128]
                for c in range(1, 8):
                    zg = zg + xf[c] * gw[:, c * 128:(c + 1) * 128]
                gdst[r:r + 8, :] = jax.nn.sigmoid(
                    jnp.broadcast_to(jnp.sum(zg, axis=-1, keepdims=True), (8, 128)))

            lane = lax.broadcasted_iota(I32, (8, 128), 1)
            qr = _al(jnp.minimum(p * QH, 512 - QH), 16)
            qsrc = [wqkv_v.at[pl.ds(kh * 512 + qr, QH)] for kh in range(2)]
            qw = _al(_shr(qr, 1), 8)
            qdst = [wqk.at[:, pl.ds(kh * 256 + qw, QH // 2)] for kh in range(2)]
            vdst = wv7.at[:, pl.ds(qw, QH // 2)]
            tick = _ticker(prods, zv, 36, 0.0, 0.78 - 0.04)
            tick2 = _ticker(prods, zv, 36 * 2, 0.04, 0.78 + 0.01)
            for r in range(0, QH, 16):
                pv = []
                for m in (2, 0, 1):
                    for kh in range(2):
                        dep = next(tick)
                        vs = _permute_cols([_u(qsrc[kh][r:r + 16, m * D + c * 128:m * D + (c + 1) * 128]) | dep
                                            for c in range(8)], lane)
                        if m == 2:
                            pv.append(vs)
                        else:
                            for c in range(8):
                                qdst[kh][m * 8 + c, r // 2:r // 2 + 8, :] = vs[c]
                for t in range(4):
                    for _ in range(3):
                        dep = next(tick2)
                    blk = [v | dep for v in (pv[0][t], pv[0][t + 4], pv[1][t], pv[1][t + 4])]
                    o7 = _rhs7(blk, [_pk(v) for v in _rhs_sums(*[_bf(v).astype(F32) for v in blk])])
                    for k in range(1, 8):
                        vdst[(k - 1) * 4 + t, r // 2:r // 2 + 8, :] = o7[k]

            pb = jnp.minimum(p, 3)
            osrc = [wo_v.at[:, pl.ds(_al((pb + 4 * t) * 128, 128), 128)] for t in range(2)]
            tick = _ticker(prods, zv, 64, 0.002, 0.3)
            for hh in range(H):
                for t in range(2):
                    dep = next(tick)
                    for q in range(2):
                        wo_f32[t, hh * 33 + q * 16:hh * 33 + (q + 1) * 16, :] = _gated(
                            osrc[t][hh * 32 + q * 16:hh * 32 + (q + 1) * 16, :], dep)
            tick = _ticker(prods, zv, 32, 0.3 + 0.01, 0.78)
            for b in range(4):
                for a in range(4):
                    for q in range(2):
                        dep = next(tick)
                        blk = [_cat([_f(_u(wo_f32[
                            t, pl.ds(a * 8 + b + 4 * kh + (q * 16 + e * 8) * 33, 8, stride=33), :]) | dep)
                            for e in range(2)], axis=0) for kh in range(2) for t in range(2)]
                        o7 = _rhs7(blk, _rhs_sums(*blk))
                        r = (b * 128 + a * 32 + q * 16) // 2
                        for k in range(1, 8):
                            wo7[(k - 1) * 4 + pb, r:r + 8, :] = _pk(o7[k])
            return carry
        lax.fori_loop(1, NFC, main1, 0)

    def phase2(q_s, k_s, v_s, of_s, oas, out_v):
        k_s[:, 0:HALO, :] = jnp.zeros((8, HALO, 128), F32)
        cexp = SCALE * LOG2E

        def main2(i, carry):
            r0 = _al(i * TM, TM)
            xsb = xs.at[:, pl.ds(_al(i * 64, 64), 64)]

            def lhs_x(k):
                if k == 3:
                    return x_raw(i, 0, 0)
                if k == 4:
                    return x_raw(i, 1, 1)
                return _cat([_bf(xsb[LSUM[k] * 4 + t]) for t in range(4)])

            for m in range(3):
                if m < 2:
                    full = _dot(x_v[pl.ds(r0, TM), :], _cat([_bf(wqk[m * 8 + c]) for c in range(8)]))
                    cbs = [full[hf * HM:(hf + 1) * HM, nh * 512:(nh + 1) * 512] for hf in range(2) for nh in range(2)]
                else:
                    cbs = _combine({k: _dot(lhs_x(k), _cat([_bf(wv7[(k - 1) * 4 + t]) for t in range(4)]))
                                    for k in (2, 4, 3, 5, 1, 7, 6)})
                for n, cb in enumerate(cbs):
                    for t in range(4):
                        val = cb[:, t * 128:(t + 1) * 128]
                        c = (n % 2) * 4 + t
                        ro = (n // 2) * HM
                        if m == 0:
                            q_s[c, ro:ro + HM, :] = val
                        else:
                            (k_s, v_s)[m - 1][c, pl.ds(r0 + HALO + ro, HM), :] = val
            for c in range(8):
                v_s[c, 0:HALO, :] = jnp.broadcast_to(v_s[c, HALO:HALO + 1, :], (HALO, 128))

            zs = [_shr(i, 20), _shr(i, 21)]
            kzs = [r0 + zz for zz in zs]
            zv = jnp.full((RB, 128), zs[0], I32)
            gb = g_s.at[pl.ds(r0, TM)]

            def gate(t, dep):
                return pltpu.bitcast(pltpu.bitcast(t, I32) | dep, F32)

            def after(t, dep):
                return gate(t, pltpu.bitcast(dep, I32) & zv)
            den = None
            last_o = None
            pend = [None] * 8
            for gi, r in enumerate(range(0, TM, RB)):
                z = zs[gi % 2]
                kz = kzs[gi % 2]
                q = [q_s[c, pl.ds(z + r, RB), :] for c in range(8)]
                if gi >= 1:
                    dep = pltpu.bitcast(den, I32) & zv
                    q = [gate(t, dep) for t in q]
                g = gb[r:r + RB, :]
                s = []
                raw = None
                for w in range(W):
                    st = HALO + r - DIL * w
                    q0 = q[0] if raw is None else after(q[0], raw)
                    acc = q0 * k_s[0, pl.ds(kz + st, RB), :]
                    for c in range(1, 8):
                        acc = acc + q[c] * k_s[c, pl.ds(kz + st, RB), :]
                    raw = acc
                    acc = acc + pltpu.roll(acc, 64, 1)
                    acc = acc + pltpu.roll(acc, 32, 1)
                    if r < HALO and w > 0:
                        pos = i * TM + r + lax.broadcasted_iota(I32, (RB, 128), 0)
                        acc = jnp.where(pos >= DIL * w, acc, -1e9 / SCALE)
                    s.append(acc)
                mx = s[0]
                for w in range(1, W):
                    mx = jnp.maximum(mx, s[w])
                e = [jnp.exp2((s[w] - mx) * cexp) for w in range(W)]
                den = e[0]
                for w in range(1, W):
                    den = den + e[w]
                inv = g / den
                pks = []
                for c in range(8):
                    st = HALO + r
                    e0 = e[0] if last_o is None else after(e[0], last_o)
                    acc = e0 * v_s[c, pl.ds(kz + st, RB), :]
                    for w in range(1, W):
                        st = HALO + r - DIL * w
                        acc = acc + e[w] * v_s[c, pl.ds(kz + st, RB), :]
                    last_o = acc
                    acc = acc * inv
                    if gi % 2 == 0:
                        pend[c] = acc
                    else:
                        pks.append(_cat([pend[c], acc], axis=0))
                if gi % 2 == 1:
                    w0 = r - RB
                    if r < HM:
                        for c in range(8):
                            of_s[c, w0:w0 + 16, :] = pks[c]
                        for t in range(4):
                            oas[20 + t, w0 // 2:w0 // 2 + 8, :] = _pk(pks[t])
                    else:
                        w1 = w0 - HM
                        for t in range(4):
                            oas[24 + t, w1 // 2:w1 // 2 + 8, :] = _pk(pks[t + 4])
                            sm = _lhs_sums(of_s[t, w1:w1 + 16, :], of_s[t + 4, w1:w1 + 16, :], pks[t], pks[t + 4])
                            for k in range(5):
                                oas[k * 4 + t, w1 // 2:w1 // 2 + 8, :] = _pk(sm[k])

            hsb = hs.at[:, :, pl.ds(_al(i * HM, HM), HM)]
            bb = _combine({k: _dot(_cat([hsb[k - 1, t] for t in range(KD)]),
                                   _cat([_bf(wd7[(k - 1) * 4 + t]) for t in range(4)]))
                           for k in (2, 4, 3, 5, 1, 7, 6)})

            def lhs_o(k):
                if k == 3:
                    return _cat([_bf(oas[20 + t]) for t in range(4)])
                if k == 4:
                    return _cat([_bf(oas[24 + t]) for t in range(4)])
                return _cat([_bf(oas[LSUM[k] * 4 + t]) for t in range(4)])

            mm = {k: _dot(lhs_o(k), _cat([_bf(wo7[(k - 1) * 4 + t]) for t in range(4)]))
                  for k in (3, 4, 2, 5, 1, 7, 6)}
            omg = 1.0 - gb[...]
            ob = [_cat([omg[(n // 2) * HM:(n // 2 + 1) * HM]] * 4) * bb[n] for n in range(4)]
            fin = {2: (ob[2] + mm[4]) + mm[2],
                   1: (ob[1] + mm[3]) + mm[5],
                   0: (ob[0] + mm[4] - mm[5] + mm[1]) + mm[7],
                   3: (ob[3] + mm[3] - mm[2] + mm[1]) + mm[6]}
            for n in (2, 1, 0, 3):
                ro = (n // 2) * HM
                co = (n % 2) * 512
                if n != 3:
                    pieces = [(0, HM, 0, 512)]
                else:
                    pieces = [(0, HM, 0, 256), (0, HM, 256, 128), (0, 64, 384, 128), (64, 64, 384, 128)]
                for (pr, pn, pc, pw) in pieces:
                    rs = pl.ds(_al(r0 + ro + pr, pn), pn)
                    cs = slice(co + pc, co + pc + pw)
                    out_v[rs, cs] = fin[n][pr:pr + pn, pc:pc + pw].astype(BF)
                    pltpu.make_async_copy(out_v.at[rs, cs], o_hbm.at[rs, cs], sems.at[SOUT]).start()
            return carry
        lax.fori_loop(0, NB, main2, 0)
        pltpu.make_async_copy(out_v, o_hbm, sems.at[SOUT]).wait()

    @pl.when(pl.program_id(0) == 0)
    def _():
        pl.run_scoped(
            phase1,
            pltpu.VMEM((D, 3 * D), BF),
            pltpu.VMEM((D, D), BF),
            pltpu.VMEM((2, 1088, 128), F32),
            pltpu.VMEM((4, D, 128), BF),
            pltpu.VMEM((4, D, 128), BF),
            pltpu.VMEM((NFC - 1, D, FC), BF),
            pltpu.VMEM((NFC - 1, D, FC), BF),
            pltpu.VMEM((20, 512, 128), BF),
            pltpu.VMEM((F, D), BF),
            pltpu.VMEM((4, 2 * TM, 128), BF),
            pltpu.VMEM((8 * D,), BF),
        )

    @pl.when(pl.program_id(0) == 1)
    def _():
        pl.run_scoped(
            phase2,
            pltpu.VMEM((8, TM, 128), F32),
            pltpu.VMEM((8, S + HALO, 128), F32),
            pltpu.VMEM((8, S + HALO, 128), F32),
            pltpu.VMEM((8, HM, 128), F32),
            pltpu.VMEM((28, 64, 128), U32),
            pltpu.VMEM((S, D), BF),
        )


@jax.jit
def pallas_gated_mix__sliding_local_dilated__glu_gated_reglu__prompt_kernel(
    A_x: jax.Array,
    A_wqkv: jax.Array,
    A_wo: jax.Array,
    B_x: jax.Array,
    B_W_gate: jax.Array,
    B_W_up: jax.Array,
    B_W_down: jax.Array,
    gate_w: jax.Array,
):
    anyspec = pl.BlockSpec(memory_space=pl.ANY)
    out = pl.pallas_call(
        _kernel,
        grid=(2,),
        in_specs=[anyspec] * 7,
        out_specs=anyspec,
        out_shape=jax.ShapeDtypeStruct((S, D), BF),
        scratch_shapes=[
            pltpu.VMEM((S, D), BF),
            pltpu.VMEM((20, 512, 128), U32),
            pltpu.VMEM((16, 512, 128), U32),
            pltpu.VMEM((28, 256, 128), U32),
            pltpu.VMEM((28, 256, 128), U32),
            pltpu.VMEM((28, F // 4, 128), U32),
            pltpu.VMEM((7, KD, S // 2, 128), BF),
            pltpu.VMEM((S, 128), F32),
            pltpu.SemaphoreType.DMA((NSEM,)),
        ],
        compiler_params=pltpu.CompilerParams(
            vmem_limit_bytes=120 * 1024 * 1024,
            disable_bounds_checks=True,
            disable_semaphore_checks=True,
            dimension_semantics=("arbitrary",)),
    )(A_x.reshape(S, D), gate_w, A_wqkv, A_wo, B_W_gate, B_W_up, B_W_down)
    return out.reshape(1, S, D)
```
